```python
import jax
import jax.numpy as jnp

def _softmax(x, axis=-1):
    return jax.nn.softmax(x, axis=axis)

def _gelu(x):
    return jax.nn.gelu(x, approximate=True)

def _silu(x):
    return jax.nn.silu(x)

def _sigmoid(x):
    return jax.nn.sigmoid(x)

def _layernorm(x, axis=-1, eps=1e-05):
    m = jnp.mean(x, axis=axis, keepdims=True)
    v = jnp.var(x, axis=axis, keepdims=True)
    return (x - m) / jnp.sqrt(v + eps)

def _scatter_add(tgt, idx, src, axis=0):
    return tgt.at[idx].add(src)

def _segment_sum(src, seg, n):
    return jax.ops.segment_sum(src, seg, n)

class _Rng:

    def __init__(self, key):
        self._k = key

    def _next(self):
        self._k, sub = jax.random.split(self._k)
        return sub

    def normal(self, shape):
        return jax.random.normal(self._next(), shape, dtype=jnp.bfloat16)

    def randint(self, lo, hi, shape):
        return jax.random.randint(self._next(), shape, lo, hi, dtype=jnp.int32)

    def uniform(self, shape, lo=0.0, hi=1.0):
        return jax.random.uniform(self._next(), shape, jnp.bfloat16, lo, hi)

    def permutation(self, n):
        return jax.random.permutation(self._next(), n)
kernel_name = 'adaLN_cond__ssm_conv_h3__glu_gated_reglu__prompt'

def setup_inputs():
    _rng = _Rng(jax.random.key(int.from_bytes(__import__("os").urandom(4), "little")))
    _w = lambda a: (lambda t: t.astype(jnp.bfloat16) if jnp.issubdtype(t.dtype, jnp.floating) else t)(jnp.asarray(a))

    def _A_setup():
        B, S, D = (1, 2048, 640)
        ks = 4
        return {'q': _w((lambda *s: _rng.normal(s) * 0.05)(B, S, D)), 'k': _w((lambda *s: _rng.normal(s) * 0.05)(B, S, D)), 'v': _w((lambda *s: _rng.normal(s) * 0.05)(B, S, D)), 'shift_k': _w((lambda *s: _rng.normal(s) * 0.05)(D, ks) * 0.5), 'ssm_k': _w((lambda *s: _rng.normal(s) * 0.05)(D, S) * (1.0 / S ** 0.5)), 'ssm_D': _w((lambda *s: _rng.normal(s) * 0.05)(D))}
    _A_in = _A_setup()

    def _B_setup():
        B, S, D, F = (1, 2048, 640, 1536)
        return {'x': _w((lambda *s: _rng.normal(s) * 0.05)(B, S, D)), 'W_gate': _w((lambda *s: _rng.normal(s) * 0.05)(D, F) * (2.0 / D) ** 0.5), 'W_up': _w((lambda *s: _rng.normal(s) * 0.05)(D, F) * (2.0 / D) ** 0.5), 'W_down': _w((lambda *s: _rng.normal(s) * 0.05)(F, D) * (1.0 / F) ** 0.5)}
    _B_in = _B_setup()
    return {'A_q': _A_in['q'], 'A_k': _A_in['k'], 'A_v': _A_in['v'], 'A_shift_k': _A_in['shift_k'], 'A_ssm_k': _A_in['ssm_k'], 'A_ssm_D': _A_in['ssm_D'], 'B_x': _B_in['x'], 'B_W_gate': _B_in['W_gate'], 'B_W_up': _B_in['W_up'], 'B_W_down': _B_in['W_down'], 'c': _w((lambda *s: _rng.normal(s) * 0.05)(1, 640)), 'w_mod': _w((lambda *s: _rng.normal(s) * 0.05)(640, 6 * 640) * 640 ** (-0.5))}

def reference(A_q, A_k, A_v, A_shift_k, A_ssm_k, A_ssm_D, B_x, B_W_gate, B_W_up, B_W_down, c, w_mod):

    def _A_ref(q, k, v, shift_k, ssm_k, ssm_D):
        B, S, D = q.shape
        ks = shift_k.shape[-1]
        k_pad = jnp.pad(k, ((0, 0), (ks - 1, 0), (0, 0)))
        k_shift = jnp.zeros_like(k)
        for t in range(ks):
            k_shift = k_shift + k_pad[:, t:t + S, :] * shift_k[:, ks - 1 - t][None, None, :]
        kv = k_shift * v
        L = 2 * S
        kv_pad = jnp.pad(kv, ((0, 0), (0, S), (0, 0)))
        kf_pad = jnp.pad(ssm_k, ((0, 0), (0, S)))
        kv_f = (lambda x, axes=(-2, -1): jnp.fft.rfft2(x.astype(jnp.float32), axes=axes))(kv_pad[:, None, :, :], axes=(1, 2))
        kf_f = (lambda x, axes=(-2, -1): jnp.fft.rfft2(x.astype(jnp.float32), axes=axes))(kf_pad[:, None, :], axes=(1, 2))
        kf_f = (lambda x, *d: x.transpose(*d))(kf_f, 1, 2, 0)
        y_f = kv_f * kf_f[None, :, :, :]
        y = (lambda x, s, axes=(-2, -1): jnp.fft.irfft2(x, s=s, axes=axes).astype(jnp.bfloat16))(y_f, (1, L), axes=(1, 2))[:, 0, :S, :]
        y = y + kv * ssm_D[None, None, :]
        return q * y

    def _B_ref(x, W_gate, W_up, W_down):
        gate = jnp.einsum('bsd,df->bsf', x, W_gate)
        up = jnp.einsum('bsd,df->bsf', x, W_up)
        gate = gate * (lambda x, dt: x.astype(dt))(gate > 0, gate.dtype)
        h = gate * up
        return jnp.einsum('bsf,fd->bsd', h, W_down)
    x = A_q
    mod = (_silu(c) @ w_mod).reshape(c.shape[0], 6, 1, -1)
    sa, ca, ga, sb, cb, gb = (mod[:, 0].copy(), mod[:, 1].copy(), mod[:, 2].copy(), mod[:, 3].copy(), mod[:, 4].copy(), mod[:, 5].copy())
    h = _layernorm(x, axis=-1) * (1 + ca) + sa
    x = x + ga * _A_ref(h, A_k, A_v, A_shift_k, A_ssm_k, A_ssm_D)
    h = _layernorm(x, axis=-1) * (1 + cb) + sb
    x = x + gb * _B_ref(h, B_W_gate, B_W_up, B_W_down)
    return x
```

```python
import functools

import numpy as np
import jax
import jax.numpy as jnp
from jax import lax
import jax.experimental.pallas as pl
import jax.experimental.pallas.tpu as pltpu

S = 2048
D = 640
FF = 1536
CH = 128
NCH = S // CH
TM = 256
NB = S // TM
EPS = 1e-5


def _dft_tables():
    f = np.concatenate([np.arange(0, CH, 2), np.arange(1, CH, 2)])
    n = np.arange(CH)
    k = ((2 * f[:, None] + 1) * n[None, :]) % (4 * CH)
    ang = np.pi * k / (2 * CH)
    fwd = np.concatenate([np.cos(ang), np.sin(ang)], axis=0)
    inv = fwd.T / CH
    return fwd.astype(np.float32), inv.astype(np.float32)


def _layernorm(x):
    m = jnp.mean(x, axis=-1, keepdims=True)
    xc = x - m
    v = jnp.mean(xc * xc, axis=-1, keepdims=True)
    return xc * lax.rsqrt(v + EPS)


def _kernel(q_ref, k_ref, v_ref, sk_ref, ssmk_ref, dd_ref, wg_ref, wu_ref, wd_ref,
            c_ref, wmod_ref, f_ref, g_ref, o_ref,
            mod_ref, kprev_ref, uhat_ref, khat_ref, kraw_ref, z_ref):
    s = pl.program_id(0)

    @pl.when(s == 0)
    def _():
        c = c_ref[...].astype(jnp.float32)
        sc = (c * jax.nn.sigmoid(c)).astype(jnp.bfloat16)
        sc8 = jnp.broadcast_to(sc, (8, D))
        mod_ref[...] = jnp.dot(sc8, wmod_ref[...], preferred_element_type=jnp.float32)
        kprev_ref[...] = jnp.zeros_like(kprev_ref)
        kraw_ref[...] = jnp.zeros_like(kraw_ref)

    k = k_ref[...].astype(jnp.float32)
    kext = jnp.concatenate([kprev_ref[...], k], axis=0)
    kprev_ref[...] = k[TM - 8:, :]
    sk = sk_ref[...].astype(jnp.float32)
    ks = k * sk[0:1, :]
    for t in range(1, 4):
        ks = ks + kext[8 - t:8 - t + TM, :] * sk[t:t + 1, :]
    kv = ks * v_ref[...].astype(jnp.float32)
    kvb = kv.astype(jnp.bfloat16)
    kv = kvb.astype(jnp.float32)

    fm = f_ref[...]
    h = CH // 2
    for cc in range(2):
        uhat_ref[2 * s + cc] = jnp.dot(fm, kvb[cc * CH:(cc + 1) * CH, :],
                                       preferred_element_type=jnp.float32)
        kr = lax.dot_general(fm, ssmk_ref[:, cc * CH:(cc + 1) * CH],
                             (((1,), (1,)), ((), ())), preferred_element_type=jnp.float32)
        kp = kraw_ref[...]
        khat_ref[2 * s + cc] = jnp.concatenate([
            kr[0:h] + kp[2 * h:3 * h],
            kr[h:2 * h] - kp[3 * h:4 * h],
            kr[2 * h:3 * h] - kp[0:h],
            kr[3 * h:4 * h] + kp[h:2 * h]], axis=0)
        kraw_ref[...] = kr

    def pos_body(p, carry):
        r0 = pl.multiple_of(p * 8, 8)
        r1 = pl.multiple_of(p * 8 + CH, 8)

        def ld(ref, idx):
            return ref[idx, pl.ds(r0, 8), :], ref[idx, pl.ds(r1, 8), :]

        ur, ui = ld(uhat_ref, 2 * s + 1)
        kr0, ki0 = ld(khat_ref, 0)
        b_r = kr0 * ur - ki0 * ui
        b_i = kr0 * ui + ki0 * ur
        zero = jnp.zeros((8, D), jnp.float32)

        def jbody(lag, c2):
            a_r, a_i, b_r, b_i, kar, kai = c2
            ur, ui = ld(uhat_ref, 2 * s - lag)
            kbr, kbi = ld(khat_ref, lag + 1)
            a_r = a_r + (kar * ur - kai * ui)
            a_i = a_i + (kar * ui + kai * ur)
            b_r = b_r + (kbr * ur - kbi * ui)
            b_i = b_i + (kbr * ui + kbi * ur)
            return a_r, a_i, b_r, b_i, kbr, kbi

        a_r, a_i, b_r, b_i, _, _ = lax.fori_loop(
            0, 2 * s + 1, jbody, (zero, zero, b_r, b_i, kr0, ki0))
        z_ref[0, pl.ds(r0, 8), :] = a_r
        z_ref[0, pl.ds(r1, 8), :] = a_i
        z_ref[1, pl.ds(r0, 8), :] = b_r
        z_ref[1, pl.ds(r1, 8), :] = b_i
        return carry

    lax.fori_loop(0, CH // 8, pos_body, 0)

    gm = g_ref[...]
    y = jnp.concatenate(
        [jnp.dot(gm, z_ref[cc].astype(jnp.bfloat16), preferred_element_type=jnp.float32)
         for cc in range(2)], axis=0)
    y = y + kv * dd_ref[...].astype(jnp.float32)

    mod = mod_ref[0:1, :]
    sa, ca, ga, sb, cb, gb = [mod[:, i * D:(i + 1) * D] for i in range(6)]
    x = q_ref[...].astype(jnp.float32)
    h1 = _layernorm(x) * (1.0 + ca) + sa
    x1 = x + ga * (h1 * y)
    h2 = (_layernorm(x1) * (1.0 + cb) + sb).astype(jnp.bfloat16)
    gate = jnp.dot(h2, wg_ref[...], preferred_element_type=jnp.float32)
    up = jnp.dot(h2, wu_ref[...], preferred_element_type=jnp.float32)
    act = (jnp.maximum(gate, 0.0) * up).astype(jnp.bfloat16)
    ff = jnp.dot(act, wd_ref[...], preferred_element_type=jnp.float32)
    o_ref[...] = (x1 + gb * ff).astype(o_ref.dtype)


@jax.jit
def pallas_adaLN_cond__ssm_conv_h3__glu_gated_reglu__prompt_kernel(
    A_q, A_k, A_v, A_shift_k, A_ssm_k, A_ssm_D, B_x, B_W_gate, B_W_up, B_W_down, c, w_mod,
):
    del B_x
    fwd, inv = _dft_tables()
    fwd = jnp.asarray(fwd, jnp.bfloat16)
    inv = jnp.asarray(inv, jnp.bfloat16)
    q = A_q.reshape(S, D)
    k = A_k.reshape(S, D)
    v = A_v.reshape(S, D)
    sk = A_shift_k.T
    dd = A_ssm_D.reshape(1, D)

    row = pl.BlockSpec((TM, D), lambda s: (s, 0))

    def full(shape):
        return pl.BlockSpec(shape, lambda s: (0, 0))

    out = pl.pallas_call(
        _kernel,
        grid=(NB,),
        in_specs=[row, row, row, full((4, D)),
                  pl.BlockSpec((D, TM), lambda s: (0, s)),
                  full((1, D)), full((D, FF)), full((D, FF)), full((FF, D)),
                  full((1, D)), full((D, 6 * D)), full((2 * CH, CH)), full((CH, 2 * CH))],
        out_specs=row,
        out_shape=jax.ShapeDtypeStruct((S, D), jnp.bfloat16),
        scratch_shapes=[
            pltpu.VMEM((8, 6 * D), jnp.float32),
            pltpu.VMEM((8, D), jnp.float32),
            pltpu.VMEM((NCH, 2 * CH, D), jnp.float32),
            pltpu.VMEM((NCH, 2 * CH, D), jnp.float32),
            pltpu.VMEM((2 * CH, D), jnp.float32),
            pltpu.VMEM((2, 2 * CH, D), jnp.float32),
        ],
        compiler_params=pltpu.CompilerParams(
            dimension_semantics=("arbitrary",),
            vmem_limit_bytes=100 * 1024 * 1024),
    )(q, k, v, sk, A_ssm_k, dd, B_W_gate, B_W_up, B_W_down, c, w_mod, fwd, inv)
    return out.reshape(1, S, D)
```

```python
import os
import numpy as np
import jax
import jax.numpy as jnp
from jax import lax
import jax.experimental.pallas as pl
import jax.experimental.pallas.tpu as pltpu

S = 2048
D = 640
FF = 1536
CH = 128
NCH = S // CH
TM = 256
NB = S // TM
NLT = D // 128
NP = CH // 8
EPS = 1e-5
NJA = 12
UPAD = NJA - 6
KROWS = 3 * CH + 8
UROWS = 3 * CH + 64
WCH = 4
F32 = jnp.float32
BF16 = jnp.bfloat16
U32 = jnp.uint32
VARS = os.environ.get('VARS', 'PABTU')
LNCH = int(os.environ.get('LNCH', 2))
LNGU = int(os.environ.get('LNGU', 10))
MIDWAIT = int(os.environ.get('MIDWAIT', 0))


def _dft_tables():
    f = np.concatenate([np.arange(0, CH, 2), np.arange(1, CH, 2)])
    n = np.arange(CH)
    k = ((2 * f[:, None] + 1) * n[None, :]) % (4 * CH)
    ang = np.pi * k / (2 * CH)
    co = np.cos(ang).reshape(NP, 8, CH)
    si = np.sin(ang).reshape(NP, 8, CH)
    fwd = np.stack([co, si], axis=1).reshape(2 * CH, CH)
    inv = fwd.T / CH
    return fwd.astype(np.float32), inv.astype(np.float32)


def _pack_np(a):
    u = np.ascontiguousarray(a, np.float32).view(np.uint32)
    b = ((u + 0x7FFF + ((u >> 16) & 1)) >> 16).astype(np.uint32)
    return b[0::2] | (b[1::2] << 16)


def _pack(x):
    return pltpu.bitcast(x.astype(BF16), U32)


def _unpack(x):
    return pltpu.bitcast(x, BF16)


def _kernel(q_hbm, k_hbm, v_hbm, sk_ref, ssmk_hbm, dd_ref, wg_hbm, wu_hbm, wd_hbm,
            c_ref, wmod_hbm, f_ref, g_ref, o_hbm,
            q_ref, k_ref, v_ref, o_ref, ssmk_ref, wg_ref, wu_ref, wd_ref, wmod_ref,
            sem_q, sem_k, sem_v, sem_o, sem_s, sem_m, sem_g, sem_u, sem_d,
            mod_ref, zprev_ref, z_ref, h2_ref, x1_ref, act_ref, y_ref, *hist):
    uh = hist[:NLT]
    kh = hist[NLT:]
    g = pl.program_id(0)
    thr = g - 1000
    never8 = lax.broadcasted_iota(jnp.int32, (8, 128), 0) < thr
    never_col = lax.broadcasted_iota(jnp.int32, (16, 1), 0) < thr
    z1 = lax.shift_right_logical(g, 10)
    z2 = lax.shift_right_logical(g, 11)
    chain = {}

    def link(name, m, mask=never8):
        prev = chain.get(name)
        return m if prev is None else jnp.where(mask, prev, m)

    def lanes(lt):
        return slice(lt * 128, (lt + 1) * 128)

    def rows(b, off, n, unit=TM):
        if isinstance(b, int):
            return slice(b * unit + off, b * unit + off + n)
        return pl.ds(pl.multiple_of(b * unit, unit) + off, n)

    def rows_copy(src, dst, sem, b):
        return pltpu.make_async_copy(src.at[rows(b, 0, TM)], dst.at[rows(b, 0, TM)], sem.at[b])

    def cols_copy(src, dst, sem, i, w):
        return pltpu.make_async_copy(src.at[:, pl.ds(i * w, w)], dst.at[:, pl.ds(i * w, w)], sem.at[i])

    cp_q = lambda b: rows_copy(q_hbm, q_ref, sem_q, b)
    cp_k = lambda b: rows_copy(k_hbm, k_ref, sem_k, b)
    cp_v = lambda b: rows_copy(v_hbm, v_ref, sem_v, b)
    cp_o = lambda b: rows_copy(o_ref, o_hbm, sem_o, b)
    cp_s = lambda lt: pltpu.make_async_copy(
        ssmk_hbm.at[pl.ds(lt * 128, 128)], ssmk_ref.at[pl.ds(lt * 128, 128)], sem_s.at[lt])
    cp_m = lambda i: cols_copy(wmod_hbm, wmod_ref, sem_m, i, D)
    cp_g = lambda i: cols_copy(wg_hbm, wg_ref, sem_g, i, FF // WCH)
    cp_u = lambda i: cols_copy(wu_hbm, wu_ref, sem_u, i, FF // WCH)
    cp_d = lambda: pltpu.make_async_copy(wd_hbm, wd_ref, sem_d.at[0])

    def dft_k(lt, j):
        cs = lanes(lt)
        kf = lax.dot_general(_unpack(f_ref[...]), ssmk_ref[cs, j * CH:(j + 1) * CH],
                             (((1,), (1,)), ((), ())), preferred_element_type=F32)
        for p in range(NP):
            kr = kf[16 * p:16 * p + 8]
            ki = kf[16 * p + 8:16 * p + 16]
            if j == 0:
                kr = kr + dd_ref[:, cs].astype(F32)
            kh[lt][j, 24 * p:24 * p + 8, :] = kr
            kh[lt][j, 24 * p + 8:24 * p + 16, :] = ki - kr
            kh[lt][j, 24 * p + 16:24 * p + 24, :] = kr + ki

    def dft_u(b, bsrc, lt):
        cs = lanes(lt)
        sk = sk_ref[:, cs].astype(F32)
        k = k_ref[rows(bsrc, 0, TM), cs].astype(F32)
        if isinstance(b, int) and b == 0:
            halo = jnp.zeros((8, 128), F32)
        else:
            halo = k_ref[rows(bsrc, -16, 16), cs].astype(F32)[8:]
        kext = jnp.concatenate([halo, k], axis=0)
        ks = k * sk[0:1, :]
        for t in range(1, 4):
            ks = ks + kext[8 - t:8 - t + TM, :] * sk[t:t + 1, :]
        kv = ks * v_ref[rows(bsrc, 0, TM), cs].astype(F32)
        for cc in range(2):
            uf = jnp.dot(_unpack(f_ref[...]), kv[cc * CH:(cc + 1) * CH, :].astype(BF16),
                         preferred_element_type=F32)
            for p in range(NP):
                ur = uf[16 * p:16 * p + 8]
                ui = uf[16 * p + 8:16 * p + 16]
                uh[lt][UPAD + 2 * b + cc, 24 * p:24 * p + 8, :] = ur + ui
                uh[lt][UPAD + 2 * b + cc, 24 * p + 8:24 * p + 16, :] = ur
                uh[lt][UPAD + 2 * b + cc, 24 * p + 16:24 * p + 24, :] = ui

    def mac(b, njs, lt, paced):
        cs = lanes(lt)
        uw = uh[lt].at[pl.ds(UPAD + 2 * b + 2 - njs, njs)]
        first = isinstance(b, int) and b == 0
        for p in range(NP):
            a = [None] * 3
            c = [None] * 3
            for q in range(3):
                rr = pl.ds(24 * p + 8 * q, 8)
                kprev = None
                for t in range(njs):
                    u = uw[njs - 1 - t, rr, :]
                    k = kh[lt][t, rr, :]
                    m = k * u
                    c[q] = link('c', m) if c[q] is None else c[q] + m
                    if t > 0:
                        m = kprev * u
                        a[q] = link('a', m) if a[q] is None else a[q] + m
                    kprev = k
                if paced:
                    chain['a'] = a[q]
                    chain['c'] = c[q]
            ar, ai = a[0] - a[2], a[0] + a[1]
            br, bi = c[0] - c[2], c[0] + c[1]
            if first:
                za = [ar, ai]
            else:
                pr = zprev_ref[16 * p:16 * p + 8, cs]
                pi = zprev_ref[16 * p + 8:16 * p + 16, cs]
                za = [ar + pi, ai - pr] if p < NP // 2 else [ar - pi, ai + pr]
            zprev_ref[16 * p:16 * p + 8, cs] = br
            zprev_ref[16 * p + 8:16 * p + 16, cs] = bi
            zb = [br + ai, bi - ar] if p < NP // 2 else [br - ai, bi + ar]
            z_ref[0, 16 * p:16 * p + 8, cs] = za[0]
            z_ref[0, 16 * p + 8:16 * p + 16, cs] = za[1]
            z_ref[1, 16 * p:16 * p + 8, cs] = zb[0]
            z_ref[1, 16 * p + 8:16 * p + 16, cs] = zb[1]

    def inv(lt):
        cs = lanes(lt)
        for cc in range(2):
            y_ref[z1, cc * CH:(cc + 1) * CH, cs] = jnp.dot(
                _unpack(g_ref[...]), z_ref[cc, :, cs].astype(BF16), preferred_element_type=F32)

    def norm(x, name=None):
        m = jnp.sum(x, axis=-1, keepdims=True) * (1.0 / D)
        if name is not None:
            m = link(name, m, never_col)
        xc = x - m
        v = jnp.sum(xc * xc, axis=-1, keepdims=True) * (1.0 / D)
        return xc * lax.rsqrt(v + EPS)

    def modrow(i):
        return mod_ref[0:1, i * D:(i + 1) * D]

    def ln_all(b, paced):
        RC = 16
        for r in range(TM // RC):
            name = 'ln%d' % (r % LNCH)
            x = q_ref[rows(b, r * RC, RC), :].astype(F32)
            h1 = norm(x, name) * modrow(1) + modrow(0)
            x1 = x + h1 * y_ref[z2, r * RC:(r + 1) * RC, :]
            x1_ref[rows(b, r * RC, RC), :] = x1
            h2 = norm(x1) * modrow(4) + modrow(3)
            if paced:
                chain[name] = h2[:, 0:1]
            h2_ref[rows(b, r * 8, 8, TM // 2), :] = _pack(h2)

    def gu(b, c):
        cs = lanes(c)
        h2 = _unpack(h2_ref[rows(b, 0, TM // 2, TM // 2), :])
        gate = jnp.dot(h2, wg_ref[:, cs], preferred_element_type=F32)
        up = jnp.dot(h2, wu_ref[:, cs], preferred_element_type=F32)
        act_ref[:, cs] = _pack(jnp.maximum(gate, 0.0) * up)
        if c == LNGU:
            for i in range(LNCH):
                chain['ln%d' % i] = up[0:16, 0:1]

    def down(b, c):
        cs = lanes(c)
        gb = mod_ref[0:1, 5 * D + c * 128:5 * D + (c + 1) * 128]
        ff = jnp.dot(_unpack(act_ref[...]), wd_ref[:, cs], preferred_element_type=F32)
        o_ref[rows(b, 0, TM), cs] = (x1_ref[rows(b, 0, TM), cs] + gb * ff).astype(BF16)

    def mod_part(i):
        c = c_ref[...].astype(F32)
        sc = jnp.broadcast_to((c * jax.nn.sigmoid(c)).astype(BF16), (8, D))
        return jnp.dot(sc, wmod_ref[:, i * D:(i + 1) * D], preferred_element_type=F32)

    def prologue():
        chain.clear()
        for lt in range(NLT):
            cp_s(lt).start()
        for b in range(2):
            cp_k(b).start()
            cp_v(b).start()
        cp_q(0).start()
        for i in range(3):
            cp_m(i).start()
        cp_k(2).start()
        cp_v(2).start()
        for i in (3, 4):
            cp_m(i).start()
        for i in range(WCH):
            cp_g(i).start()
            cp_u(i).start()
            if i == 0:
                cp_q(1).start()
                cp_k(3).start()
                cp_v(3).start()
        cp_d().start()
        cp_m(5).start()
        for lt in range(NLT):
            uh[lt][0:UPAD, 0:3 * CH, :] = jnp.zeros((UPAD, 3 * CH, 128), F32)
        for lt in range(NLT):
            cp_s(lt).wait()
            for j in range(NCH):
                dft_k(lt, j)
        cp_k(0).wait()
        cp_v(0).wait()
        for lt in range(NLT):
            dft_u(0, 0, lt)
        cp_k(1).wait()
        cp_v(1).wait()
        for lt in range(NLT):
            dft_u(1, 1, lt)
            mac(0, 2, lt, False)
            inv(lt)
            mac(1, 4, lt, False)
        cp_q(0).wait()
        for i in range(3):
            cp_m(i).wait()
        ga = mod_part(2)
        mod_ref[:, 0:D] = mod_part(0) * ga
        mod_ref[:, D:2 * D] = (1.0 + mod_part(1)) * ga
        cp_k(2).wait()
        cp_v(2).wait()
        for lt in range(NLT):
            dft_u(2, 2, lt)
        cp_m(3).wait()
        cp_m(4).wait()
        mod_ref[:, 3 * D:4 * D] = mod_part(3)
        mod_ref[:, 4 * D:5 * D] = 1.0 + mod_part(4)
        ln_all(0, False)
        if not MIDWAIT:
            for i in range(WCH):
                cp_g(i).wait()
                cp_u(i).wait()
            cp_d().wait()
            cp_m(5).wait()
            mod_ref[:, 5 * D:6 * D] = mod_part(5)

    def step(njs, do_ln, firstw=False):
        bf, bl, bm, bd = g - 1, g, g + 1, g + 2
        chain.clear()
        if do_ln:
            for lt in range(NLT):
                inv(lt)
        if njs:
            for lt in range(NLT):
                mac(bm, njs, lt, True)
        for c in range(FF // 128):
            if firstw and c % (FF // 128 // WCH) == 0:
                i = c // (FF // 128 // WCH)

                @pl.when(g == 1)
                def _():
                    cp_g(i).wait()
                    cp_u(i).wait()
            gu(bf, c)
        if firstw:
            @pl.when(g == 1)
            def _():
                cp_d().wait()
        for c in range(NLT):
            if njs:
                dft_u(bd, jnp.minimum(bd, NB - 1), c)
            down(bf, c)
        if do_ln:
            ln_all(bl, True)

    def variant(tag, cond, fn):
        def body():
            with jax.named_scope('var' + tag):
                if tag in VARS:
                    fn()
        pl.when(cond)(body)

    variant('P', g == 0, prologue)

    @pl.when(jnp.logical_and(g >= 1, g + 2 < NB))
    def _():
        cp_k(g + 2).wait()
        cp_v(g + 2).wait()

    @pl.when(jnp.logical_and(g >= 1, g + 3 < NB))
    def _():
        cp_k(g + 3).start()
        cp_v(g + 3).start()

    @pl.when(jnp.logical_and(g >= 1, g < NB))
    def _():
        cp_q(g).wait()

    @pl.when(jnp.logical_and(g >= 1, g + 1 < NB))
    def _():
        cp_q(g + 1).start()

    @pl.when(g >= 2)
    def _():
        cp_o(g - 2).start()

    if MIDWAIT:
        @pl.when(g == 1)
        def _():
            cp_m(5).wait()
            mod_ref[:, 5 * D:6 * D] = mod_part(5)

    variant('A', jnp.logical_and(g >= 1, g <= 4), lambda: step(NJA, True, MIDWAIT))
    variant('B', jnp.logical_and(g >= 5, g <= 6), lambda: step(NCH, True))
    variant('T', g == 7, lambda: step(0, True))
    variant('U', g == 8, lambda: step(0, False))

    @pl.when(g == NB)
    def _():
        cp_o(NB - 1).start()
        for b in range(NB):
            cp_o(b).wait()


@jax.jit
def pallas_adaLN_cond__ssm_conv_h3__glu_gated_reglu__prompt_kernel(
    A_q, A_k, A_v, A_shift_k, A_ssm_k, A_ssm_D, B_x, B_W_gate, B_W_up, B_W_down, c, w_mod,
):
    del B_x
    fwd, inv = _dft_tables()
    fwd = jnp.asarray(_pack_np(fwd))
    inv = jnp.asarray(_pack_np(inv))
    q = A_q.reshape(S, D)
    k = A_k.reshape(S, D)
    v = A_v.reshape(S, D)
    sk = A_shift_k.T
    dd = A_ssm_D.reshape(1, D)

    hbm = pl.BlockSpec(memory_space=pl.ANY)

    def full(shape):
        return pl.BlockSpec(shape, lambda s: (0, 0))

    out = pl.pallas_call(
        _kernel,
        grid=(NB + 1,),
        in_specs=[hbm, hbm, hbm, full((4, D)), hbm, full((1, D)), hbm, hbm, hbm,
                  full((1, D)), hbm, full((CH, CH)), full((CH // 2, 2 * CH))],
        out_specs=hbm,
        out_shape=jax.ShapeDtypeStruct((S, D), BF16),
        scratch_shapes=[
            pltpu.VMEM((S, D), BF16),
            pltpu.VMEM((S, D), BF16),
            pltpu.VMEM((S, D), BF16),
            pltpu.VMEM((S, D), BF16),
            pltpu.VMEM((D, S), BF16),
            pltpu.VMEM((D, FF), BF16),
            pltpu.VMEM((D, FF), BF16),
            pltpu.VMEM((FF, D), BF16),
            pltpu.VMEM((D, 6 * D), BF16),
            pltpu.SemaphoreType.DMA((NB,)),
            pltpu.SemaphoreType.DMA((NB,)),
            pltpu.SemaphoreType.DMA((NB,)),
            pltpu.SemaphoreType.DMA((NB,)),
            pltpu.SemaphoreType.DMA((NLT,)),
            pltpu.SemaphoreType.DMA((6,)),
            pltpu.SemaphoreType.DMA((WCH,)),
            pltpu.SemaphoreType.DMA((WCH,)),
            pltpu.SemaphoreType.DMA((1,)),
            pltpu.VMEM((8, 4096), F32),
            pltpu.VMEM((2 * CH, D), F32),
            pltpu.VMEM((2, 2 * CH, D), F32),
            pltpu.VMEM((S // 2, D), U32),
            pltpu.VMEM((S, D), F32),
            pltpu.VMEM((TM // 2, FF), U32),
            pltpu.VMEM((1, TM, D), F32),
        ] + [pltpu.VMEM((UPAD + NCH + 2, UROWS, 128), F32) for _ in range(NLT)]
          + [pltpu.VMEM((NCH, KROWS, 128), F32) for _ in range(NLT)],
        compiler_params=pltpu.CompilerParams(
            dimension_semantics=("arbitrary",),
            vmem_limit_bytes=100 * 1024 * 1024),
    )(q, k, v, sk, A_ssm_k, dd, B_W_gate, B_W_up, B_W_down, c, w_mod, fwd, inv)
    return out.reshape(1, S, D)
```

```python
import os
import numpy as np
import jax
import jax.numpy as jnp
from jax import lax
import jax.experimental.pallas as pl
import jax.experimental.pallas.tpu as pltpu

S = 2048
D = 640
FF = 1536
CH = 128
NCH = S // CH
TM = 256
NB = S // TM
NLT = D // 128
NP = CH // 8
EPS = 1e-5
NJA = 12
UPAD = NJA - 8
KROWS = 3 * CH + 8
UROWS = 3 * CH + 64
WCH = 4
F32 = jnp.float32
BF16 = jnp.bfloat16
U32 = jnp.uint32
VARS = os.environ.get('VARS', 'P1ABT')
LNCH = int(os.environ.get('LNCH', 2))
LNGU = int(os.environ.get('LNGU', 10))


def _dft_tables():
    f = np.concatenate([np.arange(0, CH, 2), np.arange(1, CH, 2)])
    n = np.arange(CH)
    k = ((2 * f[:, None] + 1) * n[None, :]) % (4 * CH)
    ang = np.pi * k / (2 * CH)
    co = np.cos(ang).reshape(NP, 8, CH)
    si = np.sin(ang).reshape(NP, 8, CH)
    fwd = np.stack([co, si], axis=1).reshape(2 * CH, CH)
    inv = fwd.T / CH
    return fwd.astype(np.float32), inv.astype(np.float32)


def _pack_np(a):
    u = np.ascontiguousarray(a, np.float32).view(np.uint32)
    b = ((u + 0x7FFF + ((u >> 16) & 1)) >> 16).astype(np.uint32)
    return b[0::2] | (b[1::2] << 16)


def _pack(x):
    return pltpu.bitcast(x.astype(BF16), U32)


def _unpack(x):
    return pltpu.bitcast(x, BF16)


def _kernel(q_hbm, k_hbm, v_hbm, sk_ref, ssmk_hbm, dd_ref, wg_hbm, wu_hbm, wd_hbm,
            c_ref, wmod_hbm, f_ref, g_ref, o_hbm,
            q_ref, k_ref, v_ref, o_ref, ssmk_ref, wg_ref, wu_ref, wd_ref, wmod_ref,
            sems,
            mod_ref, zprev_ref, z_ref, h2_ref, x1_ref, act_ref, y_ref,
            wgp_ref, wup_ref, wdp_ref, kh_ref, *uh):
    g = pl.program_id(0)
    sem_q, sem_k, sem_v, sem_o, sem_s, sem_m, sem_g, sem_u, sem_d = [8 * i for i in range(9)]
    thr = g - 1000
    never8 = lax.broadcasted_iota(jnp.int32, (8, 128), 0) < thr
    never_col = lax.broadcasted_iota(jnp.int32, (16, 1), 0) < thr
    z1 = lax.shift_right_logical(g, 10)
    z2 = lax.shift_right_logical(g, 11)
    chain = {}

    def link(name, m, mask=never8):
        prev = chain.get(name)
        return m if prev is None else jnp.where(mask, prev, m)

    def lanes(lt):
        return slice(lt * 128, (lt + 1) * 128)

    def rows(b, off, n, unit=TM):
        if isinstance(b, int):
            return slice(b * unit + off, b * unit + off + n)
        return pl.ds(pl.multiple_of(b * unit, unit) + off, n)

    def rows_copy(src, dst, sem, b):
        return pltpu.make_async_copy(src.at[rows(b, 0, TM)], dst.at[rows(b, 0, TM)], sems.at[sem + b])

    def cols_copy(src, dst, sem, i, w):
        return pltpu.make_async_copy(src.at[:, pl.ds(i * w, w)], dst.at[:, pl.ds(i * w, w)], sems.at[sem + i])

    cp_q = lambda b: rows_copy(q_hbm, q_ref, sem_q, b)
    cp_k = lambda b: rows_copy(k_hbm, k_ref, sem_k, b)
    cp_v = lambda b: rows_copy(v_hbm, v_ref, sem_v, b)
    cp_o = lambda b: rows_copy(o_ref, o_hbm, sem_o, b)
    cp_s = lambda lt: pltpu.make_async_copy(
        ssmk_hbm.at[rows(lt, 0, 128, 128)], ssmk_ref.at[rows(lt, 0, 128, 128)], sems.at[sem_s + lt])
    cp_m = lambda i: cols_copy(wmod_hbm, wmod_ref, sem_m, i, D)
    cp_g = lambda i: cols_copy(wg_hbm, wg_ref, sem_g, i, FF // WCH)
    cp_u = lambda i: cols_copy(wu_hbm, wu_ref, sem_u, i, FF // WCH)
    cp_d = lambda i: cols_copy(wd_hbm, wd_ref, sem_d, i, 128)

    def dft_k(lt, j):
        kf = lax.dot_general(_unpack(f_ref[...]), ssmk_ref[rows(lt, 0, 128, 128), j * CH:(j + 1) * CH],
                             (((1,), (1,)), ((), ())), preferred_element_type=F32)
        for p in range(NP):
            kr = kf[16 * p:16 * p + 8]
            ki = kf[16 * p + 8:16 * p + 16]
            if j == 0:
                kr = kr + dd_ref[lt].astype(F32)
            kh_ref[lt * NCH + j, 24 * p:24 * p + 8, :] = kr
            kh_ref[lt * NCH + j, 24 * p + 8:24 * p + 16, :] = ki - kr
            kh_ref[lt * NCH + j, 24 * p + 16:24 * p + 24, :] = kr + ki

    def dft_u(b, bsrc, lt):
        cs = lanes(lt)
        sk = sk_ref[:, cs].astype(F32)
        k = k_ref[rows(bsrc, 0, TM), cs].astype(F32)
        if isinstance(b, int) and b == 0:
            halo = jnp.zeros((8, 128), F32)
        else:
            halo = k_ref[rows(bsrc, -16, 16), cs].astype(F32)[8:]
        kext = jnp.concatenate([halo, k], axis=0)
        ks = k * sk[0:1, :]
        for t in range(1, 4):
            ks = ks + kext[8 - t:8 - t + TM, :] * sk[t:t + 1, :]
        kv = ks * v_ref[rows(bsrc, 0, TM), cs].astype(F32)
        for cc in range(2):
            uf = jnp.dot(_unpack(f_ref[...]), kv[cc * CH:(cc + 1) * CH, :].astype(BF16),
                         preferred_element_type=F32)
            for p in range(NP):
                ur = uf[16 * p:16 * p + 8]
                ui = uf[16 * p + 8:16 * p + 16]
                uh[lt][UPAD + 2 * b + cc, 24 * p:24 * p + 8, :] = ur + ui
                uh[lt][UPAD + 2 * b + cc, 24 * p + 8:24 * p + 16, :] = ur
                uh[lt][UPAD + 2 * b + cc, 24 * p + 16:24 * p + 24, :] = ui

    def mac(b, njs, lt, paced):
        cs = lanes(lt)
        uw = uh[lt].at[pl.ds(UPAD + 2 * b + 2 - njs, njs)]
        first = isinstance(b, int) and b == 0
        for p in range(NP):
            a = [None] * 3
            c = [None] * 3
            for q in range(3):
                rr = pl.ds(24 * p + 8 * q, 8)
                kprev = None
                for t in range(njs):
                    u = uw[njs - 1 - t, rr, :]
                    k = kh_ref[lt * NCH + t, rr, :]
                    m = k * u
                    c[q] = link('c', m) if c[q] is None else c[q] + m
                    if t > 0:
                        m = kprev * u
                        a[q] = link('a', m) if a[q] is None else a[q] + m
                    kprev = k
                if paced:
                    chain['a'] = a[q]
                    chain['c'] = c[q]
            ar, ai = a[0] - a[2], a[0] + a[1]
            br, bi = c[0] - c[2], c[0] + c[1]
            if first:
                za = [ar, ai]
            else:
                pr = zprev_ref[16 * p:16 * p + 8, cs]
                pi = zprev_ref[16 * p + 8:16 * p + 16, cs]
                za = [ar + pi, ai - pr] if p < NP // 2 else [ar - pi, ai + pr]
            zprev_ref[16 * p:16 * p + 8, cs] = br
            zprev_ref[16 * p + 8:16 * p + 16, cs] = bi
            zb = [br + ai, bi - ar] if p < NP // 2 else [br - ai, bi + ar]
            z_ref[0, 16 * p:16 * p + 8, cs] = za[0]
            z_ref[0, 16 * p + 8:16 * p + 16, cs] = za[1]
            z_ref[1, 16 * p:16 * p + 8, cs] = zb[0]
            z_ref[1, 16 * p + 8:16 * p + 16, cs] = zb[1]

    def inv(lt):
        cs = lanes(lt)
        for cc in range(2):
            y_ref[z1, cc * CH:(cc + 1) * CH, cs] = jnp.dot(
                _unpack(g_ref[...]), z_ref[cc, :, cs].astype(BF16), preferred_element_type=F32)

    def norm(x, name=None):
        m = jnp.sum(x, axis=-1, keepdims=True) * (1.0 / D)
        if name is not None:
            m = link(name, m, never_col)
        xc = x - m
        v = jnp.sum(xc * xc, axis=-1, keepdims=True) * (1.0 / D)
        return xc * lax.rsqrt(v + EPS)

    def modrow(i):
        return mod_ref[0:1, i * D:(i + 1) * D]

    RC = 16

    def ln_piece(b, r, paced, bdst=None, part=3):
        bdst = b if bdst is None else bdst
        name = 'ln%d' % (r % LNCH)
        if part & 1:
            x = q_ref[rows(b, r * RC, RC), :].astype(F32)
            h1 = norm(x, name if paced else None) * modrow(1) + modrow(0)
            x1 = x + h1 * y_ref[z2, r * RC:(r + 1) * RC, :]
            x1_ref[rows(bdst, r * RC, RC), :] = x1
            n2 = norm(x1)
            if part == 1:
                y_ref[z2, r * RC:(r + 1) * RC, :] = n2
        else:
            n2 = y_ref[z2, r * RC:(r + 1) * RC, :]
        if part & 2:
            h2 = n2 * modrow(4) + modrow(3)
            if paced:
                chain[name] = h2[:, 0:1]
            h2_ref[rows(bdst, r * 8, 8, TM // 2), :] = _pack(h2)

    def ln_all(b, paced, bdst=None, part=3):
        for r in range(TM // RC):
            ln_piece(b, r, paced, bdst, part)

    def weight(raw_ref, packed_ref, cs, first):
        if not first:
            return _unpack(packed_ref[:, cs])
        w = raw_ref[:, cs]
        packed_ref[:, cs] = pltpu.bitcast(w, U32)
        return w

    def gu(b, c, first=False):
        cs = lanes(c)
        h2 = _unpack(h2_ref[rows(b, 0, TM // 2, TM // 2), :])
        gate = jnp.dot(h2, weight(wg_ref, wgp_ref, cs, first), preferred_element_type=F32)
        up = jnp.dot(h2, weight(wu_ref, wup_ref, cs, first), preferred_element_type=F32)
        act_ref[:, cs] = _pack(jnp.maximum(gate, 0.0) * up)
        if c == LNGU and not first:
            for i in range(LNCH):
                chain['ln%d' % i] = up[0:16, 0:1]

    def down(b, c, first=False):
        cs = lanes(c)
        gb = mod_ref[0:1, 5 * D + c * 128:5 * D + (c + 1) * 128]
        ff = jnp.dot(_unpack(act_ref[...]), weight(wd_ref, wdp_ref, cs, first),
                     preferred_element_type=F32)
        o_ref[rows(b, 0, TM), cs] = (x1_ref[rows(b, 0, TM), cs] + gb * ff).astype(BF16)

    def mod_part(i):
        c = c_ref[...].astype(F32)
        sc = jnp.broadcast_to((c * jax.nn.sigmoid(c)).astype(BF16), (8, D))
        return jnp.dot(sc, wmod_ref[:, i * D:(i + 1) * D], preferred_element_type=F32)

    def prologue():
        chain.clear()
        for lt in range(NLT):
            cp_s(lt).start()
        for b in range(2):
            cp_k(b).start()
            cp_v(b).start()
        cp_q(0).start()
        for i in range(3):
            cp_m(i).start()
        cp_k(2).start()
        cp_v(2).start()
        for i in (3, 4):
            cp_m(i).start()
        cp_q(1).start()
        for i in range(WCH):
            cp_g(i).start()
            cp_u(i).start()
        cp_m(5).start()
        for i in range(3):
            cp_d(i).start()
        cp_k(3).start()
        cp_v(3).start()
        for i in range(3, NLT):
            cp_d(i).start()
        for lt in range(NLT):
            uh[lt][0:UPAD, 0:3 * CH, :] = jnp.zeros((UPAD, 3 * CH, 128), F32)

        def kbody(lt, carry):
            cp_s(lt).wait()
            for j in range(NCH):
                dft_k(lt, j)
            return carry
        lax.fori_loop(0, NLT, kbody, 0)
        cp_k(0).wait()
        cp_v(0).wait()
        for lt in range(NLT):
            dft_u(0, 0, lt)
        cp_k(1).wait()
        cp_v(1).wait()
        for lt in range(NLT):
            dft_u(1, 1, lt)
            mac(0, 2, lt, False)
            inv(lt)
            mac(1, 4, lt, False)
        cp_q(0).wait()
        for i in range(3):
            cp_m(i).wait()
        ga = mod_part(2)
        mod_ref[:, 0:D] = mod_part(0) * ga
        mod_ref[:, D:2 * D] = (1.0 + mod_part(1)) * ga
        ln_all(0, False, part=1)
        cp_k(2).wait()
        cp_v(2).wait()
        for lt in range(NLT):
            dft_u(2, 2, lt)
        cp_m(3).wait()
        cp_m(4).wait()
        mod_ref[:, 3 * D:4 * D] = mod_part(3)
        mod_ref[:, 4 * D:5 * D] = 1.0 + mod_part(4)
        ln_all(0, False, part=2)
        for lt in range(NLT):
            inv(lt)

    def first_step():
        chain.clear()
        per = FF // 128 // WCH
        for i in range(WCH):
            if i == 0:
                cp_q(1).wait()
            cp_g(i).wait()
            cp_u(i).wait()
            chain.clear()
            for lt in {0: (0, 1), 1: (2,), 2: (3,), 3: (4,)}[i]:
                mac(2, 6, lt, True)
            for r in range(4 * i, 4 * i + 4):
                ln_piece(1, r, True)
            for c in range(i * per, (i + 1) * per):
                gu(0, c, True)
        cp_m(5).wait()
        for c in range(3):
            cp_d(c).wait()
        mod_ref[:, 5 * D:6 * D] = mod_part(5)
        for c in range(3):
            down(0, c, True)
        cp_k(3).wait()
        cp_v(3).wait()
        for c in range(3, NLT):
            cp_d(c).wait()
        down(0, 3, True)
        for lt in range(3):
            dft_u(3, 3, lt)
        down(0, 4, True)
        for lt in range(3, NLT):
            dft_u(3, 3, lt)

    def step(njs):
        bf, bl, bm, bd = g - 1, jnp.minimum(g, NB - 1), g + 1, g + 2
        chain.clear()
        for lt in range(NLT):
            inv(lt)
        if njs:
            for lt in range(NLT):
                mac(bm, njs, lt, True)
        for c in range(FF // 128):
            gu(bf, c)
        for c in range(NLT):
            if njs:
                dft_u(bd, jnp.minimum(bd, NB - 1), c)
            down(bf, c)
        ln_all(bl, True, g)

    def variant(tag, cond, fn):
        def body():
            with jax.named_scope('var' + tag):
                if tag in VARS:
                    fn()
        pl.when(cond)(body)

    variant('P', g == 0, prologue)

    @pl.when(jnp.logical_and(g >= 2, g + 2 < NB))
    def _():
        cp_k(g + 2).wait()
        cp_v(g + 2).wait()

    @pl.when(jnp.logical_and(g >= 1, g + 3 < NB))
    def _():
        cp_k(g + 3).start()
        cp_v(g + 3).start()

    @pl.when(jnp.logical_and(g >= 2, g < NB))
    def _():
        cp_q(g).wait()

    @pl.when(jnp.logical_and(g >= 1, g + 1 < NB))
    def _():
        cp_q(g + 1).start()

    @pl.when(g >= 2)
    def _():
        cp_o(g - 2).start()

    variant('1', g == 1, first_step)
    variant('A', jnp.logical_and(g >= 2, g <= 4), lambda: step(NJA))
    variant('B', jnp.logical_and(g >= 5, g <= 6), lambda: step(NCH))
    variant('T', g >= 7, lambda: step(0))

    @pl.when(g == NB)
    def _():
        cp_o(NB - 1).start()
        for b in range(NB):
            cp_o(b).wait()


@jax.jit
def pallas_adaLN_cond__ssm_conv_h3__glu_gated_reglu__prompt_kernel(
    A_q, A_k, A_v, A_shift_k, A_ssm_k, A_ssm_D, B_x, B_W_gate, B_W_up, B_W_down, c, w_mod,
):
    del B_x
    fwd, inv = _dft_tables()
    fwd = jnp.asarray(_pack_np(fwd))
    inv = jnp.asarray(_pack_np(inv))
    q = A_q.reshape(S, D)
    k = A_k.reshape(S, D)
    v = A_v.reshape(S, D)
    sk = A_shift_k.T
    dd = A_ssm_D.reshape(NLT, 1, 128)

    hbm = pl.BlockSpec(memory_space=pl.ANY)

    def full(shape):
        return pl.BlockSpec(shape, lambda s: (0, 0))

    out = pl.pallas_call(
        _kernel,
        grid=(NB + 1,),
        in_specs=[hbm, hbm, hbm, full((4, D)), hbm, pl.BlockSpec((NLT, 1, 128), lambda s: (0, 0, 0)), hbm, hbm, hbm,
                  full((1, D)), hbm, full((CH, CH)), full((CH // 2, 2 * CH))],
        out_specs=hbm,
        out_shape=jax.ShapeDtypeStruct((S, D), BF16),
        scratch_shapes=[
            pltpu.VMEM((S, D), BF16),
            pltpu.VMEM((S, D), BF16),
            pltpu.VMEM((S, D), BF16),
            pltpu.VMEM((S, D), BF16),
            pltpu.VMEM((D, S), BF16),
            pltpu.VMEM((D, FF), BF16),
            pltpu.VMEM((D, FF), BF16),
            pltpu.VMEM((FF, D), BF16),
            pltpu.VMEM((D, 6 * D), BF16),
            pltpu.SemaphoreType.DMA((72,)),
            pltpu.VMEM((8, 4096), F32),
            pltpu.VMEM((2 * CH, D), F32),
            pltpu.VMEM((2, 2 * CH, D), F32),
            pltpu.VMEM(((S + TM) // 2, D), U32),
            pltpu.VMEM((S + TM, D), F32),
            pltpu.VMEM((TM // 2, FF), U32),
            pltpu.VMEM((1, TM, D), F32),
            pltpu.VMEM((D // 2, FF), U32),
            pltpu.VMEM((D // 2, FF), U32),
            pltpu.VMEM((FF // 2, D), U32),
            pltpu.VMEM((NLT * NCH, KROWS, 128), F32),
        ] + [pltpu.VMEM((UPAD + NCH + 2, UROWS, 128), F32) for _ in range(NLT)],
        compiler_params=pltpu.CompilerParams(
            dimension_semantics=("arbitrary",),
            vmem_limit_bytes=100 * 1024 * 1024),
    )(q, k, v, sk, A_ssm_k, dd, B_W_gate, B_W_up, B_W_down, c, w_mod, fwd, inv)
    return out.reshape(1, S, D)
```

```python
import os
import numpy as np
import jax
import jax.numpy as jnp
from jax import lax
import jax.experimental.pallas as pl
import jax.experimental.pallas.tpu as pltpu

S = 2048
D = 640
FF = 1536
CH = 128
NCH = S // CH
TM = 256
NB = S // TM
NLT = D // 128
NP = CH // 8
EPS = 1e-5
UPAD = NCH - 8
KROWS = 3 * CH + 8
UROWS = 3 * CH + 64
WCH = 4
RC = 16
F32 = jnp.float32
BF16 = jnp.bfloat16
U32 = jnp.uint32
VARS = os.environ.get('VARS', 'P1BCTU')
LNCH = int(os.environ.get('LNCH', 2))
LNGU = int(os.environ.get('LNGU', 10))
LNGUT = int(os.environ.get('LNGUT', 6))
USEC = int(os.environ.get('USEC', 0))
MACDELAY = int(os.environ.get('MACDELAY', -1))


def _dft_tables():
    f = np.concatenate([np.arange(0, CH, 2), np.arange(1, CH, 2)])
    n = np.arange(CH)
    k = ((2 * f[:, None] + 1) * n[None, :]) % (4 * CH)
    ang = np.pi * k / (2 * CH)
    co = np.cos(ang).reshape(NP, 8, CH)
    si = np.sin(ang).reshape(NP, 8, CH)
    fwd = np.stack([co, si], axis=1).reshape(2 * CH, CH)
    inv = fwd.T / CH
    return fwd.astype(np.float32), inv.astype(np.float32)


def _pack_np(a):
    u = np.ascontiguousarray(a, np.float32).view(np.uint32)
    b = ((u + 0x7FFF + ((u >> 16) & 1)) >> 16).astype(np.uint32)
    return b[0::2] | (b[1::2] << 16)


def _pack(x):
    return pltpu.bitcast(x.astype(BF16), U32)


def _unpack(x):
    return pltpu.bitcast(x, BF16)


def _kernel(q_hbm, k_hbm, v_hbm, sk_hbm, ssmk_hbm, dd_hbm, wg_hbm, wu_hbm, wd_hbm,
            c_hbm, wmod_hbm, f_hbm, g_hbm, o_hbm,
            q_ref, k_ref, v_ref, o_ref, ssmk_ref, wg_ref, wu_ref, wd_ref, wmod_ref, sems,
            mod_ref, zprev_ref, z_ref, h2_ref, x1_ref, act_ref, y_ref,
            wgp_ref, wup_ref, wdp_ref, kh_ref, u0, u1, u2, u3, u4,
            f_ref, g_ref, ddf_ref, sk_ref, dd_ref, c_ref):
    uh = (u0, u1, u2, u3, u4)
    g = pl.program_id(0)
    sem_q, sem_k, sem_v, sem_o, sem_s, sem_m, sem_g, sem_u, sem_d, sem_l, sem_x = (
        0, 8, 16, 24, 32, 37, 43, 47, 51, 56, 61)
    thr = g - 1000
    never8 = lax.broadcasted_iota(jnp.int32, (8, 128), 0) < thr
    never_col = lax.broadcasted_iota(jnp.int32, (16, 1), 0) < thr
    z1 = lax.shift_right_logical(g, 10)
    z2 = lax.shift_right_logical(g, 11)
    chain = {}

    def link(name, m, mask=never8):
        prev = chain.get(name)
        return m if prev is None else jnp.where(mask, prev, m)

    def lanes(lt):
        return slice(lt * 128, (lt + 1) * 128)

    def blk_copy(src, dst, sem, b):
        return pltpu.make_async_copy(src.at[b], dst.at[b], sems.at[sem + b])

    def cols_copy(src, dst, sem, i, w):
        return pltpu.make_async_copy(src.at[:, pl.ds(i * w, w)], dst.at[:, pl.ds(i * w, w)],
                                     sems.at[sem + i])

    cp_q = lambda b: blk_copy(q_hbm, q_ref, sem_q, b)
    cp_k = lambda b: blk_copy(k_hbm, k_ref, sem_k, b)
    cp_v = lambda b: blk_copy(v_hbm, v_ref, sem_v, b)
    cp_o = lambda b: blk_copy(o_ref, o_hbm, sem_o, b)
    cp_s = lambda lt: blk_copy(ssmk_hbm, ssmk_ref, sem_s, lt)
    cp_m = lambda i: cols_copy(wmod_hbm, wmod_ref, sem_m, i, D)
    cp_g = lambda i: cols_copy(wg_hbm, wg_ref, sem_g, i, FF // WCH)
    cp_u = lambda i: cols_copy(wu_hbm, wu_ref, sem_u, i, FF // WCH)
    cp_d = lambda i: cols_copy(wd_hbm, wd_ref, sem_d, i, 128)
    cp_l = lambda i: cols_copy(o_ref.at[NB - 1], o_hbm.at[NB - 1], sem_l, i, 128)

    cp_x = lambda i: pltpu.make_async_copy(
        (f_hbm, dd_hbm, sk_hbm, g_hbm, c_hbm)[i], (f_ref, dd_ref, sk_ref, g_ref, c_ref)[i],
        sems.at[sem_x + i])

    def dft_k(lt, j):
        kf = lax.dot_general(_unpack(f_ref[...]), ssmk_ref[lt, :, j * CH:(j + 1) * CH],
                             (((1,), (1,)), ((), ())), preferred_element_type=F32)
        for p in range(NP):
            kr = kf[16 * p:16 * p + 8]
            ki = kf[16 * p + 8:16 * p + 16]
            if j == 0:
                kr = kr + ddf_ref[lt]
            kh_ref[lt * NCH + j, 24 * p:24 * p + 8, :] = kr
            kh_ref[lt * NCH + j, 24 * p + 8:24 * p + 16, :] = ki - kr
            kh_ref[lt * NCH + j, 24 * p + 16:24 * p + 24, :] = kr + ki

    def dft_u(b, bsrc, lt):
        cs = lanes(lt)
        sk = sk_ref[:, cs].astype(F32)
        k = k_ref[bsrc, :, cs].astype(F32)
        if isinstance(b, int) and b == 0:
            halo = jnp.zeros((8, 128), F32)
        else:
            halo = k_ref[bsrc - 1, TM - 8:TM, cs].astype(F32)
        kext = jnp.concatenate([halo, k], axis=0)
        ks = k * sk[0:1, :]
        for t in range(1, 4):
            ks = ks + kext[8 - t:8 - t + TM, :] * sk[t:t + 1, :]
        kv = ks * v_ref[bsrc, :, cs].astype(F32)
        for cc in range(2):
            uf = jnp.dot(_unpack(f_ref[...]), kv[cc * CH:(cc + 1) * CH, :].astype(BF16),
                         preferred_element_type=F32)
            for p in range(NP):
                ur = uf[16 * p:16 * p + 8]
                ui = uf[16 * p + 8:16 * p + 16]
                uh[lt][UPAD + 2 * b + cc, 24 * p:24 * p + 8, :] = ur + ui
                uh[lt][UPAD + 2 * b + cc, 24 * p + 8:24 * p + 16, :] = ur
                uh[lt][UPAD + 2 * b + cc, 24 * p + 16:24 * p + 24, :] = ui

    def mac(b, njs, lt, paced):
        cs = lanes(lt)
        uw = uh[lt].at[pl.ds(UPAD + 2 * b + 2 - njs, njs)]
        for p in range(NP):
            base = {}
            for q in range(3):
                rr = pl.ds(24 * p + 8 * q, 8)
                acc = {}
                for o in 'ac':
                    if q == 1:
                        acc[o] = base[o]
                    elif q == 2:
                        acc[o] = link(o, base[o])
                kprev = None
                for t in range(njs):
                    u = uw[njs - 1 - t, rr, :]
                    k = kh_ref[lt * NCH + t, rr, :]
                    for o, kk in (('c', k), ('a', kprev)):
                        if kk is None:
                            continue
                        m = kk * u
                        if o not in acc:
                            acc[o] = link(o, m)
                        else:
                            acc[o] = acc[o] - m if q == 2 else acc[o] + m
                    kprev = k
                if q == 0:
                    base = acc
                else:
                    r0 = 16 * p + (8 if q == 1 else 0)
                    z_ref[0, r0:r0 + 8, cs] = acc['a']
                    z_ref[1, r0:r0 + 8, cs] = acc['c']
                    if paced:
                        chain.update(acc)

    def inv(lt, first=False):
        cs = lanes(lt)
        za, zb = [], []
        for p in range(NP):
            re, im = slice(16 * p, 16 * p + 8), slice(16 * p + 8, 16 * p + 16)
            ar, ai, br, bi = z_ref[0, re, cs], z_ref[0, im, cs], z_ref[1, re, cs], z_ref[1, im, cs]
            if first:
                za += [ar, ai]
            else:
                pr, pi = zprev_ref[re, cs], zprev_ref[im, cs]
                za += [ar + pi, ai - pr] if p < NP // 2 else [ar - pi, ai + pr]
            zb += [br + ai, bi - ar] if p < NP // 2 else [br - ai, bi + ar]
            zprev_ref[re, cs] = br
            zprev_ref[im, cs] = bi
        for cc, z in enumerate((za, zb)):
            y = jnp.dot(_unpack(g_ref[...]), jnp.concatenate(z, axis=0).astype(BF16),
                        preferred_element_type=F32)
            y_ref[z1, cc * CH:(cc + 1) * CH, cs] = y
        return y[0:8]

    def norm(x, name=None):
        m = jnp.sum(x, axis=-1, keepdims=True) * (1.0 / D)
        if name is not None:
            m = link(name, m, never_col)
        xc = x - m
        v = jnp.sum(xc * xc, axis=-1, keepdims=True) * (1.0 / D)
        return xc * lax.rsqrt(v + EPS)

    def modrow(i):
        return mod_ref[0:1, i * D:(i + 1) * D]

    act = {}

    def set_blocks(bf, bl):
        if isinstance(bf, int) or isinstance(bl, int):
            act.update(xf=x1_ref.at[bf], hf=h2_ref.at[bf], xl=x1_ref.at[bl], hl=h2_ref.at[bl])
        else:
            n = 1 if bl is None else 2
            xw, hw = x1_ref.at[pl.ds(bf, n)], h2_ref.at[pl.ds(bf, n)]
            act.update(xf=xw.at[0], hf=hw.at[0], xl=xw.at[n - 1], hl=hw.at[n - 1])

    def ln_piece(b, r, paced, part=3):
        name = 'ln%d' % (r % LNCH)
        rs = slice(r * RC, (r + 1) * RC)
        if part & 1:
            x = q_ref[b, rs, :].astype(F32)
            h1 = norm(x, name if paced else None) * modrow(1) + modrow(0)
            x1 = x + h1 * y_ref[z2, rs, :]
            act['xl'][rs, :] = x1
            n2 = norm(x1)
            if part == 1:
                y_ref[z2, rs, :] = n2
        else:
            n2 = y_ref[z2, rs, :]
        if part & 2:
            h2 = n2 * modrow(4) + modrow(3)
            if paced:
                chain[name] = h2[:, 0:1]
            act['hl'][r * 8:(r + 1) * 8, :] = _pack(h2)

    def ln_all(b, paced, part=3):
        for r in range(TM // RC):
            ln_piece(b, r, paced, part)

    def weight(raw_ref, packed_ref, cs, first):
        if not first:
            return _unpack(packed_ref[:, cs])
        w = raw_ref[:, cs]
        packed_ref[:, cs] = pltpu.bitcast(w, U32)
        return w

    def gu(b, c, first=False, lngu=-1):
        cs = lanes(c)
        h2 = _unpack(act['hf'][...])
        gate = jnp.dot(h2, weight(wg_ref, wgp_ref, cs, first), preferred_element_type=F32)
        up = jnp.dot(h2, weight(wu_ref, wup_ref, cs, first), preferred_element_type=F32)
        act_ref[:, cs] = _pack(jnp.maximum(gate, 0.0) * up)
        if c == lngu:
            for i in range(LNCH):
                chain['ln%d' % i] = up[0:16, 0:1]

    def down(b, c, first=False):
        cs = lanes(c)
        gb = mod_ref[0:1, 5 * D + c * 128:5 * D + (c + 1) * 128]
        ff = jnp.dot(_unpack(act_ref[...]), weight(wd_ref, wdp_ref, cs, first),
                     preferred_element_type=F32)
        o_ref[b, :, cs] = (act['xf'][:, cs] + gb * ff).astype(BF16)

    def mod_part(i):
        c = c_ref[...].astype(F32)
        sc = jnp.broadcast_to((c * jax.nn.sigmoid(c)).astype(BF16), (8, D))
        return jnp.dot(sc, wmod_ref[:, i * D:(i + 1) * D], preferred_element_type=F32)

    def prologue():
        chain.clear()
        set_blocks(0, 0)
        cp_x(0).start()
        cp_s(0).start()
        for i in range(1, 5):
            cp_x(i).start()
        for lt in range(1, NLT):
            cp_s(lt).start()
        for b in range(2):
            cp_k(b).start()
            cp_v(b).start()
        cp_q(0).start()
        for i in range(3):
            cp_m(i).start()
        cp_k(2).start()
        cp_v(2).start()
        for i in (3, 4):
            cp_m(i).start()
        cp_q(1).start()
        for i in range(WCH):
            cp_g(i).start()
            cp_u(i).start()
        cp_m(5).start()
        for i in range(3):
            cp_d(i).start()
        cp_k(3).start()
        cp_v(3).start()
        for i in range(3, NLT):
            cp_d(i).start()
        for lt in range(NLT):
            uh[lt][0:UPAD, 0:3 * CH, :] = jnp.zeros((UPAD, 3 * CH, 128), F32)
        for i in range(5):
            cp_x(i).wait()
        dd = dd_ref[...].astype(F32)
        for lt in range(NLT):
            ddf_ref[lt] = jnp.broadcast_to(dd[lt:lt + 1, :], (8, 128))

        def kbody(lt, carry):
            cp_s(lt).wait()
            for j in range(NCH):
                dft_k(lt, j)
            return carry
        lax.fori_loop(0, NLT, kbody, 0)
        cp_k(0).wait()
        cp_v(0).wait()
        for lt in range(NLT):
            dft_u(0, 0, lt)
        cp_k(1).wait()
        cp_v(1).wait()
        for lt in range(NLT):
            dft_u(1, 1, lt)
            mac(0, 2, lt, False)
            inv(lt, True)
            mac(1, 4, lt, False)
        cp_q(0).wait()
        for i in range(3):
            cp_m(i).wait()
        ga = mod_part(2)
        mod_ref[:, 0:D] = mod_part(0) * ga
        mod_ref[:, D:2 * D] = (1.0 + mod_part(1)) * ga
        ln_all(0, False, part=1)
        cp_k(2).wait()
        cp_v(2).wait()
        for lt in range(NLT):
            dft_u(2, 2, lt)
        cp_m(3).wait()
        cp_m(4).wait()
        mod_ref[:, 3 * D:4 * D] = mod_part(3)
        mod_ref[:, 4 * D:5 * D] = 1.0 + mod_part(4)
        ln_all(0, False, part=2)
        for lt in range(NLT):
            inv(lt)

    def first_step():
        per = FF // 128 // WCH
        set_blocks(0, 1)
        for i in range(WCH):
            if i == 0:
                cp_q(1).wait()
            cp_g(i).wait()
            cp_u(i).wait()
            chain.clear()
            for lt in {0: (0, 1), 1: (2,), 2: (3,), 3: (4,)}[i]:
                mac(2, 6, lt, True)
            for r in range(4 * i, 4 * i + 4):
                ln_piece(1, r, True)
            for c in range(i * per, (i + 1) * per):
                gu(0, c, True)
        cp_m(5).wait()
        for c in range(3):
            cp_d(c).wait()
        mod_ref[:, 5 * D:6 * D] = mod_part(5)
        for c in range(3):
            down(0, c, True)
        cp_k(3).wait()
        cp_v(3).wait()
        for c in range(3, NLT):
            cp_d(c).wait()
        down(0, 3, True)
        for lt in range(3):
            dft_u(3, 3, lt)
        down(0, 4, True)
        for lt in range(3, NLT):
            dft_u(3, 3, lt)

    def step(do_dft, do_mac, do_ln, last=False):
        chain.clear()
        set_blocks(g - 1, g if do_ln else None)
        if do_ln:
            for lt in range(NLT):
                t = inv(lt)
                if lt == MACDELAY:
                    chain.update(a=t, c=t)
        if do_mac:
            for lt in range(NLT):
                mac(g + 1, NCH, lt, True)
        for c in range(FF // 128):
            gu(g - 1, c, lngu=(LNGU if do_mac else LNGUT))
        for c in range(NLT):
            if do_dft:
                dft_u(g + 2, jnp.minimum(g + 2, NB - 1), c)
            down(g - 1, c)
            if last:
                cp_l(c).start()
        if do_ln:
            ln_all(g, True)

    def variant(tag, cond, fn):
        def body():
            with jax.named_scope('var' + tag):
                if tag in VARS:
                    fn()
        pl.when(cond)(body)

    variant('P', g == 0, prologue)

    @pl.when(jnp.logical_and(g >= 2, g + 2 < NB))
    def _():
        cp_k(g + 2).wait()
        cp_v(g + 2).wait()

    @pl.when(jnp.logical_and(g >= 1, g + 3 < NB))
    def _():
        cp_k(g + 3).start()
        cp_v(g + 3).start()

    @pl.when(jnp.logical_and(g >= 2, g < NB))
    def _():
        cp_q(g).wait()

    @pl.when(jnp.logical_and(g >= 1, g + 1 < NB))
    def _():
        cp_q(g + 1).start()

    @pl.when(g >= 2)
    def _():
        cp_o(g - 2).start()

    variant('1', g == 1, first_step)
    variant('B', jnp.logical_and(g >= 2, g <= 6 - USEC), lambda: step(True, True, True))
    if USEC:
        variant('C', g == 6, lambda: step(False, True, True))
    variant('T', g == 7, lambda: step(False, False, True))
    variant('U', g == 8, lambda: step(False, False, False, True))

    @pl.when(g == NB)
    def _():
        for b in range(NB - 1):
            cp_o(b).wait()
        if 'U' in VARS:
            for c in range(NLT):
                cp_l(c).wait()


@jax.jit
def pallas_adaLN_cond__ssm_conv_h3__glu_gated_reglu__prompt_kernel(
    A_q, A_k, A_v, A_shift_k, A_ssm_k, A_ssm_D, B_x, B_W_gate, B_W_up, B_W_down, c, w_mod,
):
    del B_x
    fwd, inv = _dft_tables()
    fwd = jnp.asarray(_pack_np(fwd))
    inv = jnp.asarray(_pack_np(inv))
    q = A_q.reshape(NB, TM, D)
    k = A_k.reshape(NB, TM, D)
    v = A_v.reshape(NB, TM, D)
    ssmk = A_ssm_k.reshape(NLT, 128, S)
    sk = A_shift_k.T
    dd = A_ssm_D.reshape(NLT, 128)

    hbm = pl.BlockSpec(memory_space=pl.ANY)

    out = pl.pallas_call(
        _kernel,
        grid=(NB + 1,),
        in_specs=[hbm] * 13,
        out_specs=hbm,
        out_shape=jax.ShapeDtypeStruct((NB, TM, D), BF16),
        scratch_shapes=[
            pltpu.VMEM((NB, TM, D), BF16),
            pltpu.VMEM((NB, TM, D), BF16),
            pltpu.VMEM((NB, TM, D), BF16),
            pltpu.VMEM((NB, TM, D), BF16),
            pltpu.VMEM((NLT, 128, S), BF16),
            pltpu.VMEM((D, FF), BF16),
            pltpu.VMEM((D, FF), BF16),
            pltpu.VMEM((FF, D), BF16),
            pltpu.VMEM((D, 6 * D), BF16),
            pltpu.SemaphoreType.DMA((66,)),
            pltpu.VMEM((8, 4096), F32),
            pltpu.VMEM((2 * CH, D), F32),
            pltpu.VMEM((2, 2 * CH, D), F32),
            pltpu.VMEM((NB, TM // 2, D), U32),
            pltpu.VMEM((NB, TM, D), F32),
            pltpu.VMEM((TM // 2, FF), U32),
            pltpu.VMEM((1, TM, D), F32),
            pltpu.VMEM((D // 2, FF), U32),
            pltpu.VMEM((D // 2, FF), U32),
            pltpu.VMEM((FF // 2, D), U32),
            pltpu.VMEM((NLT * NCH, KROWS, 128), F32),
        ] + [pltpu.VMEM((UPAD + NCH + 2, UROWS, 128), F32) for _ in range(NLT)] + [
            pltpu.VMEM((CH, CH), U32),
            pltpu.VMEM((CH // 2, 2 * CH), U32),
            pltpu.VMEM((8, 8, 128), F32),
            pltpu.VMEM((4, D), BF16),
            pltpu.VMEM((NLT, 128), BF16),
            pltpu.VMEM((1, D), BF16),
        ],
        compiler_params=pltpu.CompilerParams(
            dimension_semantics=("arbitrary",),
            vmem_limit_bytes=110 * 1024 * 1024,
            disable_bounds_checks=bool(int(os.environ.get('NOCHK', 1))),
            disable_semaphore_checks=bool(int(os.environ.get('NOCHK', 1)))),
    )(q, k, v, sk, ssmk, dd, B_W_gate, B_W_up, B_W_down, c, w_mod, fwd, inv)
    return out.reshape(1, S, D)
```

```python
import os
import numpy as np
import jax
import jax.numpy as jnp
from jax import lax
import jax.experimental.pallas as pl
import jax.experimental.pallas.tpu as pltpu

S = 2048
D = 640
FF = 1536
CH = 128
NCH = S // CH
TM = 256
NB = S // TM
NLT = D // 128
NP = CH // 8
EPS = 1e-5
UPAD = NCH - 8
KROWS = 3 * CH + 8
UROWS = 3 * CH + 64
WCH = 6
RC = 16
F32 = jnp.float32
BF16 = jnp.bfloat16
U32 = jnp.uint32
VARS = os.environ.get('VARS', 'P1BCTU')
LNCH = int(os.environ.get('LNCH', 2))
LNGU = int(os.environ.get('LNGU', 10))
LNGUT = int(os.environ.get('LNGUT', 6))
USEC = int(os.environ.get('USEC', 0))
MACDELAY = int(os.environ.get('MACDELAY', -1))


def _dft_tables():
    f = np.concatenate([np.arange(0, CH, 2), np.arange(1, CH, 2)])
    n = np.arange(CH)
    k = ((2 * f[:, None] + 1) * n[None, :]) % (4 * CH)
    ang = np.pi * k / (2 * CH)
    co = np.cos(ang).reshape(NP, 8, CH)
    si = np.sin(ang).reshape(NP, 8, CH)
    fwd = np.stack([co, si], axis=1).reshape(2 * CH, CH)
    inv = fwd.T / CH
    return fwd.astype(np.float32), inv.astype(np.float32)


def _pack_np(a):
    u = np.ascontiguousarray(a, np.float32).view(np.uint32)
    b = ((u + 0x7FFF + ((u >> 16) & 1)) >> 16).astype(np.uint32)
    return b[0::2] | (b[1::2] << 16)


def _pack(x):
    return pltpu.bitcast(x.astype(BF16), U32)


def _unpack(x):
    return pltpu.bitcast(x, BF16)


def _kernel(q_hbm, k_hbm, v_hbm, sk_hbm, ssmk_hbm, dd_hbm, wg_hbm, wu_hbm, wd_hbm,
            c_hbm, wmod_hbm, f_hbm, g_hbm, o_hbm,
            q_ref, k_ref, v_ref, o_ref, ssmk_ref, wg_ref, wu_ref, wd_ref, wmod_ref, sems,
            mod_ref, zprev_ref, z_ref, h2_ref, x1_ref, act_ref, y_ref,
            wgp_ref, wup_ref, wdp_ref, kh_ref, u0, u1, u2, u3, u4,
            f_ref, g_ref, ddf_ref, sk_ref, dd_ref, c_ref):
    uh = (u0, u1, u2, u3, u4)
    g = pl.program_id(0)
    sem_q, sem_k, sem_v, sem_o, sem_s, sem_m, sem_g, sem_u, sem_d, sem_l, sem_x = (
        0, 8, 16, 24, 32, 37, 43, 49, 55, 60, 65)
    thr = g - 1000
    never8 = lax.broadcasted_iota(jnp.int32, (8, 128), 0) < thr
    never_col = lax.broadcasted_iota(jnp.int32, (16, 1), 0) < thr
    z1 = lax.shift_right_logical(g, 10)
    z2 = lax.shift_right_logical(g, 11)
    chain = {}

    def link(name, m, mask=never8):
        prev = chain.get(name)
        return m if prev is None else jnp.where(mask, prev, m)

    def lanes(lt):
        return slice(lt * 128, (lt + 1) * 128)

    def blk_copy(src, dst, sem, b):
        return pltpu.make_async_copy(src.at[b], dst.at[b], sems.at[sem + b])

    def cols_copy(src, dst, sem, i, w):
        return pltpu.make_async_copy(src.at[:, pl.ds(i * w, w)], dst.at[:, pl.ds(i * w, w)],
                                     sems.at[sem + i])

    cp_q = lambda b: blk_copy(q_hbm, q_ref, sem_q, b)
    cp_k = lambda b: blk_copy(k_hbm, k_ref, sem_k, b)
    cp_v = lambda b: blk_copy(v_hbm, v_ref, sem_v, b)
    cp_o = lambda b: blk_copy(o_ref, o_hbm, sem_o, b)
    cp_s = lambda lt: blk_copy(ssmk_hbm, ssmk_ref, sem_s, lt)
    cp_m = lambda i: cols_copy(wmod_hbm, wmod_ref, sem_m, i, D)
    cp_g = lambda i: cols_copy(wg_hbm, wg_ref, sem_g, i, FF // WCH)
    cp_u = lambda i: cols_copy(wu_hbm, wu_ref, sem_u, i, FF // WCH)
    cp_d = lambda i: cols_copy(wd_hbm, wd_ref, sem_d, i, 128)
    cp_l = lambda i: cols_copy(o_ref.at[NB - 1], o_hbm.at[NB - 1], sem_l, i, 128)

    cp_x = lambda i: pltpu.make_async_copy(
        (f_hbm, dd_hbm, sk_hbm, g_hbm, c_hbm)[i], (f_ref, dd_ref, sk_ref, g_ref, c_ref)[i],
        sems.at[sem_x + i])

    def dft_k(lt, j):
        kf = lax.dot_general(_unpack(f_ref[...]), ssmk_ref[lt, :, j * CH:(j + 1) * CH],
                             (((1,), (1,)), ((), ())), preferred_element_type=F32)
        for p in range(NP):
            kr = kf[16 * p:16 * p + 8]
            ki = kf[16 * p + 8:16 * p + 16]
            if j == 0:
                kr = kr + ddf_ref[lt]
            kh_ref[lt * NCH + j, 24 * p:24 * p + 8, :] = kr
            kh_ref[lt * NCH + j, 24 * p + 8:24 * p + 16, :] = ki - kr
            kh_ref[lt * NCH + j, 24 * p + 16:24 * p + 24, :] = kr + ki

    def dft_u(b, bsrc, lt):
        cs = lanes(lt)
        sk = sk_ref[:, cs].astype(F32)
        k = k_ref[bsrc, :, cs].astype(F32)
        if isinstance(b, int) and b == 0:
            halo = jnp.zeros((8, 128), F32)
        else:
            halo = k_ref[bsrc - 1, TM - 8:TM, cs].astype(F32)
        kext = jnp.concatenate([halo, k], axis=0)
        ks = k * sk[0:1, :]
        for t in range(1, 4):
            ks = ks + kext[8 - t:8 - t + TM, :] * sk[t:t + 1, :]
        kv = ks * v_ref[bsrc, :, cs].astype(F32)
        for cc in range(2):
            uf = jnp.dot(_unpack(f_ref[...]), kv[cc * CH:(cc + 1) * CH, :].astype(BF16),
                         preferred_element_type=F32)
            for p in range(NP):
                ur = uf[16 * p:16 * p + 8]
                ui = uf[16 * p + 8:16 * p + 16]
                uh[lt][UPAD + 2 * b + cc, 24 * p:24 * p + 8, :] = ur + ui
                uh[lt][UPAD + 2 * b + cc, 24 * p + 8:24 * p + 16, :] = ur
                uh[lt][UPAD + 2 * b + cc, 24 * p + 16:24 * p + 24, :] = ui

    def mac(b, njs, lt, paced):
        cs = lanes(lt)
        uw = uh[lt].at[pl.ds(UPAD + 2 * b + 2 - njs, njs)]
        for p in range(NP):
            base = {}
            for q in range(3):
                rr = pl.ds(24 * p + 8 * q, 8)
                acc = {}
                for o in 'ac':
                    if q == 1:
                        acc[o] = base[o]
                    elif q == 2:
                        acc[o] = link(o, base[o])
                kprev = None
                for t in range(njs):
                    u = uw[njs - 1 - t, rr, :]
                    k = kh_ref[lt * NCH + t, rr, :]
                    for o, kk in (('c', k), ('a', kprev)):
                        if kk is None:
                            continue
                        m = kk * u
                        if o not in acc:
                            acc[o] = link(o, m)
                        else:
                            acc[o] = acc[o] - m if q == 2 else acc[o] + m
                    kprev = k
                if q == 0:
                    base = acc
                else:
                    r0 = 16 * p + (8 if q == 1 else 0)
                    z_ref[0, r0:r0 + 8, cs] = acc['a']
                    z_ref[1, r0:r0 + 8, cs] = acc['c']
                    if paced:
                        chain.update(acc)

    def inv(lt, first=False):
        cs = lanes(lt)
        za, zb = [], []
        for p in range(NP):
            re, im = slice(16 * p, 16 * p + 8), slice(16 * p + 8, 16 * p + 16)
            ar, ai, br, bi = z_ref[0, re, cs], z_ref[0, im, cs], z_ref[1, re, cs], z_ref[1, im, cs]
            if first:
                za += [ar, ai]
            else:
                pr, pi = zprev_ref[re, cs], zprev_ref[im, cs]
                za += [ar + pi, ai - pr] if p < NP // 2 else [ar - pi, ai + pr]
            zb += [br + ai, bi - ar] if p < NP // 2 else [br - ai, bi + ar]
            zprev_ref[re, cs] = br
            zprev_ref[im, cs] = bi
        for cc, z in enumerate((za, zb)):
            y = jnp.dot(_unpack(g_ref[...]), jnp.concatenate(z, axis=0).astype(BF16),
                        preferred_element_type=F32)
            y_ref[z1, cc * CH:(cc + 1) * CH, cs] = y
        return y[0:8]

    def norm(x, name=None):
        m = jnp.sum(x, axis=-1, keepdims=True) * (1.0 / D)
        if name is not None:
            m = link(name, m, never_col)
        xc = x - m
        v = jnp.sum(xc * xc, axis=-1, keepdims=True) * (1.0 / D)
        return xc * lax.rsqrt(v + EPS)

    def modrow(i):
        return mod_ref[0:1, i * D:(i + 1) * D]

    act = {}

    def set_blocks(bf, bl):
        if isinstance(bf, int) or isinstance(bl, int):
            act.update(xf=x1_ref.at[bf], hf=h2_ref.at[bf], xl=x1_ref.at[bl], hl=h2_ref.at[bl])
        else:
            n = 1 if bl is None else 2
            xw, hw = x1_ref.at[pl.ds(bf, n)], h2_ref.at[pl.ds(bf, n)]
            act.update(xf=xw.at[0], hf=hw.at[0], xl=xw.at[n - 1], hl=hw.at[n - 1])

    def ln_piece(b, r, paced, part=3):
        name = 'ln%d' % (r % LNCH)
        rs = slice(r * RC, (r + 1) * RC)
        if part & 1:
            x = q_ref[b, rs, :].astype(F32)
            h1 = norm(x, name if paced else None) * modrow(1) + modrow(0)
            x1 = x + h1 * y_ref[z2, rs, :]
            act['xl'][rs, :] = x1
            n2 = norm(x1)
            if part == 1:
                y_ref[z2, rs, :] = n2
        else:
            n2 = y_ref[z2, rs, :]
        if part & 2:
            h2 = n2 * modrow(4) + modrow(3)
            if paced:
                chain[name] = h2[:, 0:1]
            act['hl'][r * 8:(r + 1) * 8, :] = _pack(h2)

    def ln_all(b, paced, part=3):
        for r in range(TM // RC):
            ln_piece(b, r, paced, part)

    def weight(raw_ref, packed_ref, cs, first):
        if not first:
            return _unpack(packed_ref[:, cs])
        w = raw_ref[:, cs]
        packed_ref[:, cs] = pltpu.bitcast(w, U32)
        return w

    def gu(b, c, first=False, lngu=-1):
        cs = lanes(c)
        h2 = _unpack(act['hf'][...])
        gate = jnp.dot(h2, weight(wg_ref, wgp_ref, cs, first), preferred_element_type=F32)
        up = jnp.dot(h2, weight(wu_ref, wup_ref, cs, first), preferred_element_type=F32)
        act_ref[:, cs] = _pack(jnp.maximum(gate, 0.0) * up)
        if c == lngu:
            for i in range(LNCH):
                chain['ln%d' % i] = up[0:16, 0:1]

    def down(b, c, first=False):
        cs = lanes(c)
        gb = mod_ref[0:1, 5 * D + c * 128:5 * D + (c + 1) * 128]
        ff = jnp.dot(_unpack(act_ref[...]), weight(wd_ref, wdp_ref, cs, first),
                     preferred_element_type=F32)
        o_ref[b, :, cs] = (act['xf'][:, cs] + gb * ff).astype(BF16)

    def mod_part(i):
        c = c_ref[...].astype(F32)
        sc = jnp.broadcast_to((c * jax.nn.sigmoid(c)).astype(BF16), (8, D))
        return jnp.dot(sc, wmod_ref[:, i * D:(i + 1) * D], preferred_element_type=F32)

    def prologue():
        chain.clear()
        set_blocks(0, 0)
        cp_x(0).start()
        cp_s(0).start()
        for i in range(1, 5):
            cp_x(i).start()
        for lt in range(1, NLT):
            cp_s(lt).start()
        for b in range(2):
            cp_k(b).start()
            cp_v(b).start()
        cp_q(0).start()
        for i in range(3):
            cp_m(i).start()
        cp_k(2).start()
        cp_v(2).start()
        for i in (3, 4):
            cp_m(i).start()
        cp_q(1).start()
        for i in range(WCH):
            cp_g(i).start()
            cp_u(i).start()
        cp_m(5).start()
        for i in range(3):
            cp_d(i).start()
        cp_k(3).start()
        cp_v(3).start()
        for i in range(3, NLT):
            cp_d(i).start()
        for lt in range(NLT):
            uh[lt][0:UPAD, 0:3 * CH, :] = jnp.zeros((UPAD, 3 * CH, 128), F32)
        for i in range(5):
            cp_x(i).wait()
        dd = dd_ref[...].astype(F32)
        for lt in range(NLT):
            ddf_ref[lt] = jnp.broadcast_to(dd[lt:lt + 1, :], (8, 128))

        def kbody(lt, carry):
            cp_s(lt).wait()
            for j in range(NCH):
                dft_k(lt, j)
            return carry
        lax.fori_loop(0, NLT, kbody, 0)
        cp_k(0).wait()
        cp_v(0).wait()
        for lt in range(NLT):
            dft_u(0, 0, lt)
        cp_k(1).wait()
        cp_v(1).wait()
        for lt in range(NLT):
            dft_u(1, 1, lt)
            mac(0, 2, lt, False)
            inv(lt, True)
            mac(1, 4, lt, False)
        cp_q(0).wait()
        for i in range(3):
            cp_m(i).wait()
        ga = mod_part(2)
        mod_ref[:, 0:D] = mod_part(0) * ga
        mod_ref[:, D:2 * D] = (1.0 + mod_part(1)) * ga
        ln_all(0, False, part=1)
        cp_k(2).wait()
        cp_v(2).wait()
        for lt in range(NLT):
            dft_u(2, 2, lt)
        cp_m(3).wait()
        cp_m(4).wait()
        mod_ref[:, 3 * D:4 * D] = mod_part(3)
        mod_ref[:, 4 * D:5 * D] = 1.0 + mod_part(4)
        ln_all(0, False, part=2)
        for lt in range(NLT):
            inv(lt)

    def first_step():
        per = FF // 128 // WCH
        set_blocks(0, 1)
        lnr = [0, 2, 4, 7, 10, 13, 16]
        for i in range(WCH):
            if i == 0:
                cp_q(1).wait()
            cp_g(i).wait()
            cp_u(i).wait()
            chain.clear()
            if i < NLT:
                mac(2, 6, i, True)
            for r in range(lnr[i], lnr[i + 1]):
                ln_piece(1, r, False)
            for c in range(i * per, (i + 1) * per):
                gu(0, c, True)
        cp_m(5).wait()
        cp_d(0).wait()
        mod_ref[:, 5 * D:6 * D] = mod_part(5)
        down(0, 0, True)
        for c in range(1, NLT):
            if c == 3:
                cp_k(3).wait()
                cp_v(3).wait()
            cp_d(c).wait()
            down(0, c, True)
            for lt in {3: (0, 1, 2, 3), 4: (4,)}.get(c, ()):
                dft_u(3, 3, lt)

    def step(do_dft, do_mac, do_ln, last=False):
        chain.clear()
        set_blocks(g - 1, g if do_ln else None)
        if do_ln:
            for lt in range(NLT):
                t = inv(lt)
                if lt == MACDELAY:
                    chain.update(a=t, c=t)
        if do_mac:
            for lt in range(NLT):
                mac(g + 1, NCH, lt, True)
        for c in range(FF // 128):
            gu(g - 1, c, lngu=(LNGU if do_mac else LNGUT))
        for c in range(NLT):
            if do_dft:
                dft_u(g + 2, jnp.minimum(g + 2, NB - 1), c)
            down(g - 1, c)
            if last:
                cp_l(c).start()
        if do_ln:
            ln_all(g, True)

    def variant(tag, cond, fn):
        def body():
            with jax.named_scope('var' + tag):
                if tag in VARS:
                    fn()
        pl.when(cond)(body)

    variant('P', g == 0, prologue)

    @pl.when(jnp.logical_and(g >= 2, g + 2 < NB))
    def _():
        cp_k(g + 2).wait()
        cp_v(g + 2).wait()

    @pl.when(jnp.logical_and(g >= 1, g + 3 < NB))
    def _():
        cp_k(g + 3).start()
        cp_v(g + 3).start()

    @pl.when(jnp.logical_and(g >= 2, g < NB))
    def _():
        cp_q(g).wait()

    @pl.when(jnp.logical_and(g >= 1, g + 1 < NB))
    def _():
        cp_q(g + 1).start()

    @pl.when(g >= 2)
    def _():
        cp_o(g - 2).start()

    variant('1', g == 1, first_step)
    variant('B', jnp.logical_and(g >= 2, g <= 6 - USEC), lambda: step(True, True, True))
    if USEC:
        variant('C', g == 6, lambda: step(False, True, True))
    variant('T', g == 7, lambda: step(False, False, True))
    variant('U', g == 8, lambda: step(False, False, False, True))

    @pl.when(g == NB)
    def _():
        for b in range(NB - 1):
            cp_o(b).wait()
        if 'U' in VARS:
            for c in range(NLT):
                cp_l(c).wait()


@jax.jit
def pallas_adaLN_cond__ssm_conv_h3__glu_gated_reglu__prompt_kernel(
    A_q, A_k, A_v, A_shift_k, A_ssm_k, A_ssm_D, B_x, B_W_gate, B_W_up, B_W_down, c, w_mod,
):
    del B_x
    fwd, inv = _dft_tables()
    fwd = jnp.asarray(_pack_np(fwd))
    inv = jnp.asarray(_pack_np(inv))
    q = A_q.reshape(NB, TM, D)
    k = A_k.reshape(NB, TM, D)
    v = A_v.reshape(NB, TM, D)
    ssmk = A_ssm_k.reshape(NLT, 128, S)
    sk = A_shift_k.T
    dd = A_ssm_D.reshape(NLT, 128)

    hbm = pl.BlockSpec(memory_space=pl.ANY)

    out = pl.pallas_call(
        _kernel,
        grid=(NB + 1,),
        in_specs=[hbm] * 13,
        out_specs=hbm,
        out_shape=jax.ShapeDtypeStruct((NB, TM, D), BF16),
        scratch_shapes=[
            pltpu.VMEM((NB, TM, D), BF16),
            pltpu.VMEM((NB, TM, D), BF16),
            pltpu.VMEM((NB, TM, D), BF16),
            pltpu.VMEM((NB, TM, D), BF16),
            pltpu.VMEM((NLT, 128, S), BF16),
            pltpu.VMEM((D, FF), BF16),
            pltpu.VMEM((D, FF), BF16),
            pltpu.VMEM((FF, D), BF16),
            pltpu.VMEM((D, 6 * D), BF16),
            pltpu.SemaphoreType.DMA((70,)),
            pltpu.VMEM((8, 4096), F32),
            pltpu.VMEM((2 * CH, D), F32),
            pltpu.VMEM((2, 2 * CH, D), F32),
            pltpu.VMEM((NB, TM // 2, D), U32),
            pltpu.VMEM((NB, TM, D), F32),
            pltpu.VMEM((TM // 2, FF), U32),
            pltpu.VMEM((1, TM, D), F32),
            pltpu.VMEM((D // 2, FF), U32),
            pltpu.VMEM((D // 2, FF), U32),
            pltpu.VMEM((FF // 2, D), U32),
            pltpu.VMEM((NLT * NCH, KROWS, 128), F32),
        ] + [pltpu.VMEM((UPAD + NCH + 2, UROWS, 128), F32) for _ in range(NLT)] + [
            pltpu.VMEM((CH, CH), U32),
            pltpu.VMEM((CH // 2, 2 * CH), U32),
            pltpu.VMEM((8, 8, 128), F32),
            pltpu.VMEM((4, D), BF16),
            pltpu.VMEM((NLT, 128), BF16),
            pltpu.VMEM((1, D), BF16),
        ],
        compiler_params=pltpu.CompilerParams(
            dimension_semantics=("arbitrary",),
            vmem_limit_bytes=110 * 1024 * 1024,
            disable_bounds_checks=bool(int(os.environ.get('NOCHK', 1))),
            disable_semaphore_checks=bool(int(os.environ.get('NOCHK', 1)))),
    )(q, k, v, sk, ssmk, dd, B_W_gate, B_W_up, B_W_down, c, w_mod, fwd, inv)
    return out.reshape(1, S, D)
```

```python
import os
import numpy as np
import jax
import jax.numpy as jnp
from jax import lax
import jax.experimental.pallas as pl
import jax.experimental.pallas.tpu as pltpu

S = 2048
D = 640
FF = 1536
CH = 128
NCH = S // CH
TM = 256
NB = S // TM
NLT = D // 128
NP = CH // 8
EPS = 1e-5
UPAD = NCH - 8
USL = UPAD + NCH
KROWS = 3 * CH + 8
UROWS = 3 * CH + 64
ZR = 2 * CH
AR = TM // 2
WCH = 6
LPI = 8
RC = 16
F32 = jnp.float32
BF16 = jnp.bfloat16
U32 = jnp.uint32
VARS = os.environ.get('VARS', 'P1BCT')
LNCH = int(os.environ.get('LNCH', 2))
LNGU = int(os.environ.get('LNGU', 10))
LNGUT = int(os.environ.get('LNGUT', 6))
LPRIO = int(os.environ.get('LPRIO', 1))
INVPOS = int(os.environ.get('INVPOS', 1))


def _dft_tables():
    f = np.concatenate([np.arange(0, CH, 2), np.arange(1, CH, 2)])
    n = np.arange(CH)
    k = ((2 * f[:, None] + 1) * n[None, :]) % (4 * CH)
    ang = np.pi * k / (2 * CH)
    co = np.cos(ang).reshape(NP, 8, CH)
    si = np.sin(ang).reshape(NP, 8, CH)
    fwd = np.stack([co, si], axis=1).reshape(2 * CH, CH)
    inv = fwd.T / CH
    return fwd.astype(np.float32), inv.astype(np.float32)


def _pack_np(a):
    u = np.ascontiguousarray(a, np.float32).view(np.uint32)
    b = ((u + 0x7FFF + ((u >> 16) & 1)) >> 16).astype(np.uint32)
    return b[0::2] | (b[1::2] << 16)


def _pack(x):
    return pltpu.bitcast(x.astype(BF16), U32)


def _unpack(x):
    return pltpu.bitcast(x, BF16)


def _kernel(q_hbm, k_hbm, v_hbm, sk_hbm, ssmk_hbm, dd_hbm, wg_hbm, wu_hbm, wd_hbm,
            c_hbm, wmod_hbm, f_hbm, g_hbm, o_hbm,
            q_ref, k_ref, v_ref, o_ref, ssmk_ref, wg_ref, wu_ref, wd_ref, wmod_ref, sems,
            mod_ref, zprev_ref, z_ref, h2_ref, x1_ref, act_ref, y_ref,
            wgp_ref, wup_ref, wdp_ref, kh_ref, uh_ref,
            f_ref, g_ref, ddf_ref, sk_ref, dd_ref, c_ref):
    g = pl.program_id(0)
    sem_q, sem_k, sem_v, sem_o, sem_s, sem_m, sem_g, sem_u, sem_d, sem_l, sem_x = (
        0, 8, 16, 24, 32, 37, 43, 49, 55, 60, 65)
    thr = g - 1000
    never8 = lax.broadcasted_iota(jnp.int32, (8, 128), 0) < thr
    never_col = lax.broadcasted_iota(jnp.int32, (16, 1), 0) < thr
    z1 = lax.shift_right_logical(g, 10)
    z2 = lax.shift_right_logical(g, 11)
    chain = {}

    def link(name, m, mask=never8):
        prev = chain.get(name)
        return m if prev is None else jnp.where(mask, prev, m)

    def lanes(lt, w=128):
        if isinstance(lt, int):
            return slice(lt * w, (lt + 1) * w)
        return pl.ds(pl.multiple_of(lt * w, 128), w)

    def blk_copy(src, dst, sem, b):
        return pltpu.make_async_copy(src.at[b], dst.at[b], sems.at[sem + b])

    def cols_copy(src, dst, sem, i, w):
        cs = pl.ds(i * w, w) if isinstance(i, int) else lanes(i, w)
        return pltpu.make_async_copy(src.at[:, cs], dst.at[:, cs], sems.at[sem + i])

    cp_q = lambda b: blk_copy(q_hbm, q_ref, sem_q, b)
    cp_k = lambda b: blk_copy(k_hbm, k_ref, sem_k, b)
    cp_v = lambda b: blk_copy(v_hbm, v_ref, sem_v, b)
    cp_o = lambda b: blk_copy(o_ref, o_hbm, sem_o, b)
    cp_s = lambda lt: blk_copy(ssmk_hbm, ssmk_ref, sem_s, lt)
    cp_m = lambda i: pltpu.make_async_copy(
        wmod_hbm.at[:, pl.ds(i * D if isinstance(i, int) else pl.multiple_of(i * D, 128), D)],
        wmod_ref.at[i], sems.at[sem_m + i])
    cp_g = lambda i: cols_copy(wg_hbm, wg_ref, sem_g, i, FF // WCH)
    cp_u = lambda i: cols_copy(wu_hbm, wu_ref, sem_u, i, FF // WCH)
    cp_d = lambda i: cols_copy(wd_hbm, wd_ref, sem_d, i, 128)
    cp_l = lambda i: cols_copy(o_ref.at[NB - 1], o_hbm.at[NB - 1], sem_l, i, 128)

    cp_x = lambda i: pltpu.make_async_copy(
        (f_hbm, dd_hbm, sk_hbm, g_hbm, c_hbm)[i], (f_ref, dd_ref, sk_ref, g_ref, c_ref)[i],
        sems.at[sem_x + i])

    def dft_k(lt, j):
        kf = lax.dot_general(_unpack(f_ref[...]), ssmk_ref[lt, :, j * CH:(j + 1) * CH],
                             (((1,), (1,)), ((), ())), preferred_element_type=F32)
        for p in range(NP):
            kr = kf[16 * p:16 * p + 8]
            ki = kf[16 * p + 8:16 * p + 16]
            if j == 0:
                kr = kr + ddf_ref[lt]
            kh_ref[lt * NCH + j, 24 * p:24 * p + 8, :] = kr
            kh_ref[lt * NCH + j, 24 * p + 8:24 * p + 16, :] = ki - kr
            kh_ref[lt * NCH + j, 24 * p + 16:24 * p + 24, :] = kr + ki

    def dft_u(b, bsrc, lt, maybe_first=False):
        cs = lanes(lt)
        sk = sk_ref[:, cs].astype(F32)
        k = k_ref[bsrc, :, cs].astype(F32)
        if maybe_first:
            halo = k_ref[jnp.maximum(bsrc - 1, 0), TM - 8:TM, cs].astype(F32)
            halo = jnp.where(bsrc > 0, halo, 0.0)
        else:
            halo = k_ref[bsrc - 1, TM - 8:TM, cs].astype(F32)
        kext = jnp.concatenate([halo, k], axis=0)
        ks = k * sk[0:1, :]
        for t in range(1, 4):
            ks = ks + kext[8 - t:8 - t + TM, :] * sk[t:t + 1, :]
        kv = ks * v_ref[bsrc, :, cs].astype(F32)
        for cc in range(2):
            uf = jnp.dot(_unpack(f_ref[...]), kv[cc * CH:(cc + 1) * CH, :].astype(BF16),
                         preferred_element_type=F32)
            for p in range(NP):
                ur = uf[16 * p:16 * p + 8]
                ui = uf[16 * p + 8:16 * p + 16]
                uh_ref[lt * USL + UPAD + 2 * b + cc, 24 * p:24 * p + 8, :] = ur + ui
                uh_ref[lt * USL + UPAD + 2 * b + cc, 24 * p + 8:24 * p + 16, :] = ur
                uh_ref[lt * USL + UPAD + 2 * b + cc, 24 * p + 16:24 * p + 24, :] = ui

    def mac(b, njs, lt, paced):
        uw = uh_ref.at[pl.ds(lt * USL + UPAD + 2 * b + 2 - njs, njs)]
        for p in range(NP):
            base = {}
            for q in range(3):
                rr = pl.ds(24 * p + 8 * q, 8)
                acc = {}
                for o in 'ac':
                    if q == 1:
                        acc[o] = base[o]
                    elif q == 2:
                        acc[o] = link(o, base[o])
                kprev = None
                for t in range(njs):
                    u = uw[njs - 1 - t, rr, :]
                    k = kh_ref[lt * NCH + t, rr, :]
                    for o, kk in (('c', k), ('a', kprev)):
                        if kk is None:
                            continue
                        m = kk * u
                        if o not in acc:
                            acc[o] = link(o, m)
                        else:
                            acc[o] = acc[o] - m if q == 2 else acc[o] + m
                    kprev = k
                if q == 0:
                    base = acc
                else:
                    r0 = 16 * p + (8 if q == 1 else 0)
                    z_ref[2 * lt, r0:r0 + 8, :] = acc['a']
                    z_ref[2 * lt + 1, r0:r0 + 8, :] = acc['c']
                    if paced:
                        chain.update(acc)

    def inv(lt, first=False):
        cs = lanes(lt)
        za, zb = [], []
        for p in range(NP):
            re, im = slice(16 * p, 16 * p + 8), slice(16 * p + 8, 16 * p + 16)
            ar, ai = z_ref[2 * lt, re, :], z_ref[2 * lt, im, :]
            br, bi = z_ref[2 * lt + 1, re, :], z_ref[2 * lt + 1, im, :]
            if first:
                za += [ar, ai]
            else:
                pr, pi = zprev_ref[lt, re, :], zprev_ref[lt, im, :]
                za += [ar + pi, ai - pr] if p < NP // 2 else [ar - pi, ai + pr]
            zb += [br + ai, bi - ar] if p < NP // 2 else [br - ai, bi + ar]
            zprev_ref[lt, re, :] = br
            zprev_ref[lt, im, :] = bi
        for cc, z in enumerate((za, zb)):
            y = jnp.dot(_unpack(g_ref[...]), jnp.concatenate(z, axis=0).astype(BF16),
                        preferred_element_type=F32)
            y_ref[z1, cc * CH:(cc + 1) * CH, cs] = y
        return y[0:8]

    def norm(x, name=None):
        m = jnp.sum(x, axis=-1, keepdims=True) * (1.0 / D)
        if name is not None:
            m = link(name, m, never_col)
        xc = x - m
        v = jnp.sum(xc * xc, axis=-1, keepdims=True) * (1.0 / D)
        return xc * lax.rsqrt(v + EPS)

    def modrow(i):
        return mod_ref[i, 0:1, :]

    act = {}

    def set_blocks(bf, bl):
        if isinstance(bf, int):
            bl = bf if bl is None else bl
            act.update(xf=x1_ref.at[bf], hf=h2_ref.at[bf], xl=x1_ref.at[bl], hl=h2_ref.at[bl])
        else:
            n = 1 if bl is None else 2
            xw, hw = x1_ref.at[pl.ds(bf, n)], h2_ref.at[pl.ds(bf, n)]
            act.update(xf=xw.at[0], hf=hw.at[0], xl=xw.at[n - 1], hl=hw.at[n - 1])

    def ln_piece(b, r, paced, part=3):
        if isinstance(r, int):
            name = 'ln%d' % (r % LNCH)
            rs = slice(r * RC, (r + 1) * RC)
            hs = slice(r * 8, (r + 1) * 8)
        else:
            name = None
            rs = pl.ds(pl.multiple_of(r * RC, RC), RC)
            hs = pl.ds(pl.multiple_of(r * 8, 8), 8)
        if part & 1:
            x = q_ref[b, rs, :].astype(F32)
            h1 = norm(x, name if paced else None) * modrow(1) + modrow(0)
            x1 = x + h1 * y_ref[z2, rs, :]
            act['xl'][rs, :] = x1
            n2 = norm(x1)
            if part == 1:
                x1_ref[NB - 1, rs, :] = n2
        else:
            n2 = x1_ref[NB - 1, rs, :]
        if part & 2:
            h2 = n2 * modrow(4) + modrow(3)
            if paced:
                chain[name] = h2[:, 0:1]
            act['hl'][hs, :] = _pack(h2)

    def ln_all(b, paced, part=3):
        for r in range(TM // RC):
            ln_piece(b, r, paced, part)

    def tile(c, n):
        if isinstance(c, int):
            return slice(c * n, (c + 1) * n)
        return pl.ds(pl.multiple_of(c * n, 32), n)

    def weight(raw_ref, packed_ref, c, first):
        n = raw_ref.shape[0] // 2
        if not first:
            return _unpack(packed_ref[tile(c, n), :])
        w = raw_ref[:, lanes(c)]
        packed_ref[tile(c, n), :] = pltpu.bitcast(w, U32)
        return w

    def gu(b, c, first=False, lngu=-1, pair=None):
        cp, cj = (c // 2, c % 2) if pair is None else pair
        h2 = _unpack(act['hf'][...])
        gate = jnp.dot(h2, weight(wg_ref, wgp_ref, c, first), preferred_element_type=F32)
        up = jnp.dot(h2, weight(wu_ref, wup_ref, c, first), preferred_element_type=F32)
        act_ref[tile(cp, AR), lanes(cj)] = _pack(jnp.maximum(gate, 0.0) * up)
        if isinstance(c, int) and c == lngu:
            for i in range(LNCH):
                chain['ln%d' % i] = up[0:16, 0:1]

    def down(b, c, first=False):
        cs = lanes(c)
        gb = mod_ref[5, 0:1, cs]
        a = jnp.concatenate([act_ref[tile(j, AR), :] for j in range(FF // 256)], axis=1)
        ff = jnp.dot(_unpack(a), weight(wd_ref, wdp_ref, c, first),
                     preferred_element_type=F32)
        o_ref[b, :, cs] = (act['xf'][:, cs] + gb * ff).astype(BF16)

    def mod_part(i):
        c = c_ref[...].astype(F32)
        sc = jnp.broadcast_to((c * jax.nn.sigmoid(c)).astype(BF16), (8, D))
        return jnp.dot(sc, wmod_ref[i], preferred_element_type=F32)

    def prologue():
        chain.clear()
        set_blocks(0, 0)
        cp_x(0).start()
        cp_s(0).start()
        for i in range(1, 5):
            cp_x(i).start()
        for lt in range(1, NLT):
            cp_s(lt).start()
        for b in range(3):
            cp_k(b).start()
            cp_v(b).start()
        cp_q(0).start()
        for i in range(5):
            cp_m(i).start()
        cp_q(1).start()
        for i in range(WCH):
            cp_g(i).start()
            cp_u(i).start()
        cp_m(5).start()
        for i in range(3):
            cp_d(i).start()
        cp_k(3).start()
        cp_v(3).start()
        for i in range(3, NLT):
            cp_d(i).start()
        for b in range(2, NB):
            cp_q(b).start(priority=LPRIO)
            if b + 2 < NB:
                cp_k(b + 2).start(priority=LPRIO)
                cp_v(b + 2).start(priority=LPRIO)

        def zbody(j, carry):
            for lt in range(NLT):
                uh_ref[lt * USL + j, 0:3 * CH, :] = jnp.zeros((3 * CH, 128), F32)
            return carry
        lax.fori_loop(0, UPAD, zbody, 0)
        for i in range(5):
            cp_x(i).wait()
        dd = dd_ref[...].astype(F32)
        for lt in range(NLT):
            ddf_ref[lt] = jnp.broadcast_to(dd[lt:lt + 1, :], (8, 128))

        def kbody(lt, carry):
            cp_s(lt).wait()
            for j in range(NCH):
                dft_k(lt, j)
            return carry
        lax.fori_loop(0, NLT, kbody, 0)

        def ubody(b, carry):
            cp_k(b).wait()
            cp_v(b).wait()
            for lt in range(NLT):
                dft_u(b, b, lt, True)
            return carry
        lax.fori_loop(0, 3, ubody, 0)

        def cbody(lt, carry):
            mac(0, 2, lt, False)
            inv(lt, True)
            mac(1, 4, lt, False)
            return carry
        lax.fori_loop(0, NLT, cbody, 0)

        def mbody(i, carry):
            cp_m(i).wait()
            mod_ref[i] = mod_part(i)
            return carry

        def lbody(part):
            def body(i, carry):
                for r in range(LPI):
                    ln_piece(0, i * LPI + r, False, part)
                return carry
            lax.fori_loop(0, TM // RC // LPI, body, 0)
        lax.fori_loop(0, 3, mbody, 0)
        ga = mod_ref[2]
        mod_ref[0] = mod_ref[0] * ga
        mod_ref[1] = (1.0 + mod_ref[1]) * ga
        cp_q(0).wait()
        lbody(1)
        for lt in range(NLT):
            inv(lt)
        lax.fori_loop(3, 5, mbody, 0)
        mod_ref[4] = 1.0 + mod_ref[4]
        lbody(2)

    def first_step():
        per = FF // 128 // WCH
        set_blocks(0, 1)
        cp_q(1).wait()

        def gbody(i, carry):
            cp_g(i).wait()
            cp_u(i).wait()
            chain.clear()
            for c in range(per):
                gu(0, i * per + c, True, pair=(i, c))
            mac(2, 6, jnp.minimum(i, NLT - 1), True)
            for r in range(3):
                ln_piece(1, jnp.minimum(3 * i + r, TM // RC - 1), False)
            return carry
        lax.fori_loop(0, WCH, gbody, 0)
        cp_m(5).wait()
        cp_d(0).wait()
        mod_ref[5] = mod_part(5)
        down(0, 0, True)
        for c in range(1, NLT):
            if c == 3:
                cp_k(3).wait()
                cp_v(3).wait()
            cp_d(c).wait()
            down(0, c, True)
            for lt in {3: (0, 1, 2, 3), 4: (4,)}.get(c, ()):
                dft_u(3, 3, lt)
        cp_o(0).start()

    def step(bf, do_dft, do_mac, do_ln, last=False):
        chain.clear()
        set_blocks(bf, bf + 1 if do_ln else None)
        for c in range(FF // 128):
            if c == INVPOS and do_ln:
                for lt in range(NLT):
                    inv(lt)
                if do_mac:
                    for lt in range(NLT):
                        mac(bf + 2, NCH, lt, True)
            gu(bf, c, lngu=(LNGU if do_mac else LNGUT))
        for c in range(NLT):
            if do_dft:
                dft_u(bf + 3, bf + 3, c)
            down(bf, c)
            if last:
                cp_l(c).start()
        if do_ln:
            ln_all(bf + 1, True)
        if not last:
            cp_o(bf).start()

    def tail():
        step(NB - 3, False, True, True)
        step(NB - 2, False, False, True)
        step(NB - 1, False, False, False, True)
        for b in range(NB - 1):
            cp_o(b).wait()
        for c in range(NLT):
            cp_l(c).wait()

    def variant(tag, cond, fn):
        def body():
            with jax.named_scope('var' + tag):
                fn()
        pl.when(cond)(body)

    variant('P', g == 0, prologue)

    @pl.when(jnp.logical_and(g >= 2, g + 2 < NB))
    def _():
        cp_k(g + 2).wait()
        cp_v(g + 2).wait()

    @pl.when(g >= 2)
    def _():
        cp_q(g).wait()

    @pl.when(g == NB - 2)
    def _():
        cp_q(NB - 1).wait()

    variant('1', g == 1, first_step)
    variant('B', jnp.logical_and(g >= 2, g <= NB - 3), lambda: step(g - 1, True, True, True))
    variant('T', g == NB - 2, tail)


@jax.jit
def pallas_adaLN_cond__ssm_conv_h3__glu_gated_reglu__prompt_kernel(
    A_q, A_k, A_v, A_shift_k, A_ssm_k, A_ssm_D, B_x, B_W_gate, B_W_up, B_W_down, c, w_mod,
):
    del B_x
    fwd, inv = _dft_tables()
    fwd = jnp.asarray(_pack_np(fwd))
    inv = jnp.asarray(_pack_np(inv))
    q = A_q.reshape(NB, TM, D)
    k = A_k.reshape(NB, TM, D)
    v = A_v.reshape(NB, TM, D)
    ssmk = A_ssm_k.reshape(NLT, 128, S)
    sk = A_shift_k.T
    dd = A_ssm_D.reshape(NLT, 128)

    hbm = pl.BlockSpec(memory_space=pl.ANY)

    out = pl.pallas_call(
        _kernel,
        grid=(NB - 1,),
        in_specs=[hbm] * 13,
        out_specs=hbm,
        out_shape=jax.ShapeDtypeStruct((NB, TM, D), BF16),
        scratch_shapes=[
            pltpu.VMEM((NB, TM, D), BF16),
            pltpu.VMEM((NB, TM, D), BF16),
            pltpu.VMEM((NB, TM, D), BF16),
            pltpu.VMEM((NB, TM, D), BF16),
            pltpu.VMEM((NLT, 128, S), BF16),
            pltpu.VMEM((D, FF), BF16),
            pltpu.VMEM((D, FF), BF16),
            pltpu.VMEM((FF, D), BF16),
            pltpu.VMEM((6, D, D), BF16),
            pltpu.SemaphoreType.DMA((70,)),
            pltpu.VMEM((8, 8, D), F32),
            pltpu.VMEM((NLT, ZR, 128), F32),
            pltpu.VMEM((2 * NLT, ZR, 128), F32),
            pltpu.VMEM((NB, TM // 2, D), U32),
            pltpu.VMEM((NB, TM, D), F32),
            pltpu.VMEM((FF // 256 * AR, 256), U32),
            pltpu.VMEM((1, TM, D), F32),
            pltpu.VMEM((FF // 128 * D // 2, 128), U32),
            pltpu.VMEM((FF // 128 * D // 2, 128), U32),
            pltpu.VMEM((NLT * FF // 2, 128), U32),
            pltpu.VMEM((NLT * NCH, KROWS, 128), F32),
            pltpu.VMEM((NLT * USL, UROWS, 128), F32),
            pltpu.VMEM((CH, CH), U32),
            pltpu.VMEM((CH // 2, 2 * CH), U32),
            pltpu.VMEM((8, 8, 128), F32),
            pltpu.VMEM((4, D), BF16),
            pltpu.VMEM((NLT, 128), BF16),
            pltpu.VMEM((1, D), BF16),
        ],
        compiler_params=pltpu.CompilerParams(
            dimension_semantics=("arbitrary",),
            vmem_limit_bytes=110 * 1024 * 1024,
            disable_bounds_checks=bool(int(os.environ.get('NOCHK', 1))),
            disable_semaphore_checks=bool(int(os.environ.get('NOCHK', 1)))),
    )(q, k, v, sk, ssmk, dd, B_W_gate, B_W_up, B_W_down, c, w_mod, fwd, inv)
    return out.reshape(1, S, D)
```

```python
import os
import numpy as np
import jax
import jax.numpy as jnp
from jax import lax
import jax.experimental.pallas as pl
import jax.experimental.pallas.tpu as pltpu

S = 2048
D = 640
FF = 1536
CH = 128
NCH = S // CH
TM = 256
NB = S // TM
NLT = D // 128
NP = CH // 8
EPS = 1e-5
UPAD = NCH - 8
USL = UPAD + NCH
KROWS = 3 * CH + 8
UROWS = 3 * CH + 64
ZR = 2 * CH
AR = TM // 2
WCH = 6
LPI = 8
RC = 16
F32 = jnp.float32
BF16 = jnp.bfloat16
U32 = jnp.uint32
VARS = os.environ.get('VARS', 'P1BCT')
LNCH = int(os.environ.get('LNCH', 2))
LNGU = int(os.environ.get('LNGU', 11))
LNGUC = int(os.environ.get('LNGUC', 10))
LNGUT = int(os.environ.get('LNGUT', 6))
LPRIO = int(os.environ.get('LPRIO', 1))
DFTAT = [int(x) for x in os.environ.get('DFTAT', '12,13,14,15,16').split(',')]
INVAT = [int(x) for x in os.environ.get('INVAT', '1,2,3,4,5').split(',')]


def _dft_tables():
    f = np.concatenate([np.arange(0, CH, 2), np.arange(1, CH, 2)])
    n = np.arange(CH)
    k = ((2 * f[:, None] + 1) * n[None, :]) % (4 * CH)
    ang = np.pi * k / (2 * CH)
    co = np.cos(ang).reshape(NP, 8, CH)
    si = np.sin(ang).reshape(NP, 8, CH)
    fwd = np.stack([co, si], axis=1).reshape(2 * CH, CH)
    inv = fwd.T / CH
    return fwd.astype(np.float32), inv.astype(np.float32)


def _pack_np(a):
    u = np.ascontiguousarray(a, np.float32).view(np.uint32)
    b = ((u + 0x7FFF + ((u >> 16) & 1)) >> 16).astype(np.uint32)
    return b[0::2] | (b[1::2] << 16)


def _pack(x):
    return pltpu.bitcast(x.astype(BF16), U32)


def _unpack(x):
    return pltpu.bitcast(x, BF16)


def _kernel(q_hbm, k_hbm, v_hbm, sk_hbm, ssmk_hbm, dd_hbm, wg_hbm, wu_hbm, wd_hbm,
            c_hbm, wmod_hbm, f_hbm, g_hbm, o_hbm,
            q_ref, k_ref, v_ref, o_ref, ssmk_ref, wg_ref, wu_ref, wd_ref, wmod_ref, sems,
            mod_ref, zprev_ref, z_ref, h2_ref, x1_ref, act_ref, y_ref,
            wgp_ref, wup_ref, wdp_ref, kh_ref, uh_ref,
            f_ref, g_ref, ddf_ref, sk_ref, dd_ref, c_ref):
    g = pl.program_id(0)
    sem_q, sem_k, sem_v, sem_o, sem_s, sem_m, sem_g, sem_u, sem_d, sem_l, sem_x = (
        0, 8, 16, 24, 32, 37, 43, 49, 55, 60, 65)
    thr = g - 1000
    never8 = lax.broadcasted_iota(jnp.int32, (8, 128), 0) < thr
    never_col = lax.broadcasted_iota(jnp.int32, (16, 1), 0) < thr
    z1 = lax.shift_right_logical(g, 10)
    z2 = lax.shift_right_logical(g, 11)
    chain = {}

    def link(name, m, mask=never8):
        prev = chain.get(name)
        return m if prev is None else jnp.where(mask, prev, m)

    def lanes(lt, w=128):
        if isinstance(lt, int):
            return slice(lt * w, (lt + 1) * w)
        return pl.ds(pl.multiple_of(lt * w, 128), w)

    def blk_copy(src, dst, sem, b):
        return pltpu.make_async_copy(src.at[b], dst.at[b], sems.at[sem + b])

    def colds(i, w):
        return pl.ds(i * w, w) if isinstance(i, int) else lanes(i, w)

    def cols_copy(src, dst, sem, i, w):
        cs = colds(i, w)
        return pltpu.make_async_copy(src.at[:, cs], dst.at[:, cs], sems.at[sem + i])

    cp_q = lambda b: blk_copy(q_hbm, q_ref, sem_q, b)
    cp_k = lambda b: blk_copy(k_hbm, k_ref, sem_k, b)
    cp_v = lambda b: blk_copy(v_hbm, v_ref, sem_v, b)
    cp_o = lambda b: blk_copy(o_ref, o_hbm, sem_o, b)
    cp_s = lambda lt: blk_copy(ssmk_hbm, ssmk_ref, sem_s, lt)
    cp_m = lambda i: pltpu.make_async_copy(
        wmod_hbm.at[:, pl.ds(i * D if isinstance(i, int) else pl.multiple_of(i * D, 128), D)],
        wmod_ref.at[i], sems.at[sem_m + i])
    cp_g = lambda i: pltpu.make_async_copy(
        wg_hbm.at[:, colds(i, FF // WCH)], wg_ref.at[i], sems.at[sem_g + i])
    cp_u = lambda i: pltpu.make_async_copy(
        wu_hbm.at[:, colds(i, FF // WCH)], wu_ref.at[i], sems.at[sem_u + i])
    cp_d = lambda i: cols_copy(wd_hbm, wd_ref, sem_d, i, 128)
    cp_l = lambda i: cols_copy(o_ref.at[NB - 1], o_hbm.at[NB - 1], sem_l, i, 128)

    cp_x = lambda i: pltpu.make_async_copy(
        (f_hbm, dd_hbm, sk_hbm, g_hbm, c_hbm)[i], (f_ref, dd_ref, sk_ref, g_ref, c_ref)[i],
        sems.at[sem_x + i])

    def dft_k(lt, j):
        kf = lax.dot_general(_unpack(f_ref[...]), ssmk_ref[lt, :, j * CH:(j + 1) * CH],
                             (((1,), (1,)), ((), ())), preferred_element_type=F32)
        for p in range(NP):
            kr = kf[16 * p:16 * p + 8]
            ki = kf[16 * p + 8:16 * p + 16]
            if j == 0:
                kr = kr + ddf_ref[lt]
            kh_ref[lt * NCH + j, 24 * p:24 * p + 8, :] = kr
            kh_ref[lt * NCH + j, 24 * p + 8:24 * p + 16, :] = ki - kr
            kh_ref[lt * NCH + j, 24 * p + 16:24 * p + 24, :] = kr + ki

    def dft_u(b, bsrc, lt, maybe_first=False):
        cs = lanes(lt)
        sk = sk_ref[:, cs].astype(F32)
        k = k_ref[bsrc, :, cs].astype(F32)
        if maybe_first:
            halo = k_ref[jnp.maximum(bsrc - 1, 0), TM - 8:TM, cs].astype(F32)
            halo = jnp.where(bsrc > 0, halo, 0.0)
        else:
            halo = k_ref[bsrc - 1, TM - 8:TM, cs].astype(F32)
        kext = jnp.concatenate([halo, k], axis=0)
        ks = k * sk[0:1, :]
        for t in range(1, 4):
            ks = ks + kext[8 - t:8 - t + TM, :] * sk[t:t + 1, :]
        kv = ks * v_ref[bsrc, :, cs].astype(F32)
        for cc in range(2):
            uf = jnp.dot(_unpack(f_ref[...]), kv[cc * CH:(cc + 1) * CH, :].astype(BF16),
                         preferred_element_type=F32)
            for p in range(NP):
                ur = uf[16 * p:16 * p + 8]
                ui = uf[16 * p + 8:16 * p + 16]
                uh_ref[lt * USL + UPAD + 2 * b + cc, 24 * p:24 * p + 8, :] = ur + ui
                uh_ref[lt * USL + UPAD + 2 * b + cc, 24 * p + 8:24 * p + 16, :] = ur
                uh_ref[lt * USL + UPAD + 2 * b + cc, 24 * p + 16:24 * p + 24, :] = ui

    def mac(b, njs, lt, paced):
        uw = uh_ref.at[pl.ds(lt * USL + UPAD + 2 * b + 2 - njs, njs)]
        for p in range(NP):
            base = {}
            for q in range(3):
                rr = pl.ds(24 * p + 8 * q, 8)
                acc = {}
                for o in 'ac':
                    if q == 1:
                        acc[o] = base[o]
                    elif q == 2:
                        acc[o] = link(o, base[o])
                kprev = None
                for t in range(njs):
                    u = uw[njs - 1 - t, rr, :]
                    k = kh_ref[lt * NCH + t, rr, :]
                    for o, kk in (('c', k), ('a', kprev)):
                        if kk is None:
                            continue
                        m = kk * u
                        if o not in acc:
                            acc[o] = link(o, m)
                        else:
                            acc[o] = acc[o] - m if q == 2 else acc[o] + m
                    kprev = k
                if q == 0:
                    base = acc
                else:
                    r0 = 16 * p + (8 if q == 1 else 0)
                    z_ref[2 * lt, r0:r0 + 8, :] = acc['a']
                    z_ref[2 * lt + 1, r0:r0 + 8, :] = acc['c']
                    if paced:
                        chain.update(acc)

    def inv(lt, first=False, ys=0):
        cs = lanes(lt)
        za, zb = [], []
        for p in range(NP):
            re, im = slice(16 * p, 16 * p + 8), slice(16 * p + 8, 16 * p + 16)
            ar, ai = z_ref[2 * lt, re, :], z_ref[2 * lt, im, :]
            br, bi = z_ref[2 * lt + 1, re, :], z_ref[2 * lt + 1, im, :]
            if first:
                za += [ar, ai]
            else:
                pr, pi = zprev_ref[lt, re, :], zprev_ref[lt, im, :]
                za += [ar + pi, ai - pr] if p < NP // 2 else [ar - pi, ai + pr]
            zb += [br + ai, bi - ar] if p < NP // 2 else [br - ai, bi + ar]
            zprev_ref[lt, re, :] = br
            zprev_ref[lt, im, :] = bi
        for cc, z in enumerate((za, zb)):
            y = jnp.dot(_unpack(g_ref[...]), jnp.concatenate(z, axis=0).astype(BF16),
                        preferred_element_type=F32)
            y_ref[z1 + ys, cc * CH:(cc + 1) * CH, cs] = y
        return y[0:8]

    def norm(x, name=None):
        m = jnp.sum(x, axis=-1, keepdims=True) * (1.0 / D)
        if name is not None:
            m = link(name, m, never_col)
        xc = x - m
        v = jnp.sum(xc * xc, axis=-1, keepdims=True) * (1.0 / D)
        return xc * lax.rsqrt(v + EPS)

    def modrow(i):
        return mod_ref[i, 0:1, :]

    act = {}

    def set_blocks(bf, bl):
        if isinstance(bf, int):
            bl = bf if bl is None else bl
            act.update(xf=x1_ref.at[bf], hf=h2_ref.at[bf], xl=x1_ref.at[bl], hl=h2_ref.at[bl])
        else:
            n = 1 if bl is None else 2
            xw, hw = x1_ref.at[pl.ds(bf, n)], h2_ref.at[pl.ds(bf, n)]
            act.update(xf=xw.at[0], hf=hw.at[0], xl=xw.at[n - 1], hl=hw.at[n - 1])

    def ln_piece(b, r, paced, part=3, ys=0):
        if isinstance(r, int):
            name = 'ln%d' % (r % LNCH)
            rs = slice(r * RC, (r + 1) * RC)
            hs = slice(r * 8, (r + 1) * 8)
        else:
            name = None
            rs = pl.ds(pl.multiple_of(r * RC, RC), RC)
            hs = pl.ds(pl.multiple_of(r * 8, 8), 8)
        if part & 1:
            x = q_ref[b, rs, :].astype(F32)
            h1 = norm(x, name if paced else None) * modrow(1) + modrow(0)
            x1 = x + h1 * y_ref[z2 + ys, rs, :]
            act['xl'][rs, :] = x1
            n2 = norm(x1)
            if part == 1:
                x1_ref[NB - 1 - b, rs, :] = n2
        else:
            n2 = x1_ref[NB - 1 - b, rs, :]
        if part & 2:
            h2 = n2 * modrow(4) + modrow(3)
            if paced:
                chain[name] = h2[:, 0:1]
            act['hl'][hs, :] = _pack(h2)

    def ln_all(b, paced, part=3):
        for r in range(TM // RC):
            ln_piece(b, r, paced, part)

    def tile(c, n):
        if isinstance(c, int):
            return slice(c * n, (c + 1) * n)
        return pl.ds(pl.multiple_of(c * n, 32), n)

    def weight(raw, packed_ref, c, n, first):
        if not first:
            return _unpack(packed_ref[tile(c, n), :])
        w = raw()
        packed_ref[tile(c, n), :] = pltpu.bitcast(w, U32)
        return w

    def gu(b, c, first=False, lngu=-1, pair=None):
        cp, cj = (c // 2, c % 2) if pair is None else pair
        h2 = _unpack(act['hf'][...])
        gate = jnp.dot(h2, weight(lambda: wg_ref[cp, :, lanes(cj)], wgp_ref, c, D // 2, first), preferred_element_type=F32)
        up = jnp.dot(h2, weight(lambda: wu_ref[cp, :, lanes(cj)], wup_ref, c, D // 2, first), preferred_element_type=F32)
        act_ref[tile(cp, AR), lanes(cj)] = _pack(jnp.maximum(gate, 0.0) * up)
        if isinstance(c, int) and c == lngu:
            for i in range(LNCH):
                chain['ln%d' % i] = up[0:16, 0:1]

    def down(b, c, first=False):
        cs = lanes(c)
        gb = mod_ref[5, 0:1, cs]
        a = jnp.concatenate([act_ref[tile(j, AR), :] for j in range(FF // 256)], axis=1)
        ff = jnp.dot(_unpack(a), weight(lambda: wd_ref[:, cs], wdp_ref, c, FF // 2, first),
                     preferred_element_type=F32)
        o_ref[b, :, cs] = (act['xf'][:, cs] + gb * ff).astype(BF16)

    def mod_part(i):
        c = c_ref[...].astype(F32)
        sc = jnp.broadcast_to((c * jax.nn.sigmoid(c)).astype(BF16), (8, D))
        return jnp.dot(sc, wmod_ref[i], preferred_element_type=F32)

    def prologue():
        chain.clear()
        set_blocks(0, 0)
        cp_x(0).start()
        cp_s(0).start()
        for i in range(1, 5):
            cp_x(i).start()
        for lt in range(1, NLT):
            cp_s(lt).start()
        for b in range(3):
            cp_k(b).start()
            cp_v(b).start()
        cp_q(0).start()
        cp_q(1).start()
        for i in range(5):
            cp_m(i).start()
        for i in range(WCH):
            cp_g(i).start()
            cp_u(i).start()
        cp_m(5).start()
        for i in range(3):
            cp_d(i).start()
        cp_k(3).start()
        cp_v(3).start()
        for i in range(3, NLT):
            cp_d(i).start()
        for b in range(2, NB):
            cp_q(b).start(priority=LPRIO)
            if b + 2 < NB:
                cp_k(b + 2).start(priority=LPRIO)
                cp_v(b + 2).start(priority=LPRIO)

        def zbody(j, carry):
            for lt in range(NLT):
                uh_ref[lt * USL + j, 0:3 * CH, :] = jnp.zeros((3 * CH, 128), F32)
            return carry
        lax.fori_loop(0, UPAD, zbody, 0)
        for i in range(5):
            cp_x(i).wait()
        dd = dd_ref[...].astype(F32)
        for lt in range(NLT):
            ddf_ref[lt] = jnp.broadcast_to(dd[lt:lt + 1, :], (8, 128))

        def kbody(lt, carry):
            cp_s(lt).wait()
            for j in range(NCH):
                dft_k(lt, j)
            return carry
        lax.fori_loop(0, NLT, kbody, 0)

        def ubody(b, carry):
            cp_k(b).wait()
            cp_v(b).wait()
            for lt in range(NLT):
                dft_u(b, b, lt, True)
            return carry
        lax.fori_loop(0, 3, ubody, 0)

        def cbody(lt, carry):
            mac(0, 2, lt, False)
            inv(lt, True)
            mac(1, 4, lt, False)
            inv(lt, ys=1)
            return carry
        lax.fori_loop(0, NLT, cbody, 0)

        def mbody(i, carry):
            cp_m(i).wait()
            mod_ref[i] = mod_part(i)
            return carry

        def lbody(part):
            n = TM // RC // LPI

            def body(i, carry):
                b = i // n
                act.update(xl=x1_ref.at[b], hl=h2_ref.at[b])
                for r in range(LPI):
                    ln_piece(b, (i % n) * LPI + r, False, part, b)
                return carry
            lax.fori_loop(0, 2 * n, body, 0)
        lax.fori_loop(0, 3, mbody, 0)
        ga = mod_ref[2]
        mod_ref[0] = mod_ref[0] * ga
        mod_ref[1] = (1.0 + mod_ref[1]) * ga
        cp_q(0).wait()
        cp_q(1).wait()
        lbody(1)
        lax.fori_loop(3, 5, mbody, 0)
        mod_ref[4] = 1.0 + mod_ref[4]
        lbody(2)

    def first_step():
        per = FF // 128 // WCH
        set_blocks(0, 1)

        def gbody(i, carry):
            cp_g(i).wait()
            cp_u(i).wait()
            chain.clear()
            for c in range(per):
                gu(0, i * per + c, True, pair=(i, c))
            mac(2, 6, jnp.minimum(i, NLT - 1), True)
            return carry
        lax.fori_loop(0, WCH, gbody, 0)
        cp_m(5).wait()
        cp_d(0).wait()
        mod_ref[5] = mod_part(5)
        down(0, 0, True)
        for c in range(1, NLT):
            if c == 3:
                cp_k(3).wait()
                cp_v(3).wait()
            cp_d(c).wait()
            down(0, c, True)
            for lt in {3: (0, 1, 2, 3), 4: (4,)}.get(c, ()):
                dft_u(3, 3, lt)
        cp_o(0).start()

    def step(bf, do_dft, do_mac, do_ln, last=False):
        chain.clear()
        set_blocks(bf, bf + 1 if do_ln else None)
        for c in range(FF // 128):
            for lt in range(NLT):
                if do_ln and c == INVAT[lt]:
                    inv(lt)
                    if do_mac:
                        mac(bf + 2, NCH, lt, True)
                if do_dft and c == DFTAT[lt]:
                    dft_u(bf + 3, bf + 3, lt)
            gu(bf, c, lngu=(LNGU if do_dft else LNGUC if do_mac else LNGUT))
        for c in range(NLT):
            for lt in range(NLT):
                if do_dft and c + FF // 128 == DFTAT[lt]:
                    dft_u(bf + 3, bf + 3, lt)
            down(bf, c)
            if last:
                cp_l(c).start()
        if do_ln:
            ln_all(bf + 1, True)
        if not last:
            cp_o(bf).start()

    def tail():
        step(NB - 3, False, True, True)
        step(NB - 2, False, False, True)
        step(NB - 1, False, False, False, True)
        for b in range(NB - 1):
            cp_o(b).wait()
        for c in range(NLT):
            cp_l(c).wait()

    def variant(tag, cond, fn):
        def body():
            with jax.named_scope('var' + tag):
                fn()
        pl.when(cond)(body)

    variant('P', g == 0, prologue)

    @pl.when(jnp.logical_and(g >= 2, g + 2 < NB))
    def _():
        cp_k(g + 2).wait()
        cp_v(g + 2).wait()

    @pl.when(g >= 2)
    def _():
        cp_q(g).wait()

    @pl.when(g == NB - 2)
    def _():
        cp_q(NB - 1).wait()

    variant('1', g == 1, first_step)
    variant('B', jnp.logical_and(g >= 2, g <= NB - 3), lambda: step(g - 1, True, True, True))
    variant('T', g == NB - 2, tail)


@jax.jit
def pallas_adaLN_cond__ssm_conv_h3__glu_gated_reglu__prompt_kernel(
    A_q, A_k, A_v, A_shift_k, A_ssm_k, A_ssm_D, B_x, B_W_gate, B_W_up, B_W_down, c, w_mod,
):
    del B_x
    fwd, inv = _dft_tables()
    fwd = jnp.asarray(_pack_np(fwd))
    inv = jnp.asarray(_pack_np(inv))
    q = A_q.reshape(NB, TM, D)
    k = A_k.reshape(NB, TM, D)
    v = A_v.reshape(NB, TM, D)
    ssmk = A_ssm_k.reshape(NLT, 128, S)
    sk = A_shift_k.T
    dd = A_ssm_D.reshape(NLT, 128)

    hbm = pl.BlockSpec(memory_space=pl.ANY)

    out = pl.pallas_call(
        _kernel,
        grid=(NB - 1,),
        in_specs=[hbm] * 13,
        out_specs=hbm,
        out_shape=jax.ShapeDtypeStruct((NB, TM, D), BF16),
        scratch_shapes=[
            pltpu.VMEM((NB, TM, D), BF16),
            pltpu.VMEM((NB, TM, D), BF16),
            pltpu.VMEM((NB, TM, D), BF16),
            pltpu.VMEM((NB, TM, D), BF16),
            pltpu.VMEM((NLT, 128, S), BF16),
            pltpu.VMEM((WCH, D, FF // WCH), BF16),
            pltpu.VMEM((WCH, D, FF // WCH), BF16),
            pltpu.VMEM((FF, D), BF16),
            pltpu.VMEM((6, D, D), BF16),
            pltpu.SemaphoreType.DMA((70,)),
            pltpu.VMEM((8, 8, D), F32),
            pltpu.VMEM((NLT, ZR, 128), F32),
            pltpu.VMEM((2 * NLT, ZR, 128), F32),
            pltpu.VMEM((NB, TM // 2, D), U32),
            pltpu.VMEM((NB, TM, D), F32),
            pltpu.VMEM((FF // 256 * AR, 256), U32),
            pltpu.VMEM((2, TM, D), F32),
            pltpu.VMEM((FF // 128 * D // 2, 128), U32),
            pltpu.VMEM((FF // 128 * D // 2, 128), U32),
            pltpu.VMEM((NLT * FF // 2, 128), U32),
            pltpu.VMEM((NLT * NCH, KROWS, 128), F32),
            pltpu.VMEM((NLT * USL, UROWS, 128), F32),
            pltpu.VMEM((CH, CH), U32),
            pltpu.VMEM((CH // 2, 2 * CH), U32),
            pltpu.VMEM((8, 8, 128), F32),
            pltpu.VMEM((4, D), BF16),
            pltpu.VMEM((NLT, 128), BF16),
            pltpu.VMEM((1, D), BF16),
        ],
        compiler_params=pltpu.CompilerParams(
            dimension_semantics=("arbitrary",),
            vmem_limit_bytes=110 * 1024 * 1024,
            disable_bounds_checks=bool(int(os.environ.get('NOCHK', 1))),
            disable_semaphore_checks=bool(int(os.environ.get('NOCHK', 1)))),
    )(q, k, v, sk, ssmk, dd, B_W_gate, B_W_up, B_W_down, c, w_mod, fwd, inv)
    return out.reshape(1, S, D)
```

```python
import numpy as np
import jax
import jax.numpy as jnp
from jax import lax
import jax.experimental.pallas as pl
import jax.experimental.pallas.tpu as pltpu

S = 2048
D = 640
FF = 1536
CH = 128
NCH = S // CH
TM = 256
NB = S // TM
NLT = D // 128
NFT = FF // 128
NP = CH // 8
EPS = 1e-5
UPAD = NCH - 10
USL = UPAD + NCH
KROWS = 3 * CH + 8
UROWS = 3 * CH + 64
WCH = 6
RC = 16
LN_CHAINS = 2
F32 = jnp.float32
BF16 = jnp.bfloat16
U32 = jnp.uint32


def _dft_tables():
    f = np.concatenate([np.arange(0, CH, 2), np.arange(1, CH, 2)])
    n = np.arange(CH)
    k = ((2 * f[:, None] + 1) * n[None, :]) % (4 * CH)
    ang = np.pi * k / (2 * CH)
    co = np.cos(ang).reshape(NP, 8, CH)
    si = np.sin(ang).reshape(NP, 8, CH)
    fwd = np.stack([co, si], axis=1).reshape(2 * CH, CH)
    return fwd, fwd.T / CH


def _pack_np(a):
    u = np.ascontiguousarray(a, np.float32).view(np.uint32)
    b = ((u + 0x7FFF + ((u >> 16) & 1)) >> 16).astype(np.uint32)
    return b[0::2] | (b[1::2] << 16)


def _pack(x):
    return pltpu.bitcast(x.astype(BF16), U32)


def _unpack(x):
    return pltpu.bitcast(x, BF16)


def _dot(a, b):
    return jnp.dot(a, b, preferred_element_type=F32)


def _kernel(q_hbm, k_hbm, v_hbm, sk_hbm, ssmk_hbm, dd_hbm, wg_hbm, wu_hbm, wd_hbm,
            c_hbm, wmod_hbm, f_hbm, g_hbm, o_hbm,
            q_ref, k_ref, v_ref, o_ref, ssmk_ref, wg_ref, wu_ref, wd_ref, wmod_ref, sems,
            mod_ref, zprev_ref, z_ref, h2_ref, x1_ref, act_ref, y_ref,
            wgp_ref, wup_ref, wdp_ref, kh_ref, uh_ref,
            f_ref, g_ref, ddf_ref, sk_ref, dd_ref, c_ref):
    g = pl.program_id(0)
    never8 = lax.broadcasted_iota(jnp.int32, (8, 128), 0) < g - 1000
    never_col = lax.broadcasted_iota(jnp.int32, (RC, 1), 0) < g - 1000
    z1 = lax.shift_right_logical(g, 10)
    z2 = lax.shift_right_logical(g, 11)
    chain = {}

    def link(name, m, mask=never8):
        prev = chain.get(name)
        return m if prev is None else jnp.where(mask, prev, m)

    def span(i, w, align):
        if isinstance(i, int):
            return pl.ds(i * w, w)
        return pl.ds(pl.multiple_of(i * w, align), w)

    def lanes(i, w=128):
        return span(i, w, 128)

    sem_q, sem_k, sem_v, sem_o, sem_s, sem_m, sem_g, sem_u, sem_d, sem_l, sem_x = (
        0, 8, 16, 24, 32, 37, 43, 49, 55, 60, 65)

    def copy(src, dst, sem):
        return pltpu.make_async_copy(src, dst, sems.at[sem])

    cp_q = lambda b: copy(q_hbm.at[b], q_ref.at[b], sem_q + b)
    cp_k = lambda b: copy(k_hbm.at[b], k_ref.at[b], sem_k + b)
    cp_v = lambda b: copy(v_hbm.at[b], v_ref.at[b], sem_v + b)
    cp_o = lambda b: copy(o_ref.at[b], o_hbm.at[b], sem_o + b)
    cp_s = lambda i: copy(ssmk_hbm.at[i], ssmk_ref.at[i], sem_s + i)
    cp_m = lambda i: copy(wmod_hbm.at[:, lanes(i, D)], wmod_ref.at[i], sem_m + i)
    cp_g = lambda i: copy(wg_hbm.at[:, lanes(i, FF // WCH)], wg_ref.at[i], sem_g + i)
    cp_u = lambda i: copy(wu_hbm.at[:, lanes(i, FF // WCH)], wu_ref.at[i], sem_u + i)
    cp_d = lambda i: copy(wd_hbm.at[:, lanes(i)], wd_ref.at[:, lanes(i)], sem_d + i)
    cp_l = lambda i: copy(o_ref.at[NB - 1, :, lanes(i)], o_hbm.at[NB - 1, :, lanes(i)], sem_l + i)
    cp_x = lambda i: copy((f_hbm, dd_hbm, sk_hbm, g_hbm, c_hbm)[i],
                          (f_ref, dd_ref, sk_ref, g_ref, c_ref)[i], sem_x + i)

    def dft_k(lt, j):
        kf = lax.dot_general(_unpack(f_ref[...]), ssmk_ref[lt, :, j * CH:(j + 1) * CH],
                             (((1,), (1,)), ((), ())), preferred_element_type=F32)
        slot = lt * NCH + j
        for p in range(NP):
            kr = kf[16 * p:16 * p + 8]
            ki = kf[16 * p + 8:16 * p + 16]
            if j == 0:
                kr = kr + ddf_ref[lt]
            kh_ref[slot, 24 * p:24 * p + 8, :] = kr
            kh_ref[slot, 24 * p + 8:24 * p + 16, :] = ki - kr
            kh_ref[slot, 24 * p + 16:24 * p + 24, :] = kr + ki

    def dft_u(b, lt, maybe_first=False):
        cs = lanes(lt)
        sk = sk_ref[:, cs].astype(F32)
        k = k_ref[b, :, cs].astype(F32)
        if maybe_first:
            halo = k_ref[jnp.maximum(b - 1, 0), TM - 8:TM, cs].astype(F32)
            halo = jnp.where(b > 0, halo, 0.0)
        else:
            halo = k_ref[b - 1, TM - 8:TM, cs].astype(F32)
        kext = jnp.concatenate([halo, k], axis=0)
        ks = k * sk[0:1, :]
        for t in range(1, 4):
            ks = ks + kext[8 - t:8 - t + TM, :] * sk[t:t + 1, :]
        kv = ks * v_ref[b, :, cs].astype(F32)
        for cc in range(2):
            uf = _dot(_unpack(f_ref[...]), kv[cc * CH:(cc + 1) * CH, :].astype(BF16))
            slot = lt * USL + UPAD + 2 * b + cc
            for p in range(NP):
                ur = uf[16 * p:16 * p + 8]
                ui = uf[16 * p + 8:16 * p + 16]
                uh_ref[slot, 24 * p:24 * p + 8, :] = ur + ui
                uh_ref[slot, 24 * p + 8:24 * p + 16, :] = ur
                uh_ref[slot, 24 * p + 16:24 * p + 24, :] = ui

    def mac(b, njs, lt, paced):
        uw = uh_ref.at[pl.ds(lt * USL + UPAD + 2 * b + 2 - njs, njs)]
        for p in range(NP):
            base = {}
            for q in range(3):
                rr = pl.ds(24 * p + 8 * q, 8)
                acc = {}
                for o in 'ac':
                    if q == 1:
                        acc[o] = base[o]
                    elif q == 2:
                        acc[o] = link(o, base[o])
                kprev = None
                for t in range(njs):
                    u = uw[njs - 1 - t, rr, :]
                    k = kh_ref[lt * NCH + t, rr, :]
                    for o, kk in (('c', k), ('a', kprev)):
                        if kk is None:
                            continue
                        m = kk * u
                        if o not in acc:
                            acc[o] = link(o, m)
                        else:
                            acc[o] = acc[o] - m if q == 2 else acc[o] + m
                    kprev = k
                if q == 0:
                    base = acc
                else:
                    r0 = 16 * p + (8 if q == 1 else 0)
                    z_ref[2 * lt, r0:r0 + 8, :] = acc['a']
                    z_ref[2 * lt + 1, r0:r0 + 8, :] = acc['c']
                    if paced:
                        chain.update(acc)

    def inv(lt, first=False, ys=0):
        za, zb = [], []
        for p in range(NP):
            re, im = slice(16 * p, 16 * p + 8), slice(16 * p + 8, 16 * p + 16)
            ar, ai = z_ref[2 * lt, re, :], z_ref[2 * lt, im, :]
            br, bi = z_ref[2 * lt + 1, re, :], z_ref[2 * lt + 1, im, :]
            if first:
                za += [ar, ai]
            else:
                pr, pi = zprev_ref[lt, re, :], zprev_ref[lt, im, :]
                za += [ar + pi, ai - pr] if p < NP // 2 else [ar - pi, ai + pr]
            zb += [br + ai, bi - ar] if p < NP // 2 else [br - ai, bi + ar]
            zprev_ref[lt, re, :] = br
            zprev_ref[lt, im, :] = bi
        for cc, z in enumerate((za, zb)):
            y_ref[z1 + ys, cc * CH:(cc + 1) * CH, lanes(lt)] = _dot(
                _unpack(g_ref[...]), jnp.concatenate(z, axis=0).astype(BF16))

    def norm(x, name=None):
        m = jnp.sum(x, axis=-1, keepdims=True) * (1.0 / D)
        if name is not None:
            m = link(name, m, never_col)
        xc = x - m
        v = jnp.sum(xc * xc, axis=-1, keepdims=True) * (1.0 / D)
        return xc * lax.rsqrt(v + EPS)

    def modrow(i):
        return mod_ref[i, 0:1, :]

    blk = {}

    def set_blocks(bf, bl):
        if isinstance(bf, int):
            blk.update(xf=x1_ref.at[bf], hf=h2_ref.at[bf], xl=x1_ref.at[bl], hl=h2_ref.at[bl])
        else:
            xw, hw = x1_ref.at[pl.ds(bf, 2)], h2_ref.at[pl.ds(bf, 2)]
            blk.update(xf=xw.at[0], hf=hw.at[0], xl=xw.at[1], hl=hw.at[1])

    def ln_piece(b, r, paced, part=3, ys=0):
        name = 'ln%d' % (r % LN_CHAINS) if paced else None
        rs = slice(r * RC, (r + 1) * RC)
        if part & 1:
            x = q_ref[b, rs, :].astype(F32)
            h1 = norm(x, name) * modrow(1) + modrow(0)
            x1 = x + h1 * y_ref[z2 + ys, rs, :]
            blk['xl'][rs, :] = x1
            n2 = norm(x1)
            if part == 1:
                x1_ref[NB - 1 - b, rs, :] = n2
        else:
            n2 = x1_ref[NB - 1 - b, rs, :]
        if part & 2:
            h2 = n2 * modrow(4) + modrow(3)
            if paced:
                chain[name] = h2[:, 0:1]
            blk['hl'][r * RC // 2:(r + 1) * RC // 2, :] = _pack(h2)

    def mod_part(i):
        c = c_ref[...].astype(F32)
        sc = jnp.broadcast_to((c * jax.nn.sigmoid(c)).astype(BF16), (8, D))
        return _dot(sc, wmod_ref[i])

    def weight(raw, packed_ref, c, n, first):
        rows = span(c, n, 32)
        if not first:
            return _unpack(packed_ref[rows, :])
        w = raw()
        packed_ref[rows, :] = pltpu.bitcast(w, U32)
        return w

    def gate_up(cp, cj, first=False, start_ln=False):
        c = 2 * cp + cj
        h2 = _unpack(blk['hf'][...])
        gate = _dot(h2, weight(lambda: wg_ref[cp, :, lanes(cj)], wgp_ref, c, D // 2, first))
        up = _dot(h2, weight(lambda: wu_ref[cp, :, lanes(cj)], wup_ref, c, D // 2, first))
        act_ref[span(cp, TM // 2, 32), lanes(cj)] = _pack(jnp.maximum(gate, 0.0) * up)
        if start_ln:
            for i in range(LN_CHAINS):
                chain['ln%d' % i] = up[0:RC, 0:1]

    def down(b, c, first=False):
        cs = lanes(c)
        a = jnp.concatenate([act_ref[span(j, TM // 2, 32), :] for j in range(NFT // 2)], axis=1)
        ff = _dot(_unpack(a), weight(lambda: wd_ref[:, cs], wdp_ref, c, FF // 2, first))
        o_ref[b, :, cs] = (blk['xf'][:, cs] + mod_ref[5, 0:1, cs] * ff).astype(BF16)

    def loop(lo, hi, body):
        def wrapped(i, carry):
            body(i)
            return carry
        lax.fori_loop(lo, hi, wrapped, 0)

    def prologue():
        for i in range(5):
            cp_x(i).start()
        for lt in range(NLT):
            cp_s(lt).start()
        for b in range(3):
            cp_k(b).start()
            cp_v(b).start()
        cp_q(0).start()
        cp_q(1).start()
        for i in range(5):
            cp_m(i).start()
        for i in range(WCH):
            cp_g(i).start()
            cp_u(i).start()
        cp_m(5).start()
        for i in range(3):
            cp_d(i).start()
        cp_k(3).start()
        cp_v(3).start()
        for i in range(3, NLT):
            cp_d(i).start()
        for b in range(2, NB):
            cp_q(b).start(priority=1)
            if b + 2 < NB:
                cp_k(b + 2).start(priority=1)
                cp_v(b + 2).start(priority=1)

        def zero_fill(j):
            for lt in range(NLT):
                uh_ref[lt * USL + j, 0:3 * CH, :] = jnp.zeros((3 * CH, 128), F32)
        loop(0, UPAD, zero_fill)
        for i in range(5):
            cp_x(i).wait()
        dd = dd_ref[...].astype(F32)
        for lt in range(NLT):
            ddf_ref[lt] = jnp.broadcast_to(dd[lt:lt + 1, :], (8, 128))

        def filter_spectra(lt):
            cp_s(lt).wait()
            for j in range(NCH):
                dft_k(lt, j)
        loop(0, NLT, filter_spectra)

        def input_spectra(b):
            cp_k(b).wait()
            cp_v(b).wait()
            for lt in range(NLT):
                dft_u(b, lt, True)
        loop(0, 3, input_spectra)

        def conv01(lt):
            mac(0, 2, lt, False)
            inv(lt, first=True)
            mac(1, 4, lt, False)
            inv(lt, ys=1)
        loop(0, NLT, conv01)

        def modulation(i):
            cp_m(i).wait()
            mod_ref[i] = mod_part(i)

        def ln01(part):
            def body(b):
                blk.update(xl=x1_ref.at[b], hl=h2_ref.at[b])
                for r in range(TM // RC):
                    ln_piece(b, r, False, part, b)
            loop(0, 2, body)
        loop(0, 3, modulation)
        ga = mod_ref[2]
        mod_ref[0] = mod_ref[0] * ga
        mod_ref[1] = (1.0 + mod_ref[1]) * ga
        cp_q(0).wait()
        cp_q(1).wait()
        ln01(1)
        loop(3, 5, modulation)
        mod_ref[4] = 1.0 + mod_ref[4]
        ln01(2)

    def first_step():
        set_blocks(0, 1)

        def chunk(i):
            cp_g(i).wait()
            cp_u(i).wait()
            chain.clear()
            gate_up(i, 0, first=True)
            gate_up(i, 1, first=True)
            mac(2, 6, jnp.minimum(i, NLT - 1), True)
        loop(0, WCH, chunk)
        cp_m(5).wait()
        cp_d(0).wait()
        mod_ref[5] = mod_part(5)
        down(0, 0, first=True)
        for c in range(1, NLT):
            if c == 3:
                cp_k(3).wait()
                cp_v(3).wait()
            cp_d(c).wait()
            down(0, c, first=True)
            for lt in {3: (0, 1, 2, 3), 4: (4,)}.get(c, ()):
                dft_u(3, lt)
        cp_o(0).start()

    def step(b, do_dft, do_mac, do_ln, ln_after):
        chain.clear()
        set_blocks(b, b + 1 if do_ln else b)
        for c in range(NFT):
            if do_ln and 1 <= c <= NLT:
                inv(c - 1)
                if do_mac:
                    mac(b + 2, NCH - 2 if do_dft else NCH, c - 1, True)
            gate_up(c // 2, c % 2, start_ln=(c == ln_after))
        for c in range(NLT):
            if do_dft:
                dft_u(b + 3, c)
            down(b, c)
            if not do_ln:
                cp_l(c).start()
        if do_ln:
            for r in range(TM // RC):
                ln_piece(b + 1, r, True)
            cp_o(b).start()

    def tail():
        step(NB - 3, False, True, True, 10)
        step(NB - 2, False, False, True, 6)
        step(NB - 1, False, False, False, -1)
        for b in range(NB - 1):
            cp_o(b).wait()
        for c in range(NLT):
            cp_l(c).wait()

    pl.when(g == 0)(prologue)

    @pl.when(jnp.logical_and(g >= 2, g + 2 < NB))
    def _():
        cp_k(g + 2).wait()
        cp_v(g + 2).wait()

    @pl.when(g >= 2)
    def _():
        cp_q(g).wait()

    @pl.when(g == NB - 2)
    def _():
        cp_q(NB - 1).wait()

    pl.when(g == 1)(first_step)
    pl.when(jnp.logical_and(g >= 2, g <= NB - 3))(lambda: step(g - 1, True, True, True, 9))
    pl.when(g == NB - 2)(tail)


@jax.jit
def pallas_adaLN_cond__ssm_conv_h3__glu_gated_reglu__prompt_kernel(
    A_q, A_k, A_v, A_shift_k, A_ssm_k, A_ssm_D, B_x, B_W_gate, B_W_up, B_W_down, c, w_mod,
):
    del B_x
    fwd, inv = _dft_tables()
    hbm = pl.BlockSpec(memory_space=pl.ANY)
    out = pl.pallas_call(
        _kernel,
        grid=(NB - 1,),
        in_specs=[hbm] * 13,
        out_specs=hbm,
        out_shape=jax.ShapeDtypeStruct((NB, TM, D), BF16),
        scratch_shapes=[
            pltpu.VMEM((NB, TM, D), BF16),
            pltpu.VMEM((NB, TM, D), BF16),
            pltpu.VMEM((NB, TM, D), BF16),
            pltpu.VMEM((NB, TM, D), BF16),
            pltpu.VMEM((NLT, 128, S), BF16),
            pltpu.VMEM((WCH, D, FF // WCH), BF16),
            pltpu.VMEM((WCH, D, FF // WCH), BF16),
            pltpu.VMEM((FF, D), BF16),
            pltpu.VMEM((6, D, D), BF16),
            pltpu.SemaphoreType.DMA((70,)),
            pltpu.VMEM((8, 8, D), F32),
            pltpu.VMEM((NLT, 2 * CH, 128), F32),
            pltpu.VMEM((2 * NLT, 2 * CH, 128), F32),
            pltpu.VMEM((NB, TM // 2, D), U32),
            pltpu.VMEM((NB, TM, D), F32),
            pltpu.VMEM((NFT // 2 * TM // 2, 256), U32),
            pltpu.VMEM((2, TM, D), F32),
            pltpu.VMEM((NFT * D // 2, 128), U32),
            pltpu.VMEM((NFT * D // 2, 128), U32),
            pltpu.VMEM((NLT * FF // 2, 128), U32),
            pltpu.VMEM((NLT * NCH, KROWS, 128), F32),
            pltpu.VMEM((NLT * USL, UROWS, 128), F32),
            pltpu.VMEM((CH, CH), U32),
            pltpu.VMEM((CH // 2, 2 * CH), U32),
            pltpu.VMEM((8, 8, 128), F32),
            pltpu.VMEM((4, D), BF16),
            pltpu.VMEM((NLT, 128), BF16),
            pltpu.VMEM((1, D), BF16),
        ],
        compiler_params=pltpu.CompilerParams(
            dimension_semantics=("arbitrary",),
            vmem_limit_bytes=110 * 1024 * 1024,
            disable_bounds_checks=True,
            disable_semaphore_checks=True),
    )(A_q.reshape(NB, TM, D), A_k.reshape(NB, TM, D), A_v.reshape(NB, TM, D), A_shift_k.T,
      A_ssm_k.reshape(NLT, 128, S), A_ssm_D.reshape(NLT, 128), B_W_gate, B_W_up, B_W_down,
      c, w_mod, jnp.asarray(_pack_np(fwd)), jnp.asarray(_pack_np(inv)))
    return out.reshape(1, S, D)
```

```python
import numpy as np
import jax
import jax.numpy as jnp
from jax import lax
import jax.experimental.pallas as pl
import jax.experimental.pallas.tpu as pltpu

S = 2048
D = 640
FF = 1536
CH = 128
NCH = S // CH
TM = 256
NB = S // TM
NLT = D // 128
NFT = FF // 128
NP = CH // 8
EPS = 1e-5
UPAD = NCH - 10
USL = UPAD + NCH
KROWS = 3 * CH + 8
UROWS = 3 * CH + 64
WCH = 6
RC = 16
LN_CHAINS = 2
PACE_STEADY = dict(mac=(1, 1, 1, 0, 1, 1, 1, 1), s1=(1, 2), s2=(1, 1))
PACE_LAST_MAC = dict(mac=(1,), s1=(1,), s2=(0, 1))
PACE_LAST_LN = dict(s2=(1, 1))
DFT_BEFORE = (1, 2, 3, 4, 16)
F32 = jnp.float32
BF16 = jnp.bfloat16
U32 = jnp.uint32


def _dft_tables():
    h, m2, sl = np.meshgrid(np.arange(2), np.arange(8), np.arange(8), indexing='ij')
    m = (8 * h + sl + 16 * m2).reshape(NP, 8)
    k = ((4 * m[:, :, None] + 1) * np.arange(CH)) % (4 * CH)
    ang = np.pi * k / (2 * CH)
    fwd = np.stack([np.cos(ang), np.sin(ang)], axis=1).reshape(2 * CH, CH)
    m1 = 8 * np.arange(2)[:, None, None] + np.arange(8)[None, None, :]
    n2 = np.arange(8)[None, :, None]
    tw = np.exp(-1j * np.pi * (4 * m1 + 1) * n2 / (2 * CH))
    tw = np.stack([tw.real, tw.imag], axis=2).reshape(32, 8).T
    tw = np.concatenate([tw, np.zeros((8, 96))], axis=1)
    return fwd, fwd.T, tw.astype(np.float32)


def _cmul(x, k, n):
    re, im = x
    k = k % n
    if k == 0:
        return x
    if 4 * k == n:
        return im, -re
    c, s = np.cos(2 * np.pi * k / n), np.sin(2 * np.pi * k / n)
    if (8 * k) % n == 0:
        if c * s > 0:
            return (re + im) * c, (im - re) * c
        return (im - re) * s, (re + im) * -s
    return re * c + im * s, im * c - re * s


def _fft(xs):
    n = len(xs)
    if n == 1:
        return xs
    ev, od = _fft(xs[0::2]), _fft(xs[1::2])
    out = [None] * n
    for k in range(n // 2):
        (er, ei) = ev[k]
        if 4 * k == n:
            (tr, ti) = od[k]
            out[k] = (er + ti, ei - tr)
            out[k + n // 2] = (er - ti, ei + tr)
        else:
            tr, ti = _cmul(od[k], k, n)
            out[k] = (er + tr, ei + ti)
            out[k + n // 2] = (er - tr, ei - ti)
    return out


def _re_rot(x, ang):
    c, s = np.cos(ang), np.sin(ang)
    if abs(s) < 1e-12:
        return x[0] if c > 0 else -x[0]
    if abs(c) < 1e-12:
        return x[1] if s > 0 else -x[1]
    return x[0] * c + x[1] * s


def _pack_np(a):
    u = np.ascontiguousarray(a, np.float32).view(np.uint32)
    b = ((u + 0x7FFF + ((u >> 16) & 1)) >> 16).astype(np.uint32)
    return b[0::2] | (b[1::2] << 16)


def _pack(x):
    return pltpu.bitcast(x.astype(BF16), U32)


def _unpack(x):
    return pltpu.bitcast(x, BF16)


def _dot(a, b):
    return jnp.dot(a, b, preferred_element_type=F32)


def _kernel(q_hbm, k_hbm, v_hbm, sk_hbm, ssmk_hbm, dd_hbm, wg_hbm, wu_hbm, wd_hbm,
            c_hbm, wmod_hbm, f_hbm, g_hbm, tw_hbm, o_hbm,
            q_ref, k_ref, v_ref, o_ref, ssmk_ref, wg_ref, wu_ref, wd_ref, wmod_ref, sems,
            mod_ref, zprev_ref, z_ref, h2_ref, x1_ref, act_ref, y_ref,
            wgp_ref, wup_ref, wdp_ref, kh_ref, uh_ref, tb_ref, twb_ref,
            f_ref, g_ref, ddf_ref, tw_ref, sk_ref, dd_ref, c_ref):
    g = pl.program_id(0)
    never8 = lax.broadcasted_iota(jnp.int32, (8, 128), 0) < g - 1000
    never_col = lax.broadcasted_iota(jnp.int32, (RC, 1), 0) < g - 1000
    z1 = lax.shift_right_logical(g, 10)
    z2 = lax.shift_right_logical(g, 11)
    chain = {}
    cfg = dict(PACE_STEADY)

    def link(name, m, mask=never8):
        prev = chain.get(name)
        return m if prev is None else jnp.where(mask, prev, m)

    def pace(name, v, n):
        for _ in range(n):
            v = pltpu.roll(v, 1, 1)
        chain[name] = v

    def span(i, w, align):
        if isinstance(i, int):
            return pl.ds(i * w, w)
        return pl.ds(pl.multiple_of(i * w, align), w)

    def lanes(i, w=128):
        return span(i, w, 128)

    sem_q, sem_k, sem_v, sem_o, sem_s, sem_m, sem_g, sem_u, sem_d, sem_l, sem_x = (
        0, 8, 16, 24, 32, 37, 43, 49, 55, 60, 65)

    def copy(src, dst, sem):
        return pltpu.make_async_copy(src, dst, sems.at[sem])

    cp_q = lambda b: copy(q_hbm.at[b], q_ref.at[b], sem_q + b)
    cp_k = lambda b: copy(k_hbm.at[b], k_ref.at[b], sem_k + b)
    cp_v = lambda b: copy(v_hbm.at[b], v_ref.at[b], sem_v + b)
    cp_o = lambda b: copy(o_ref.at[b], o_hbm.at[b], sem_o + b)
    cp_s = lambda i: copy(ssmk_hbm.at[i], ssmk_ref.at[i], sem_s + i)
    cp_m = lambda i: copy(wmod_hbm.at[:, lanes(i, D)], wmod_ref.at[i], sem_m + i)
    cp_g = lambda i: copy(wg_hbm.at[:, lanes(i, FF // WCH)], wg_ref.at[i], sem_g + i)
    cp_u = lambda i: copy(wu_hbm.at[:, lanes(i, FF // WCH)], wu_ref.at[i], sem_u + i)
    cp_d = lambda i: copy(wd_hbm.at[:, lanes(i)], wd_ref.at[:, lanes(i)], sem_d + i)
    cp_l = lambda i: copy(o_ref.at[NB - 1, :, lanes(i)], o_hbm.at[NB - 1, :, lanes(i)], sem_l + i)
    cp_x = lambda i: copy((f_hbm, dd_hbm, sk_hbm, g_hbm, c_hbm, tw_hbm)[i],
                          (f_ref, dd_ref, sk_ref, g_ref, c_ref, tw_ref)[i], sem_x + i)

    def dft_k(lt, j):
        kf = lax.dot_general(_unpack(f_ref[...]), ssmk_ref[lt, :, j * CH:(j + 1) * CH],
                             (((1,), (1,)), ((), ())), preferred_element_type=F32)
        slot = lt * NCH + j
        for p in range(NP):
            kr = kf[16 * p:16 * p + 8]
            ki = kf[16 * p + 8:16 * p + 16]
            if j == 0:
                kr = kr + ddf_ref[lt]
            kr, ki = kr * (1.0 / CH), ki * (1.0 / CH)
            kh_ref[slot, 24 * p:24 * p + 8, :] = kr
            kh_ref[slot, 24 * p + 8:24 * p + 16, :] = ki - kr
            kh_ref[slot, 24 * p + 16:24 * p + 24, :] = kr + ki

    def dft_u(b, lt, maybe_first=False):
        cs = lanes(lt)
        sk = sk_ref[:, cs].astype(F32)
        k = k_ref[b, :, cs].astype(F32)
        if maybe_first:
            halo = k_ref[jnp.maximum(b - 1, 0), TM - 8:TM, cs].astype(F32)
            halo = jnp.where(b > 0, halo, 0.0)
        else:
            halo = k_ref[b - 1, TM - 8:TM, cs].astype(F32)
        kext = jnp.concatenate([halo, k], axis=0)
        ks = k * sk[0:1, :]
        for t in range(1, 4):
            ks = ks + kext[8 - t:8 - t + TM, :] * sk[t:t + 1, :]
        kv = ks * v_ref[b, :, cs].astype(F32)
        for cc in range(2):
            uf = _dot(_unpack(f_ref[...]), kv[cc * CH:(cc + 1) * CH, :].astype(BF16))
            slot = lt * USL + UPAD + 2 * b + cc
            for p in range(NP):
                ur = uf[16 * p:16 * p + 8]
                ui = uf[16 * p + 8:16 * p + 16]
                uh_ref[slot, 24 * p:24 * p + 8, :] = ur + ui
                uh_ref[slot, 24 * p + 8:24 * p + 16, :] = ur
                uh_ref[slot, 24 * p + 16:24 * p + 24, :] = ui

    def mac(b, njs, lt, chained, paced=False):
        uw = uh_ref.at[pl.ds(lt * USL + UPAD + 2 * b + 2 - njs, njs)]
        for p in range(NP):
            base = {}
            for q in range(3):
                rr = pl.ds(24 * p + 8 * q, 8)
                acc = {}
                for o in 'ac':
                    if q == 1:
                        acc[o] = base[o]
                    elif q == 2:
                        acc[o] = link(o, base[o])
                kprev = None
                for t in range(njs):
                    u = uw[njs - 1 - t, rr, :]
                    k = kh_ref[lt * NCH + t, rr, :]
                    for o, kk in (('c', k), ('a', kprev)):
                        if kk is None:
                            continue
                        m = kk * u
                        if o not in acc:
                            acc[o] = link(o, m)
                        else:
                            acc[o] = acc[o] - m if q == 2 else acc[o] + m
                    kprev = k
                if q == 0:
                    base = acc
                else:
                    r0 = 16 * p + (8 if q == 1 else 0)
                    z_ref[2 * lt, r0:r0 + 8, :] = acc['a']
                    z_ref[2 * lt + 1, r0:r0 + 8, :] = acc['c']
                    if chained and q == 1:
                        chain.update(acc)
                    if chained and q == 2:
                        chain.update(a=acc['c'], c=acc['a'])
                        n = cfg['mac'][p % len(cfg['mac'])]
                        if paced and n:
                            pace('s1', link('s1', acc['a'] + acc['c']), n)

    def overlap(lt, cc, first=False):
        z = []
        for p in range(NP):
            re, im = slice(16 * p, 16 * p + 8), slice(16 * p + 8, 16 * p + 16)
            zr, zi = z_ref[2 * lt + cc, re, :], z_ref[2 * lt + cc, im, :]
            if cc == 0 and first:
                z.append((zr, zi))
            else:
                prev = zprev_ref.at[lt] if cc == 0 else z_ref.at[2 * lt]
                z.append((zr + prev[im, :], zi - prev[re, :]))
            if cc == 1:
                zprev_ref[lt, re, :] = zr
                zprev_ref[lt, im, :] = zi
        return z

    def inv(lt, first=False, ys=0):
        for cc in range(2):
            z = jnp.concatenate([t for pair in overlap(lt, cc, first) for t in pair], axis=0)
            y_ref[z1 + ys, cc * CH:(cc + 1) * CH, lanes(lt)] = _dot(_unpack(g_ref[...]), z.astype(BF16))

    def inv_vpu1(u, paced=True):
        lt, cc = u // 2, u % 2
        z = overlap(lt, cc)
        for h in range(2):
            zz = z[8 * h:8 * h + 8]
            if paced:
                zz[0] = (link('s1', zz[0][0]), zz[0][1])
            for n2, (re, im) in enumerate(_fft(zz)):
                if n2 > 0:
                    tr, ti = twb_ref[(h * 8 + n2) * 2], twb_ref[(h * 8 + n2) * 2 + 1]
                    re, im = re * tr - im * ti, re * ti + im * tr
                tb_ref[u, 144 * h + 9 * n2:144 * h + 9 * n2 + 8, :] = re
                tb_ref[u, 144 * h + 72 + 9 * n2:144 * h + 72 + 9 * n2 + 8, :] = im
            if paced:
                pace('s1', re, cfg['s1'][h % len(cfg['s1'])])

    def inv_vpu2(u):
        lt, cc = u // 2, u % 2
        ld = lambda o, sl: tb_ref[u, pl.ds(o + sl, 8, stride=9), :]
        xs = [(ld(144 * h, sl), ld(144 * h + 72, sl)) for h in range(2) for sl in range(8)]
        xe, xo = xs[0::2], xs[1::2]
        xe[0] = (link('s2', xe[0][0]), xe[0][1])
        ev = _fft(xe)
        ye = [_re_rot(ev[n1 % 8], np.pi * n1 / 32) for n1 in range(16)]
        pace('s2', ye[-1], cfg['s2'][0])
        xo[0] = (link('s2', xo[0][0]), xo[0][1])
        od = _fft(xo)
        for n1 in range(16):
            y = ye[n1] + _re_rot(od[n1 % 8], np.pi * n1 / 32 + 2 * np.pi * n1 / 16)
            y_ref[z1, cc * CH + 8 * n1:cc * CH + 8 * n1 + 8, lanes(lt)] = y
        pace('s2', y, cfg['s2'][1])

    def norm(x, name=None):
        m = jnp.sum(x, axis=-1, keepdims=True) * (1.0 / D)
        if name is not None:
            m = link(name, m, never_col)
        xc = x - m
        v = jnp.sum(xc * xc, axis=-1, keepdims=True) * (1.0 / D)
        return xc * lax.rsqrt(v + EPS)

    def modrow(i):
        return mod_ref[i, 0:1, :]

    blk = {}

    def set_blocks(bf, bl):
        if isinstance(bf, int):
            blk.update(xf=x1_ref.at[bf], hf=h2_ref.at[bf], xl=x1_ref.at[bl], hl=h2_ref.at[bl])
        else:
            xw, hw = x1_ref.at[pl.ds(bf, 2)], h2_ref.at[pl.ds(bf, 2)]
            blk.update(xf=xw.at[0], hf=hw.at[0], xl=xw.at[1], hl=hw.at[1])

    def ln_piece(b, r, paced, part=3, ys=0):
        name = 'ln%d' % (r % LN_CHAINS) if paced else None
        rs = slice(r * RC, (r + 1) * RC)
        if part & 1:
            x = q_ref[b, rs, :].astype(F32)
            h1 = norm(x, name) * modrow(1) + modrow(0)
            x1 = x + h1 * y_ref[z2 + ys, rs, :]
            blk['xl'][rs, :] = x1
            n2 = norm(x1)
            if part == 1:
                x1_ref[NB - 1 - b, rs, :] = n2
        else:
            n2 = x1_ref[NB - 1 - b, rs, :]
        if part & 2:
            h2 = n2 * modrow(4) + modrow(3)
            if paced:
                chain[name] = h2[:, 0:1]
            blk['hl'][r * RC // 2:(r + 1) * RC // 2, :] = _pack(h2)

    def mod_part(i):
        c = c_ref[...].astype(F32)
        sc = jnp.broadcast_to((c * jax.nn.sigmoid(c)).astype(BF16), (8, D))
        return _dot(sc, wmod_ref[i])

    def weight(raw, packed_ref, c, n, first):
        rows = span(c, n, 32)
        if not first:
            return _unpack(packed_ref[rows, :])
        w = raw()
        packed_ref[rows, :] = pltpu.bitcast(w, U32)
        return w

    def gate_up(cp, cj, first=False):
        c = 2 * cp + cj
        h2 = _unpack(blk['hf'][...])
        gate = _dot(h2, weight(lambda: wg_ref[cp, :, lanes(cj)], wgp_ref, c, D // 2, first))
        up = _dot(h2, weight(lambda: wu_ref[cp, :, lanes(cj)], wup_ref, c, D // 2, first))
        act_ref[span(cp, TM // 2, 32), lanes(cj)] = _pack(jnp.maximum(gate, 0.0) * up)

    def down(b, c, first=False):
        cs = lanes(c)
        a = jnp.concatenate([act_ref[span(j, TM // 2, 32), :] for j in range(NFT // 2)], axis=1)
        ff = _dot(_unpack(a), weight(lambda: wd_ref[:, cs], wdp_ref, c, FF // 2, first))
        o_ref[b, :, cs] = (blk['xf'][:, cs] + mod_ref[5, 0:1, cs] * ff).astype(BF16)

    def loop(lo, hi, body):
        def wrapped(i, carry):
            body(i)
            return carry
        lax.fori_loop(lo, hi, wrapped, 0)

    def prologue():
        for i in range(6):
            cp_x(i).start()
        for lt in range(NLT):
            cp_s(lt).start()
        for b in range(3):
            cp_k(b).start()
            cp_v(b).start()
        cp_q(0).start()
        cp_q(1).start()
        for i in range(5):
            cp_m(i).start()
        for i in range(WCH):
            cp_g(i).start()
            cp_u(i).start()
        cp_m(5).start()
        for i in range(3):
            cp_d(i).start()
        cp_k(3).start()
        cp_v(3).start()
        for i in range(3, NLT):
            cp_d(i).start()
        for b in range(2, NB):
            cp_q(b).start(priority=1)
            if b + 2 < NB:
                cp_k(b + 2).start(priority=1)
                cp_v(b + 2).start(priority=1)

        def zero_fill(j):
            for lt in range(NLT):
                uh_ref[lt * USL + j, 0:3 * CH, :] = jnp.zeros((3 * CH, 128), F32)
        loop(0, UPAD, zero_fill)
        for i in range(6):
            cp_x(i).wait()
        tw = tw_ref[...]
        for i in range(32):
            twb_ref[i] = jnp.broadcast_to(tw[:, i:i + 1], (8, 128))
        dd = dd_ref[...].astype(F32)
        for lt in range(NLT):
            ddf_ref[lt] = jnp.broadcast_to(dd[lt:lt + 1, :], (8, 128))

        def filter_spectra(lt):
            cp_s(lt).wait()
            for j in range(NCH):
                dft_k(lt, j)
        loop(0, NLT, filter_spectra)

        def input_spectra(b):
            cp_k(b).wait()
            cp_v(b).wait()
            for lt in range(NLT):
                dft_u(b, lt, True)
        loop(0, 3, input_spectra)

        def conv01(lt):
            mac(0, 2, lt, False)
            inv(lt, first=True)
            mac(1, 4, lt, False)
            inv(lt, ys=1)
        loop(0, NLT, conv01)

        def modulation(i):
            cp_m(i).wait()
            mod_ref[i] = mod_part(i)

        def ln01(part):
            def body(b):
                blk.update(xl=x1_ref.at[b], hl=h2_ref.at[b])
                for r in range(TM // RC):
                    ln_piece(b, r, False, part, b)
            loop(0, 2, body)
        loop(0, 3, modulation)
        ga = mod_ref[2]
        mod_ref[0] = mod_ref[0] * ga
        mod_ref[1] = (1.0 + mod_ref[1]) * ga
        cp_q(0).wait()
        cp_q(1).wait()
        ln01(1)
        loop(3, 5, modulation)
        mod_ref[4] = 1.0 + mod_ref[4]
        ln01(2)

    def first_step():
        set_blocks(0, 1)

        def chunk(i):
            cp_g(i).wait()
            cp_u(i).wait()
            chain.clear()
            gate_up(i, 0, first=True)
            gate_up(i, 1, first=True)
            mac(2, 6, jnp.minimum(i, NLT - 1), True)
        loop(0, WCH, chunk)
        chain.clear()
        cp_m(5).wait()
        cp_d(0).wait()
        mod_ref[5] = mod_part(5)
        down(0, 0, first=True)
        for c in range(1, NLT):
            if c == 3:
                cp_k(3).wait()
                cp_v(3).wait()
            cp_d(c).wait()
            down(0, c, first=True)
            for u in {1: range(0, 4), 2: range(4, 8), 3: range(8, 10)}.get(c, ()):
                inv_vpu1(u, False)
            for lt in {3: (0, 1, 2, 3), 4: (4,)}.get(c, ()):
                dft_u(3, lt)
        cp_o(0).start()

    def step(b, do_dft, do_mac, do_ln):
        chain.clear()
        set_blocks(b, b + 1 if do_ln else b)
        if do_ln:
            for u in range(2 * NLT):
                inv_vpu2(u)
        if do_mac:
            for lt in range(NLT):
                mac(b + 2, NCH - 2 if do_dft else NCH, lt, True, True)
            for u in range(2 * NLT):
                inv_vpu1(u)
        for c in range(NFT + NLT):
            for lt in range(NLT):
                if do_dft and DFT_BEFORE[lt] == c:
                    dft_u(b + 3, lt)
            if c < NFT:
                gate_up(c // 2, c % 2)
            else:
                down(b, c - NFT)
                if not do_ln:
                    cp_l(c - NFT).start()
        if do_ln:
            for r in range(TM // RC):
                ln_piece(b + 1, r, True)
            cp_o(b).start()

    def tail():
        cfg.update(PACE_LAST_MAC)
        step(NB - 3, False, True, True)
        cfg.update(PACE_LAST_LN)
        step(NB - 2, False, False, True)
        step(NB - 1, False, False, False)
        for b in range(NB - 1):
            cp_o(b).wait()
        for c in range(NLT):
            cp_l(c).wait()

    pl.when(g == 0)(prologue)

    @pl.when(jnp.logical_and(g >= 2, g + 2 < NB))
    def _():
        cp_k(g + 2).wait()
        cp_v(g + 2).wait()

    @pl.when(g >= 2)
    def _():
        cp_q(g).wait()

    @pl.when(g == NB - 2)
    def _():
        cp_q(NB - 1).wait()

    pl.when(g == 1)(first_step)
    pl.when(jnp.logical_and(g >= 2, g <= NB - 3))(lambda: step(g - 1, True, True, True))
    pl.when(g == NB - 2)(tail)


@jax.jit
def pallas_adaLN_cond__ssm_conv_h3__glu_gated_reglu__prompt_kernel(
    A_q, A_k, A_v, A_shift_k, A_ssm_k, A_ssm_D, B_x, B_W_gate, B_W_up, B_W_down, c, w_mod,
):
    del B_x
    fwd, inv, tw = _dft_tables()
    hbm = pl.BlockSpec(memory_space=pl.ANY)
    out = pl.pallas_call(
        _kernel,
        grid=(NB - 1,),
        in_specs=[hbm] * 14,
        out_specs=hbm,
        out_shape=jax.ShapeDtypeStruct((NB, TM, D), BF16),
        scratch_shapes=[
            pltpu.VMEM((NB, TM, D), BF16),
            pltpu.VMEM((NB, TM, D), BF16),
            pltpu.VMEM((NB, TM, D), BF16),
            pltpu.VMEM((NB, TM, D), BF16),
            pltpu.VMEM((NLT, 128, S), BF16),
            pltpu.VMEM((WCH, D, FF // WCH), BF16),
            pltpu.VMEM((WCH, D, FF // WCH), BF16),
            pltpu.VMEM((FF, D), BF16),
            pltpu.VMEM((6, D, D), BF16),
            pltpu.SemaphoreType.DMA((71,)),
            pltpu.VMEM((8, 8, D), F32),
            pltpu.VMEM((NLT, 2 * CH, 128), F32),
            pltpu.VMEM((2 * NLT, 2 * CH, 128), F32),
            pltpu.VMEM((NB, TM // 2, D), U32),
            pltpu.VMEM((NB, TM, D), F32),
            pltpu.VMEM((NFT // 2 * TM // 2, 256), U32),
            pltpu.VMEM((2, TM, D), F32),
            pltpu.VMEM((NFT * D // 2, 128), U32),
            pltpu.VMEM((NFT * D // 2, 128), U32),
            pltpu.VMEM((NLT * FF // 2, 128), U32),
            pltpu.VMEM((NLT * NCH, KROWS, 128), F32),
            pltpu.VMEM((NLT * USL, UROWS, 128), F32),
            pltpu.VMEM((2 * NLT, 288, 128), F32),
            pltpu.VMEM((32, 8, 128), F32),
            pltpu.VMEM((CH, CH), U32),
            pltpu.VMEM((CH // 2, 2 * CH), U32),
            pltpu.VMEM((8, 8, 128), F32),
            pltpu.VMEM((8, 128), F32),
            pltpu.VMEM((4, D), BF16),
            pltpu.VMEM((NLT, 128), BF16),
            pltpu.VMEM((1, D), BF16),
        ],
        compiler_params=pltpu.CompilerParams(
            dimension_semantics=("arbitrary",),
            vmem_limit_bytes=110 * 1024 * 1024,
            disable_bounds_checks=True,
            disable_semaphore_checks=True),
    )(A_q.reshape(NB, TM, D), A_k.reshape(NB, TM, D), A_v.reshape(NB, TM, D), A_shift_k.T,
      A_ssm_k.reshape(NLT, 128, S), A_ssm_D.reshape(NLT, 128), B_W_gate, B_W_up, B_W_down,
      c, w_mod, jnp.asarray(_pack_np(fwd)), jnp.asarray(_pack_np(inv)), jnp.asarray(tw))
    return out.reshape(1, S, D)
```

```python
import numpy as np
import jax
import jax.numpy as jnp
from jax import lax
import jax.experimental.pallas as pl
import jax.experimental.pallas.tpu as pltpu

S = 2048
D = 640
FF = 1536
CH = 128
NCH = S // CH
TM = 256
NB = S // TM
NLT = D // 128
NFT = FF // 128
NP = CH // 8
EPS = 1e-5
UPAD = NCH - 10
USL = UPAD + NCH
KROWS = 3 * CH + 8
UROWS = 3 * CH + 64
TBR = 320
WCH = 6
RC = 16
LN_CHAINS = 2
PACE_STEADY = dict(mac=(1, 1, 1, 0, 1, 1, 1, 1), s1=(1, 2), s2=(1, 1))
PACE_LAST_MAC = dict(mac=(1,), s1=(1,), s2=(0, 1))
PACE_LAST_LN = dict(s2=(1, 1))
DFT_BEFORE = (1, 2, 3, 4, 16)
F32 = jnp.float32
BF16 = jnp.bfloat16
U32 = jnp.uint32


def _dft_tables():
    h, m2, sl = np.meshgrid(np.arange(2), np.arange(8), np.arange(8), indexing='ij')
    m = (8 * h + sl + 16 * m2).reshape(NP, 8)
    k = ((4 * m[:, :, None] + 1) * np.arange(CH)) % (4 * CH)
    ang = np.pi * k / (2 * CH)
    fwd = np.stack([np.cos(ang), np.sin(ang)], axis=1).reshape(2 * CH, CH)
    m1 = 8 * np.arange(2)[:, None, None] + np.arange(8)[None, None, :]
    n2 = np.arange(8)[None, :, None]
    tw = np.exp(-1j * np.pi * (4 * m1 + 1) * n2 / (2 * CH))
    tw = np.stack([tw.real, tw.imag], axis=2).reshape(32, 8).T
    tw = np.concatenate([tw, np.zeros((8, 96))], axis=1)
    return fwd, fwd.T, tw.astype(np.float32)


def _cmul(x, k, n):
    re, im = x
    k = k % n
    if k == 0:
        return x
    if 4 * k == n:
        return im, -re
    c, s = float(np.cos(2 * np.pi * k / n)), float(np.sin(2 * np.pi * k / n))
    if (8 * k) % n == 0:
        if c * s > 0:
            return (re + im) * c, (im - re) * c
        return (im - re) * s, (re + im) * -s
    return re * c + im * s, im * c - re * s


def _fft(xs):
    n = len(xs)
    if n == 1:
        return xs
    ev, od = _fft(xs[0::2]), _fft(xs[1::2])
    out = [None] * n
    for k in range(n // 2):
        (er, ei) = ev[k]
        if 4 * k == n:
            (tr, ti) = od[k]
            out[k] = (er + ti, ei - tr)
            out[k + n // 2] = (er - ti, ei + tr)
        else:
            tr, ti = _cmul(od[k], k, n)
            out[k] = (er + tr, ei + ti)
            out[k + n // 2] = (er - tr, ei - ti)
    return out


def _re_rot(x, ang):
    c, s = float(np.cos(ang)), float(np.sin(ang))
    if abs(s) < 1e-12:
        return x[0] if c > 0 else -x[0]
    if abs(c) < 1e-12:
        return x[1] if s > 0 else -x[1]
    return x[0] * c + x[1] * s


def _pack_np(a):
    u = np.ascontiguousarray(a, np.float32).view(np.uint32)
    b = ((u + 0x7FFF + ((u >> 16) & 1)) >> 16).astype(np.uint32)
    return b[0::2] | (b[1::2] << 16)


def _pack(x):
    return pltpu.bitcast(x.astype(BF16), U32)


def _unpack(x):
    return pltpu.bitcast(x, BF16)


def _dot(a, b):
    return jnp.dot(a, b, preferred_element_type=F32)


def _kernel(q_hbm, k_hbm, v_hbm, sk_hbm, ssmk_hbm, dd_hbm, wg_hbm, wu_hbm, wd_hbm,
            c_hbm, wmod_hbm, f_hbm, g_hbm, tw_hbm, o_hbm,
            q_ref, k_ref, v_ref, o_ref, ssmk_ref, wg_ref, wu_ref, wd_ref, wmod_ref, sems,
            mod_ref, zprev_ref, z_ref, h2_ref, x1_ref, act_ref, y_ref,
            wgp_ref, wup_ref, wdp_ref, kh_ref, uh_ref, tb_ref, twb_ref,
            f_ref, g_ref, ddf_ref, tw_ref, sk_ref, dd_ref, c_ref):
    g = pl.program_id(0)
    never8 = lax.broadcasted_iota(jnp.int32, (8, 128), 0) < g - 1000
    never_col = lax.broadcasted_iota(jnp.int32, (RC, 1), 0) < g - 1000
    z1 = lax.shift_right_logical(g, 10)
    z2 = lax.shift_right_logical(g, 11)
    chain = {}
    cfg = dict(PACE_STEADY)

    def link(name, m, mask=never8):
        prev = chain.get(name)
        return m if prev is None else jnp.where(mask, prev, m)

    def pace(name, v, n):
        for _ in range(n):
            v = pltpu.roll(v, 1, 1)
        chain[name] = v

    def span(i, w, align):
        if isinstance(i, int):
            return pl.ds(i * w, w)
        return pl.ds(pl.multiple_of(i * w, align), w)

    def lanes(i, w=128):
        return span(i, w, 128)

    sem_q, sem_k, sem_v, sem_o, sem_s, sem_m, sem_g, sem_u, sem_d, sem_l, sem_x = (
        0, 8, 16, 24, 32, 37, 43, 49, 55, 60, 65)

    def copy(src, dst, sem):
        return pltpu.make_async_copy(src, dst, sems.at[sem])

    cp_q = lambda b: copy(q_hbm.at[b], q_ref.at[b], sem_q + b)
    cp_k = lambda b: copy(k_hbm.at[b], k_ref.at[b], sem_k + b)
    cp_v = lambda b: copy(v_hbm.at[b], v_ref.at[b], sem_v + b)
    cp_o = lambda b: copy(o_ref.at[b], o_hbm.at[b], sem_o + b)
    cp_s = lambda i: copy(ssmk_hbm.at[i], ssmk_ref.at[i], sem_s + i)
    cp_m = lambda i: copy(wmod_hbm.at[:, lanes(i, D)], wmod_ref.at[i], sem_m + i)
    cp_g = lambda i: copy(wg_hbm.at[:, lanes(i, FF // WCH)], wg_ref.at[i], sem_g + i)
    cp_u = lambda i: copy(wu_hbm.at[:, lanes(i, FF // WCH)], wu_ref.at[i], sem_u + i)
    cp_d = lambda i: copy(wd_hbm.at[:, lanes(i)], wd_ref.at[:, lanes(i)], sem_d + i)
    cp_l = lambda i: copy(o_ref.at[NB - 1, :, lanes(i)], o_hbm.at[NB - 1, :, lanes(i)], sem_l + i)
    cp_x = lambda i: copy((f_hbm, dd_hbm, sk_hbm, g_hbm, c_hbm, tw_hbm)[i],
                          (f_ref, dd_ref, sk_ref, g_ref, c_ref, tw_ref)[i], sem_x + i)

    def dft_k(lt, j):
        kf = lax.dot_general(_unpack(f_ref[...]), ssmk_ref[lt, :, j * CH:(j + 1) * CH],
                             (((1,), (1,)), ((), ())), preferred_element_type=F32)
        slot = lt * NCH + j
        for p in range(NP):
            kr = kf[16 * p:16 * p + 8]
            ki = kf[16 * p + 8:16 * p + 16]
            if j == 0:
                kr = kr + ddf_ref[lt]
            kr, ki = kr * (1.0 / CH), ki * (1.0 / CH)
            kh_ref[slot, 24 * p:24 * p + 8, :] = kr
            kh_ref[slot, 24 * p + 8:24 * p + 16, :] = ki - kr
            kh_ref[slot, 24 * p + 16:24 * p + 24, :] = kr + ki

    def dft_u(b, lt, maybe_first=False):
        cs = lanes(lt)
        sk = sk_ref[:, cs].astype(F32)
        k = k_ref[b, :, cs].astype(F32)
        if maybe_first:
            halo = k_ref[jnp.maximum(b - 1, 0), TM - 8:TM, cs].astype(F32)
            halo = jnp.where(b > 0, halo, 0.0)
        else:
            halo = k_ref[b - 1, TM - 8:TM, cs].astype(F32)
        kext = jnp.concatenate([halo, k], axis=0)
        ks = k * sk[0:1, :]
        for t in range(1, 4):
            ks = ks + kext[8 - t:8 - t + TM, :] * sk[t:t + 1, :]
        kv = ks * v_ref[b, :, cs].astype(F32)
        for cc in range(2):
            uf = _dot(_unpack(f_ref[...]), kv[cc * CH:(cc + 1) * CH, :].astype(BF16))
            slot = lt * USL + UPAD + 2 * b + cc
            for p in range(NP):
                ur = uf[16 * p:16 * p + 8]
                ui = uf[16 * p + 8:16 * p + 16]
                uh_ref[slot, 24 * p:24 * p + 8, :] = ur + ui
                uh_ref[slot, 24 * p + 8:24 * p + 16, :] = ur
                uh_ref[slot, 24 * p + 16:24 * p + 24, :] = ui

    def mac(b, njs, lt, chained, paced=False):
        uw = uh_ref.at[pl.ds(lt * USL + UPAD + 2 * b + 2 - njs, njs)]
        for p in range(NP):
            base = {}
            for q in range(3):
                rr = pl.ds(24 * p + 8 * q, 8)
                acc = {}
                for o in 'ac':
                    if q == 1:
                        acc[o] = base[o]
                    elif q == 2:
                        acc[o] = link(o, base[o])
                kprev = None
                for t in range(njs):
                    u = uw[njs - 1 - t, rr, :]
                    k = kh_ref[lt * NCH + t, rr, :]
                    for o, kk in (('c', k), ('a', kprev)):
                        if kk is None:
                            continue
                        m = kk * u
                        if o not in acc:
                            acc[o] = link(o, m)
                        else:
                            acc[o] = acc[o] - m if q == 2 else acc[o] + m
                    kprev = k
                if q == 0:
                    base = acc
                else:
                    r0 = 16 * p + (8 if q == 1 else 0)
                    z_ref[2 * lt, r0:r0 + 8, :] = acc['a']
                    z_ref[2 * lt + 1, r0:r0 + 8, :] = acc['c']
                    if chained and q == 1:
                        chain.update(acc)
                    if chained and q == 2:
                        chain.update(a=acc['c'], c=acc['a'])
                        n = cfg['mac'][p % len(cfg['mac'])]
                        if paced and n:
                            pace('s1', link('s1', acc['a'] + acc['c']), n)

    def overlap(lt, cc, first=False):
        z = []
        for p in range(NP):
            re, im = slice(16 * p, 16 * p + 8), slice(16 * p + 8, 16 * p + 16)
            zr, zi = z_ref[2 * lt + cc, re, :], z_ref[2 * lt + cc, im, :]
            if cc == 0 and first:
                z.append((zr, zi))
            else:
                prev = zprev_ref.at[lt] if cc == 0 else z_ref.at[2 * lt]
                z.append((zr + prev[im, :], zi - prev[re, :]))
            if cc == 1:
                zprev_ref[lt, re, :] = zr
                zprev_ref[lt, im, :] = zi
        return z

    def inv(lt, first=False, ys=0):
        for cc in range(2):
            z = jnp.concatenate([t for pair in overlap(lt, cc, first) for t in pair], axis=0)
            y_ref[z1 + ys, cc * CH:(cc + 1) * CH, lanes(lt)] = _dot(_unpack(g_ref[...]), z.astype(BF16))

    def inv_vpu1(u, paced=True):
        lt, cc = u // 2, u % 2
        z = overlap(lt, cc)
        for h in range(2):
            zz = z[8 * h:8 * h + 8]
            if paced:
                zz[0] = (link('s1', zz[0][0]), zz[0][1])
            for n2, (re, im) in enumerate(_fft(zz)):
                if n2 > 0:
                    tr, ti = twb_ref[(h * 8 + n2) * 2], twb_ref[(h * 8 + n2) * 2 + 1]
                    re, im = re * tr - im * ti, re * ti + im * tr
                tb_ref[u, 144 * h + 9 * n2:144 * h + 9 * n2 + 8, :] = re
                tb_ref[u, 144 * h + 72 + 9 * n2:144 * h + 72 + 9 * n2 + 8, :] = im
            if paced:
                pace('s1', re, cfg['s1'][h % len(cfg['s1'])])

    def inv_vpu2(u):
        lt, cc = u // 2, u % 2
        ld = lambda o, sl: tb_ref[u, pl.ds(o + sl, 8, stride=9), :]
        xs = [(ld(144 * h, sl), ld(144 * h + 72, sl)) for h in range(2) for sl in range(8)]
        xe, xo = xs[0::2], xs[1::2]
        xe[0] = (link('s2', xe[0][0]), xe[0][1])
        ev = _fft(xe)
        ye = [_re_rot(ev[n1 % 8], np.pi * n1 / 32) for n1 in range(16)]
        pace('s2', ye[-1], cfg['s2'][0])
        xo[0] = (link('s2', xo[0][0]), xo[0][1])
        od = _fft(xo)
        for n1 in range(16):
            y = ye[n1] + _re_rot(od[n1 % 8], np.pi * n1 / 32 + 2 * np.pi * n1 / 16)
            y_ref[z1, cc * CH + 8 * n1:cc * CH + 8 * n1 + 8, lanes(lt)] = y
        pace('s2', y, cfg['s2'][1])

    def norm(x, name=None):
        m = jnp.sum(x, axis=-1, keepdims=True) * (1.0 / D)
        if name is not None:
            m = link(name, m, never_col)
        xc = x - m
        v = jnp.sum(xc * xc, axis=-1, keepdims=True) * (1.0 / D)
        return xc * lax.rsqrt(v + EPS)

    def modrow(i):
        return mod_ref[i, 0:1, :]

    blk = {}

    def set_blocks(bf, bl):
        if isinstance(bf, int):
            blk.update(xf=x1_ref.at[bf], hf=h2_ref.at[bf], xl=x1_ref.at[bl], hl=h2_ref.at[bl])
        else:
            xw, hw = x1_ref.at[pl.ds(bf, 2)], h2_ref.at[pl.ds(bf, 2)]
            blk.update(xf=xw.at[0], hf=hw.at[0], xl=xw.at[1], hl=hw.at[1])

    def ln_piece(b, r, paced, part=3, ys=0):
        name = 'ln%d' % (r % LN_CHAINS) if paced else None
        rs = slice(r * RC, (r + 1) * RC)
        if part & 1:
            x = q_ref[b, rs, :].astype(F32)
            h1 = norm(x, name) * modrow(1) + modrow(0)
            x1 = x + h1 * y_ref[z2 + ys, rs, :]
            blk['xl'][rs, :] = x1
            n2 = norm(x1)
            if part == 1:
                x1_ref[NB - 1 - b, rs, :] = n2
        else:
            n2 = x1_ref[NB - 1 - b, rs, :]
        if part & 2:
            h2 = n2 * modrow(4) + modrow(3)
            if paced:
                chain[name] = h2[:, 0:1]
            blk['hl'][r * RC // 2:(r + 1) * RC // 2, :] = _pack(h2)

    def mod_part(i):
        c = c_ref[...].astype(F32)
        sc = jnp.broadcast_to((c * jax.nn.sigmoid(c)).astype(BF16), (8, D))
        return _dot(sc, wmod_ref[i])

    def weight(raw, packed_ref, c, n, first):
        rows = span(c, n, 32)
        if not first:
            return _unpack(packed_ref[rows, :])
        w = raw()
        packed_ref[rows, :] = pltpu.bitcast(w, U32)
        return w

    def gate_up(cp, cj, first=False):
        c = 2 * cp + cj
        h2 = _unpack(blk['hf'][...])
        gate = _dot(h2, weight(lambda: wg_ref[cp, :, lanes(cj)], wgp_ref, c, D // 2, first))
        up = _dot(h2, weight(lambda: wu_ref[cp, :, lanes(cj)], wup_ref, c, D // 2, first))
        act_ref[span(cp, TM // 2, 32), lanes(cj)] = _pack(jnp.maximum(gate, 0.0) * up)

    def down(b, c, first=False):
        cs = lanes(c)
        a = jnp.concatenate([act_ref[span(j, TM // 2, 32), :] for j in range(NFT // 2)], axis=1)
        ff = _dot(_unpack(a), weight(lambda: wd_ref[:, cs], wdp_ref, c, FF // 2, first))
        o_ref[b, :, cs] = (blk['xf'][:, cs] + mod_ref[5, 0:1, cs] * ff).astype(BF16)

    def loop(lo, hi, body):
        def wrapped(i, carry):
            body(i)
            return carry
        lax.fori_loop(lo, hi, wrapped, 0)

    def prologue():
        for i in range(6):
            cp_x(i).start()
        for lt in range(NLT):
            cp_s(lt).start()
        for b in range(3):
            cp_k(b).start()
            cp_v(b).start()
        cp_q(0).start()
        cp_q(1).start()
        for i in range(5):
            cp_m(i).start()
        for i in range(WCH):
            cp_g(i).start()
            cp_u(i).start()
        cp_m(5).start()
        for i in range(3):
            cp_d(i).start()
        cp_k(3).start()
        cp_v(3).start()
        for i in range(3, NLT):
            cp_d(i).start()
        for b in range(2, NB):
            cp_q(b).start(priority=1)
            if b + 2 < NB:
                cp_k(b + 2).start(priority=1)
                cp_v(b + 2).start(priority=1)

        def zero_fill(j):
            for lt in range(NLT):
                uh_ref[lt * USL + j, 0:3 * CH, :] = jnp.zeros((3 * CH, 128), F32)
        loop(0, UPAD, zero_fill)
        for i in range(6):
            cp_x(i).wait()
        tw = tw_ref[...]
        for i in range(32):
            twb_ref[i] = jnp.broadcast_to(tw[:, i:i + 1], (8, 128))
        dd = dd_ref[...].astype(F32)
        for lt in range(NLT):
            ddf_ref[lt] = jnp.broadcast_to(dd[lt:lt + 1, :], (8, 128))

        def filter_spectra(lt):
            cp_s(lt).wait()
            for j in range(NCH):
                dft_k(lt, j)
        loop(0, NLT, filter_spectra)

        def input_spectra(b):
            cp_k(b).wait()
            cp_v(b).wait()
            for lt in range(NLT):
                dft_u(b, lt, True)
        loop(0, 3, input_spectra)

        def conv01(lt):
            mac(0, 2, lt, False)
            inv(lt, first=True)
            mac(1, 4, lt, False)
            inv(lt, ys=1)
        loop(0, NLT, conv01)

        def modulation(i):
            cp_m(i).wait()
            mod_ref[i] = mod_part(i)

        def ln01(part):
            def body(b):
                blk.update(xl=x1_ref.at[b], hl=h2_ref.at[b])
                for r in range(TM // RC):
                    ln_piece(b, r, False, part, b)
            loop(0, 2, body)

        def clear_staging(u):
            tb_ref[u] = jnp.zeros((TBR, 128), F32)
        loop(0, 2 * NLT, clear_staging)
        loop(0, 3, modulation)
        ga = mod_ref[2]
        mod_ref[0] = mod_ref[0] * ga
        mod_ref[1] = (1.0 + mod_ref[1]) * ga
        cp_q(0).wait()
        cp_q(1).wait()
        ln01(1)
        loop(3, 5, modulation)
        mod_ref[4] = 1.0 + mod_ref[4]
        ln01(2)

    def first_step():
        set_blocks(0, 1)

        def chunk(i):
            cp_g(i).wait()
            cp_u(i).wait()
            chain.clear()
            gate_up(i, 0, first=True)
            gate_up(i, 1, first=True)
            mac(2, 6, jnp.minimum(i, NLT - 1), True)
        loop(0, WCH, chunk)
        chain.clear()
        cp_m(5).wait()
        cp_d(0).wait()
        mod_ref[5] = mod_part(5)
        down(0, 0, first=True)
        for c in range(1, NLT):
            if c == 3:
                cp_k(3).wait()
                cp_v(3).wait()
            cp_d(c).wait()
            down(0, c, first=True)
            for u in {1: range(0, 4), 2: range(4, 8), 3: range(8, 10)}.get(c, ()):
                inv_vpu1(u, False)
            for lt in {3: (0, 1, 2, 3), 4: (4,)}.get(c, ()):
                dft_u(3, lt)
        cp_o(0).start()

    def step(b, do_dft, do_mac, do_ln):
        chain.clear()
        set_blocks(b, b + 1 if do_ln else b)
        if do_ln:
            for u in range(2 * NLT):
                inv_vpu2(u)
        if do_mac:
            for lt in range(NLT):
                mac(b + 2, NCH - 2 if do_dft else NCH, lt, True, True)
            for u in range(2 * NLT):
                inv_vpu1(u)
        for c in range(NFT + NLT):
            for lt in range(NLT):
                if do_dft and DFT_BEFORE[lt] == c:
                    dft_u(b + 3, lt)
            if c < NFT:
                gate_up(c // 2, c % 2)
            else:
                down(b, c - NFT)
                if not do_ln:
                    cp_l(c - NFT).start()
        if do_ln:
            for r in range(TM // RC):
                ln_piece(b + 1, r, True)
            cp_o(b).start()

    def tail():
        cfg.update(PACE_LAST_MAC)
        step(NB - 3, False, True, True)
        cfg.update(PACE_LAST_LN)
        step(NB - 2, False, False, True)
        step(NB - 1, False, False, False)
        for b in range(NB - 1):
            cp_o(b).wait()
        for c in range(NLT):
            cp_l(c).wait()

    pl.when(g == 0)(prologue)

    @pl.when(jnp.logical_and(g >= 2, g + 2 < NB))
    def _():
        cp_k(g + 2).wait()
        cp_v(g + 2).wait()

    @pl.when(g >= 2)
    def _():
        cp_q(g).wait()

    @pl.when(g == NB - 2)
    def _():
        cp_q(NB - 1).wait()

    pl.when(g == 1)(first_step)
    pl.when(jnp.logical_and(g >= 2, g <= NB - 3))(lambda: step(g - 1, True, True, True))
    pl.when(g == NB - 2)(tail)


@jax.jit
def pallas_adaLN_cond__ssm_conv_h3__glu_gated_reglu__prompt_kernel(
    A_q, A_k, A_v, A_shift_k, A_ssm_k, A_ssm_D, B_x, B_W_gate, B_W_up, B_W_down, c, w_mod,
):
    del B_x
    fwd, inv, tw = _dft_tables()
    hbm = pl.BlockSpec(memory_space=pl.ANY)
    out = pl.pallas_call(
        _kernel,
        grid=(NB - 1,),
        in_specs=[hbm] * 14,
        out_specs=hbm,
        out_shape=jax.ShapeDtypeStruct((NB, TM, D), BF16),
        scratch_shapes=[
            pltpu.VMEM((NB, TM, D), BF16),
            pltpu.VMEM((NB, TM, D), BF16),
            pltpu.VMEM((NB, TM, D), BF16),
            pltpu.VMEM((NB, TM, D), BF16),
            pltpu.VMEM((NLT, 128, S), BF16),
            pltpu.VMEM((WCH, D, FF // WCH), BF16),
            pltpu.VMEM((WCH, D, FF // WCH), BF16),
            pltpu.VMEM((FF, D), BF16),
            pltpu.VMEM((6, D, D), BF16),
            pltpu.SemaphoreType.DMA((71,)),
            pltpu.VMEM((8, 8, D), F32),
            pltpu.VMEM((NLT, 2 * CH, 128), F32),
            pltpu.VMEM((2 * NLT, 2 * CH, 128), F32),
            pltpu.VMEM((NB, TM // 2, D), U32),
            pltpu.VMEM((NB, TM, D), F32),
            pltpu.VMEM((NFT // 2 * TM // 2, 256), U32),
            pltpu.VMEM((2, TM, D), F32),
            pltpu.VMEM((NFT * D // 2, 128), U32),
            pltpu.VMEM((NFT * D // 2, 128), U32),
            pltpu.VMEM((NLT * FF // 2, 128), U32),
            pltpu.VMEM((NLT * NCH, KROWS, 128), F32),
            pltpu.VMEM((NLT * USL, UROWS, 128), F32),
            pltpu.VMEM((2 * NLT, TBR, 128), F32),
            pltpu.VMEM((32, 8, 128), F32),
            pltpu.VMEM((CH, CH), U32),
            pltpu.VMEM((CH // 2, 2 * CH), U32),
            pltpu.VMEM((8, 8, 128), F32),
            pltpu.VMEM((8, 128), F32),
            pltpu.VMEM((4, D), BF16),
            pltpu.VMEM((NLT, 128), BF16),
            pltpu.VMEM((1, D), BF16),
        ],
        compiler_params=pltpu.CompilerParams(
            dimension_semantics=("arbitrary",),
            vmem_limit_bytes=110 * 1024 * 1024,
            disable_bounds_checks=True,
            disable_semaphore_checks=True),
    )(A_q.reshape(NB, TM, D), A_k.reshape(NB, TM, D), A_v.reshape(NB, TM, D), A_shift_k.T,
      A_ssm_k.reshape(NLT, 128, S), A_ssm_D.reshape(NLT, 128), B_W_gate, B_W_up, B_W_down,
      c, w_mod, jnp.asarray(_pack_np(fwd)), jnp.asarray(_pack_np(inv)), jnp.asarray(tw))
    return out.reshape(1, S, D)
```

```python
import numpy as np
import jax
import jax.numpy as jnp
from jax import lax
import jax.experimental.pallas as pl
import jax.experimental.pallas.tpu as pltpu

S = 2048
D = 640
FF = 1536
CH = 128
NCH = S // CH
TM = 256
NB = S // TM
NLT = D // 128
NFT = FF // 128
NP = CH // 8
EPS = 1e-5
UPAD = 4
USL = UPAD + NCH
KROWS = 3 * CH + 8
UROWS = 3 * CH + 64
TBR = 320
WCH = 6
RC = 16
LN_CHAINS = 2
PACE_GU1 = dict(s1=(1,), s2=(1, 1))
PACE_DOWN01 = dict(mac=(1, 1, 0), s1=(1,))
PACE_STEADY = dict(mac=(1, 1, 1, 0, 1, 1, 1, 1), s1=(1, 2), s2=(1, 1))
PACE_LAST_MAC = dict(mac=(1,), s1=(1,), s2=(0, 1))
PACE_LAST_LN = dict(s2=(1, 1))
DFT_BEFORE = (1, 2, 3, 4, 16)
DFT3_BEFORE = (0, 0, 0, 1, 4)
DFT4_BEFORE = (3, 5, 6, 6, 8)
F32 = jnp.float32
BF16 = jnp.bfloat16
U32 = jnp.uint32


def _dft_tables():
    h, m2, sl = np.meshgrid(np.arange(2), np.arange(8), np.arange(8), indexing='ij')
    m = (8 * h + sl + 16 * m2).reshape(NP, 8)
    k = ((4 * m[:, :, None] + 1) * np.arange(CH)) % (4 * CH)
    ang = np.pi * k / (2 * CH)
    fwd = np.stack([np.cos(ang), np.sin(ang)], axis=1).reshape(2 * CH, CH)
    m1 = 8 * np.arange(2)[:, None, None] + np.arange(8)[None, None, :]
    n2 = np.arange(8)[None, :, None]
    tw = np.exp(-1j * np.pi * (4 * m1 + 1) * n2 / (2 * CH))
    tw = np.stack([tw.real, tw.imag], axis=2).reshape(32, 8).T
    tw = np.concatenate([tw, np.zeros((8, 96))], axis=1)
    return fwd, fwd.T, tw.astype(np.float32)


def _cmul(x, k, n):
    re, im = x
    k = k % n
    if k == 0:
        return x
    if 4 * k == n:
        return im, -re
    c, s = float(np.cos(2 * np.pi * k / n)), float(np.sin(2 * np.pi * k / n))
    if (8 * k) % n == 0:
        if c * s > 0:
            return (re + im) * c, (im - re) * c
        return (im - re) * s, (re + im) * -s
    return re * c + im * s, im * c - re * s


def _fft(xs):
    n = len(xs)
    if n == 1:
        return xs
    ev, od = _fft(xs[0::2]), _fft(xs[1::2])
    out = [None] * n
    for k in range(n // 2):
        (er, ei) = ev[k]
        if 4 * k == n:
            (tr, ti) = od[k]
            out[k] = (er + ti, ei - tr)
            out[k + n // 2] = (er - ti, ei + tr)
        else:
            tr, ti = _cmul(od[k], k, n)
            out[k] = (er + tr, ei + ti)
            out[k + n // 2] = (er - tr, ei - ti)
    return out


def _re_rot(x, ang):
    c, s = float(np.cos(ang)), float(np.sin(ang))
    if abs(s) < 1e-12:
        return x[0] if c > 0 else -x[0]
    if abs(c) < 1e-12:
        return x[1] if s > 0 else -x[1]
    return x[0] * c + x[1] * s


def _pack_np(a):
    u = np.ascontiguousarray(a, np.float32).view(np.uint32)
    b = ((u + 0x7FFF + ((u >> 16) & 1)) >> 16).astype(np.uint32)
    return b[0::2] | (b[1::2] << 16)


def _pack(x):
    return pltpu.bitcast(x.astype(BF16), U32)


def _unpack(x):
    return pltpu.bitcast(x, BF16)


def _dot(a, b):
    return jnp.dot(a, b, preferred_element_type=F32)


def _kernel(q_hbm, k_hbm, v_hbm, sk_hbm, ssmk_hbm, dd_hbm, wg_hbm, wu_hbm, wd_hbm,
            c_hbm, wmod_hbm, f_hbm, g_hbm, tw_hbm, o_hbm,
            q_ref, k_ref, v_ref, o_ref, ssmk_ref, wg_ref, wu_ref, wd_ref, wmod_ref, sems,
            mod_ref, zprev_ref, z_ref, h2_ref, x1_ref, act_ref, y_ref,
            wgp_ref, wup_ref, wdp_ref, kh_ref, uh_ref, tb_ref, twb_ref,
            f_ref, g_ref, ddf_ref, tw_ref, sk_ref, dd_ref, c_ref):
    g = pl.program_id(0)
    never8 = lax.broadcasted_iota(jnp.int32, (8, 128), 0) < g - 1000
    never_col = lax.broadcasted_iota(jnp.int32, (RC, 1), 0) < g - 1000
    z1 = lax.shift_right_logical(g, 10)
    z2 = lax.shift_right_logical(g, 11)
    chain = {}
    cfg = dict(PACE_STEADY)

    def link(name, m, mask=never8):
        prev = chain.get(name)
        return m if prev is None else jnp.where(mask, prev, m)

    def pace(name, v, n):
        for _ in range(n):
            v = pltpu.roll(v, 1, 1)
        chain[name] = v

    def span(i, w, align):
        if isinstance(i, int):
            return pl.ds(i * w, w)
        return pl.ds(pl.multiple_of(i * w, align), w)

    def lanes(i, w=128):
        return span(i, w, 128)

    sem_q, sem_k, sem_v, sem_o, sem_s, sem_m, sem_g, sem_u, sem_d, sem_l, sem_x = (
        0, 8, 16, 24, 32, 37, 43, 49, 55, 56, 61)

    def copy(src, dst, sem):
        return pltpu.make_async_copy(src, dst, sems.at[sem])

    cp_q = lambda b: copy(q_hbm.at[b], q_ref.at[b], sem_q + b)
    cp_k = lambda b: copy(k_hbm.at[b], k_ref.at[b], sem_k + b)
    cp_v = lambda b: copy(v_hbm.at[b], v_ref.at[b], sem_v + b)
    cp_o = lambda b: copy(o_ref.at[b], o_hbm.at[b], sem_o + b)
    cp_s = lambda i: copy(ssmk_hbm.at[i], ssmk_ref.at[i], sem_s + i)
    cp_m = lambda i: copy(wmod_hbm.at[:, lanes(i, D)], wmod_ref.at[i], sem_m + i)
    cp_g = lambda i: copy(wg_hbm.at[:, lanes(i, FF // WCH)], wg_ref.at[i], sem_g + i)
    cp_u = lambda i: copy(wu_hbm.at[:, lanes(i, FF // WCH)], wu_ref.at[i], sem_u + i)
    cp_d = lambda: copy(wd_hbm, wd_ref, sem_d)
    cp_l = lambda i: copy(o_ref.at[NB - 1, :, lanes(i)], o_hbm.at[NB - 1, :, lanes(i)], sem_l + i)
    cp_x = lambda i: copy((f_hbm, dd_hbm, sk_hbm, g_hbm, c_hbm, tw_hbm)[i],
                          (f_ref, dd_ref, sk_ref, g_ref, c_ref, tw_ref)[i], sem_x + i)

    def dft_k(lt, j, maybe_first):
        kf = lax.dot_general(_unpack(f_ref[...]), ssmk_ref[lt, :, lanes(j)],
                             (((1,), (1,)), ((), ())), preferred_element_type=F32)
        slot = lt * NCH + j
        for p in range(NP):
            kr = kf[16 * p:16 * p + 8]
            ki = kf[16 * p + 8:16 * p + 16]
            if maybe_first:
                kr = kr + jnp.where(j == 0, ddf_ref[lt], 0.0)
            kr, ki = kr * (1.0 / CH), ki * (1.0 / CH)
            kh_ref[slot, 24 * p:24 * p + 8, :] = kr
            kh_ref[slot, 24 * p + 8:24 * p + 16, :] = ki - kr
            kh_ref[slot, 24 * p + 16:24 * p + 24, :] = kr + ki

    def dft_u(b, lt, maybe_first=False):
        cs = lanes(lt)
        sk = sk_ref[:, cs].astype(F32)
        k = k_ref[b, :, cs].astype(F32)
        if maybe_first:
            halo = k_ref[jnp.maximum(b - 1, 0), TM - 8:TM, cs].astype(F32)
            halo = jnp.where(b > 0, halo, 0.0)
        else:
            halo = k_ref[b - 1, TM - 8:TM, cs].astype(F32)
        kext = jnp.concatenate([halo, k], axis=0)
        ks = k * sk[0:1, :]
        for t in range(1, 4):
            ks = ks + kext[8 - t:8 - t + TM, :] * sk[t:t + 1, :]
        kv = ks * v_ref[b, :, cs].astype(F32)
        for cc in range(2):
            uf = _dot(_unpack(f_ref[...]), kv[cc * CH:(cc + 1) * CH, :].astype(BF16))
            slot = lt * USL + UPAD + 2 * b + cc
            for p in range(NP):
                ur = uf[16 * p:16 * p + 8]
                ui = uf[16 * p + 8:16 * p + 16]
                uh_ref[slot, 24 * p:24 * p + 8, :] = ur + ui
                uh_ref[slot, 24 * p + 8:24 * p + 16, :] = ur
                uh_ref[slot, 24 * p + 16:24 * p + 24, :] = ui

    def mac(b, njs, lt, chained, paced=False):
        uw = uh_ref.at[pl.ds(lt * USL + UPAD + 2 * b + 2 - njs, njs)]
        for p in range(NP):
            base = {}
            for q in range(3):
                rr = pl.ds(24 * p + 8 * q, 8)
                acc = {}
                for o in 'ac':
                    if q == 1:
                        acc[o] = base[o]
                    elif q == 2:
                        acc[o] = link(o, base[o])
                kprev = None
                for t in range(njs):
                    u = uw[njs - 1 - t, rr, :]
                    k = kh_ref[lt * NCH + t, rr, :]
                    for o, kk in (('c', k), ('a', kprev)):
                        if kk is None:
                            continue
                        m = kk * u
                        if o not in acc:
                            acc[o] = link(o, m)
                        else:
                            acc[o] = acc[o] - m if q == 2 else acc[o] + m
                    kprev = k
                if q == 0:
                    base = acc
                else:
                    r0 = 16 * p + (8 if q == 1 else 0)
                    z_ref[2 * lt, r0:r0 + 8, :] = acc['a']
                    z_ref[2 * lt + 1, r0:r0 + 8, :] = acc['c']
                    if chained and q == 1:
                        chain.update(acc)
                    if chained and q == 2:
                        chain.update(a=acc['c'], c=acc['a'])
                        n = cfg['mac'][p % len(cfg['mac'])]
                        if paced and n:
                            pace('s1', link('s1', acc['a'] + acc['c']), n)

    def overlap(lt, cc, first=False, keep=True):
        z = []
        for p in range(NP):
            re, im = slice(16 * p, 16 * p + 8), slice(16 * p + 8, 16 * p + 16)
            zr, zi = z_ref[2 * lt + cc, re, :], z_ref[2 * lt + cc, im, :]
            if cc == 0 and first:
                z.append((zr, zi))
            else:
                prev = zprev_ref.at[lt] if cc == 0 else z_ref.at[2 * lt]
                z.append((zr + prev[im, :], zi - prev[re, :]))
            if cc == 1 and keep:
                zprev_ref[lt, re, :] = zr
                zprev_ref[lt, im, :] = zi
        return z

    def inv(lt, first=False, ys=0):
        for cc in range(2):
            z = jnp.concatenate([t for pair in overlap(lt, cc, first) for t in pair], axis=0)
            y_ref[z1 + ys, cc * CH:(cc + 1) * CH, lanes(lt)] = _dot(_unpack(g_ref[...]), z.astype(BF16))

    def inv_vpu1(lt, cc, paced=True, keep=True):
        u = 2 * lt + cc
        z = overlap(lt, cc, keep=keep)
        for h in range(2):
            zz = z[8 * h:8 * h + 8]
            if paced:
                zz[0] = (link('s1', zz[0][0]), zz[0][1])
            for n2, (re, im) in enumerate(_fft(zz)):
                if n2 > 0:
                    tr, ti = twb_ref[(h * 8 + n2) * 2], twb_ref[(h * 8 + n2) * 2 + 1]
                    re, im = re * tr - im * ti, re * ti + im * tr
                tb_ref[u, 144 * h + 9 * n2:144 * h + 9 * n2 + 8, :] = re
                tb_ref[u, 144 * h + 72 + 9 * n2:144 * h + 72 + 9 * n2 + 8, :] = im
            if paced:
                pace('s1', re, cfg['s1'][h % len(cfg['s1'])])

    def inv_vpu2(lt, cc):
        u = 2 * lt + cc
        ld = lambda o, sl: tb_ref[u, pl.ds(o + sl, 8, stride=9), :]
        xs = [(ld(144 * h, sl), ld(144 * h + 72, sl)) for h in range(2) for sl in range(8)]
        xe, xo = xs[0::2], xs[1::2]
        xe[0] = (link('s2', xe[0][0]), xe[0][1])
        ev = _fft(xe)
        ye = [_re_rot(ev[n1 % 8], np.pi * n1 / 32) for n1 in range(16)]
        pace('s2', ye[-1], cfg['s2'][0])
        xo[0] = (link('s2', xo[0][0]), xo[0][1])
        od = _fft(xo)
        for n1 in range(16):
            y = ye[n1] + _re_rot(od[n1 % 8], np.pi * n1 / 32 + 2 * np.pi * n1 / 16)
            y_ref[z1, cc * CH + 8 * n1:cc * CH + 8 * n1 + 8, lanes(lt)] = y
        pace('s2', y, cfg['s2'][1])

    def norm(x, name=None):
        m = jnp.sum(x, axis=-1, keepdims=True) * (1.0 / D)
        if name is not None:
            m = link(name, m, never_col)
        xc = x - m
        v = jnp.sum(xc * xc, axis=-1, keepdims=True) * (1.0 / D)
        return xc * lax.rsqrt(v + EPS)

    def modrow(i):
        return mod_ref[i, 0:1, :]

    blk = {}

    def set_blocks(bf, bl):
        if isinstance(bf, int):
            blk.update(xf=x1_ref.at[bf], hf=h2_ref.at[bf], xl=x1_ref.at[bl], hl=h2_ref.at[bl])
        else:
            xw, hw = x1_ref.at[pl.ds(bf, 2)], h2_ref.at[pl.ds(bf, 2)]
            blk.update(xf=xw.at[0], hf=hw.at[0], xl=xw.at[1], hl=hw.at[1])

    def ln_piece(b, r, paced, part=3, ys=0):
        name = 'ln%d' % (r % LN_CHAINS) if paced else None
        rs = slice(r * RC, (r + 1) * RC)
        if part & 1:
            x = q_ref[b, rs, :].astype(F32)
            h1 = norm(x, name) * modrow(1) + modrow(0)
            x1 = x + h1 * y_ref[z2 + ys, rs, :]
            blk['xl'][rs, :] = x1
            n2 = norm(x1)
            if part == 1:
                x1_ref[NB - 1 - b, rs, :] = n2
        else:
            n2 = x1_ref[NB - 1 - b, rs, :]
        if part & 2:
            h2 = n2 * modrow(4) + modrow(3)
            if paced:
                chain[name] = h2[:, 0:1]
            blk['hl'][r * RC // 2:(r + 1) * RC // 2, :] = _pack(h2)

    def mod_part(i):
        c = c_ref[...].astype(F32)
        sc = jnp.broadcast_to((c * jax.nn.sigmoid(c)).astype(BF16), (8, D))
        return _dot(sc, wmod_ref[i])

    def weight(raw, packed_ref, c, n, first):
        rows = span(c, n, 32)
        if not first:
            return _unpack(packed_ref[rows, :])
        w = raw()
        packed_ref[rows, :] = pltpu.bitcast(w, U32)
        return w

    def gate_up(cp, cj, first=False, a0=0):
        c = 2 * cp + cj
        h2 = _unpack(blk['hf'][...])
        gate = _dot(h2, weight(lambda: wg_ref[cp, :, lanes(cj)], wgp_ref, c, D // 2, first))
        up = _dot(h2, weight(lambda: wu_ref[cp, :, lanes(cj)], wup_ref, c, D // 2, first))
        act_ref[span(a0 + cp, TM // 2, 32), lanes(cj)] = _pack(jnp.maximum(gate, 0.0) * up)

    def down(b, c, first=False, a0=0):
        cs = lanes(c)
        a = jnp.concatenate([act_ref[span(a0 + j, TM // 2, 32), :] for j in range(NFT // 2)], axis=1)
        ff = _dot(_unpack(a), weight(lambda: wd_ref[:, cs], wdp_ref, c, FF // 2, first))
        o_ref[b, :, cs] = (blk['xf'][:, cs] + mod_ref[5, 0:1, cs] * ff).astype(BF16)

    def loop(lo, hi, body):
        def wrapped(i, carry):
            body(i)
            return carry
        lax.fori_loop(lo, hi, wrapped, 0)

    def prologue():
        for i in range(6):
            cp_x(i).start()
        for lt in range(NLT):
            cp_s(lt).start()
        for b in range(3):
            cp_k(b).start()
            cp_v(b).start()
        cp_q(0).start()
        cp_q(1).start()
        for i in range(5):
            cp_m(i).start()
        for i in range(WCH):
            cp_g(i).start()
            cp_u(i).start()
        cp_m(5).start()
        cp_d().start()
        cp_k(3).start()
        cp_v(3).start()
        for b in range(2, NB):
            cp_q(b).start(priority=1)
            if b + 2 < NB:
                cp_k(b + 2).start(priority=1)
                cp_v(b + 2).start(priority=1)

        def zero_fill(j):
            for lt in range(NLT):
                uh_ref[lt * USL + j, 0:3 * CH, :] = jnp.zeros((3 * CH, 128), F32)
        loop(0, UPAD, zero_fill)

        def clear_staging(u):
            tb_ref[u] = jnp.zeros((TBR, 128), F32)
        loop(0, 2 * NLT, clear_staging)
        for i in range(6):
            cp_x(i).wait()
        tw = tw_ref[...]
        for i in range(32):
            twb_ref[i] = jnp.broadcast_to(tw[:, i:i + 1], (8, 128))
        dd = dd_ref[...].astype(F32)
        for lt in range(NLT):
            ddf_ref[lt] = jnp.broadcast_to(dd[lt:lt + 1, :], (8, 128))

        def filter_spectra(i):
            lt, half = i // 2, i % 2

            @pl.when(half == 0)
            def _():
                cp_s(lt).wait()
            for j in range(NCH // 2):
                dft_k(lt, half * (NCH // 2) + j, j == 0)
        loop(0, 2 * NLT, filter_spectra)

        def input_spectra(b):
            cp_k(b).wait()
            cp_v(b).wait()
            for lt in range(NLT):
                dft_u(b, lt, True)
        loop(0, 3, input_spectra)

        def conv01(lt):
            mac(0, 2, lt, False)
            inv(lt, first=True)
            mac(1, 4, lt, False)
            inv(lt, ys=1)
        loop(0, NLT, conv01)

        def ln01(part):
            def body(b):
                blk.update(xl=x1_ref.at[b], hl=h2_ref.at[b])
                for r in range(TM // RC):
                    ln_piece(b, r, False, part, b)
            loop(0, 2, body)
        cp_q(0).wait()
        cp_q(1).wait()

        def modulation(i):
            cp_m(i).wait()
            mod_ref[i] = mod_part(i)

            @pl.when(i == 2)
            def _():
                ga = mod_ref[2]
                mod_ref[0] = mod_ref[0] * ga
                mod_ref[1] = (1.0 + mod_ref[1]) * ga
                ln01(1)
        loop(0, 5, modulation)
        mod_ref[4] = 1.0 + mod_ref[4]
        ln01(2)

    def first_step():
        set_blocks(0, 1)

        def chunk(i):
            cp_g(i).wait()
            cp_u(i).wait()
            chain.clear()
            gate_up(i, 0, first=True)
            gate_up(i, 1, first=True)
            lt = jnp.minimum(i, NLT - 1)
            mac(2, 6, lt, True)
        loop(0, WCH, chunk)

        def chunk1(i):
            chain.clear()
            cfg.update(PACE_GU1)
            set_blocks(1, 1)
            for j in range(3):
                gate_up(3 * i + j, 0, a0=NFT // 2)
                gate_up(3 * i + j, 1, a0=NFT // 2)
            for j in range(3):
                lt = jnp.minimum(3 * i + j, NLT - 1)
                for cc in range(2):
                    inv_vpu1(lt, cc, keep=False)
                    inv_vpu2(lt, cc)
        loop(0, WCH // 3, chunk1)
        cp_m(5).wait()
        cp_d().wait()
        cp_q(2).wait()
        for b in (3, 4):
            cp_k(b).wait()
            cp_v(b).wait()
        chain.clear()
        cfg.update(PACE_DOWN01)
        mod_ref[5] = mod_part(5)
        for lt in range(NLT):
            zprev_ref[lt] = z_ref[2 * lt + 1]
        set_blocks(0, 2)
        for c in range(2 * NLT):
            if c == NLT:
                set_blocks(1, 2)
            for lt in range(NLT):
                if DFT3_BEFORE[lt] == c:
                    dft_u(3, lt)
                    mac(3, 8, lt, True, True)
                if DFT4_BEFORE[lt] == c:
                    dft_u(4, lt)
            down(c // NLT, c % NLT, first=(c < NLT), a0=(c // NLT) * (NFT // 2))
            if c % NLT == NLT - 1:
                cp_o(c // NLT).start()
        for u in range(2 * NLT):
            inv_vpu1(u // 2, u % 2)
        for r in range(TM // RC):
            ln_piece(2, r, True)
        cfg.update(PACE_STEADY)

    def step(b, do_dft, do_mac, do_ln):
        chain.clear()
        set_blocks(b, b + 1 if do_ln else b)
        if do_ln:
            for u in range(2 * NLT):
                inv_vpu2(u // 2, u % 2)
        if do_mac:
            for lt in range(NLT):
                mac(b + 2, NCH - 2 if do_dft else NCH, lt, True, True)
            for u in range(2 * NLT):
                inv_vpu1(u // 2, u % 2)
        for c in range(NFT + NLT):
            for lt in range(NLT):
                if do_dft and DFT_BEFORE[lt] == c:
                    dft_u(b + 3, lt)
            if c < NFT:
                gate_up(c // 2, c % 2)
            else:
                down(b, c - NFT)
                if not do_ln:
                    cp_l(c - NFT).start()
        if do_ln:
            for r in range(TM // RC):
                ln_piece(b + 1, r, True)
            cp_o(b).start()

    def tail():
        cfg.update(PACE_LAST_MAC)
        step(NB - 3, False, True, True)
        cfg.update(PACE_LAST_LN)
        step(NB - 2, False, False, True)
        step(NB - 1, False, False, False)
        for b in range(NB - 1):
            cp_o(b).wait()
        for c in range(NLT):
            cp_l(c).wait()

    pl.when(g == 0)(prologue)

    @pl.when(jnp.logical_and(g >= 2, g + 3 < NB))
    def _():
        cp_k(g + 3).wait()
        cp_v(g + 3).wait()

    @pl.when(g >= 2)
    def _():
        cp_q(g + 1).wait()

    @pl.when(g == NB - 3)
    def _():
        cp_q(NB - 1).wait()

    pl.when(g == 1)(first_step)
    pl.when(jnp.logical_and(g >= 2, g <= NB - 4))(lambda: step(g, True, True, True))
    pl.when(g == NB - 3)(tail)


@jax.jit
def pallas_adaLN_cond__ssm_conv_h3__glu_gated_reglu__prompt_kernel(
    A_q, A_k, A_v, A_shift_k, A_ssm_k, A_ssm_D, B_x, B_W_gate, B_W_up, B_W_down, c, w_mod,
):
    del B_x
    fwd, inv, tw = _dft_tables()
    hbm = pl.BlockSpec(memory_space=pl.ANY)
    out = pl.pallas_call(
        _kernel,
        grid=(NB - 2,),
        in_specs=[hbm] * 14,
        out_specs=hbm,
        out_shape=jax.ShapeDtypeStruct((NB, TM, D), BF16),
        scratch_shapes=[
            pltpu.VMEM((NB, TM, D), BF16),
            pltpu.VMEM((NB, TM, D), BF16),
            pltpu.VMEM((NB, TM, D), BF16),
            pltpu.VMEM((NB, TM, D), BF16),
            pltpu.VMEM((NLT, 128, S), BF16),
            pltpu.VMEM((WCH, D, FF // WCH), BF16),
            pltpu.VMEM((WCH, D, FF // WCH), BF16),
            pltpu.VMEM((FF, D), BF16),
            pltpu.VMEM((6, D, D), BF16),
            pltpu.SemaphoreType.DMA((67,)),
            pltpu.VMEM((8, 8, D), F32),
            pltpu.VMEM((NLT, 2 * CH, 128), F32),
            pltpu.VMEM((2 * NLT, 2 * CH, 128), F32),
            pltpu.VMEM((NB, TM // 2, D), U32),
            pltpu.VMEM((NB, TM, D), F32),
            pltpu.VMEM((NFT * TM // 2, 256), U32),
            pltpu.VMEM((2, TM, D), F32),
            pltpu.VMEM((NFT * D // 2, 128), U32),
            pltpu.VMEM((NFT * D // 2, 128), U32),
            pltpu.VMEM((NLT * FF // 2, 128), U32),
            pltpu.VMEM((NLT * NCH, KROWS, 128), F32),
            pltpu.VMEM((NLT * USL, UROWS, 128), F32),
            pltpu.VMEM((2 * NLT, TBR, 128), F32),
            pltpu.VMEM((32, 8, 128), F32),
            pltpu.VMEM((CH, CH), U32),
            pltpu.VMEM((CH // 2, 2 * CH), U32),
            pltpu.VMEM((8, 8, 128), F32),
            pltpu.VMEM((8, 128), F32),
            pltpu.VMEM((4, D), BF16),
            pltpu.VMEM((NLT, 128), BF16),
            pltpu.VMEM((1, D), BF16),
        ],
        compiler_params=pltpu.CompilerParams(
            dimension_semantics=("arbitrary",),
            vmem_limit_bytes=110 * 1024 * 1024,
            disable_bounds_checks=True,
            disable_semaphore_checks=True),
    )(A_q.reshape(NB, TM, D), A_k.reshape(NB, TM, D), A_v.reshape(NB, TM, D), A_shift_k.T,
      A_ssm_k.reshape(NLT, 128, S), A_ssm_D.reshape(NLT, 128), B_W_gate, B_W_up, B_W_down,
      c, w_mod, jnp.asarray(_pack_np(fwd)), jnp.asarray(_pack_np(inv)), jnp.asarray(tw))
    return out.reshape(1, S, D)
```
